```python
import jax
import jax.numpy as jnp

def _softmax(x, axis=-1):
    return jax.nn.softmax(x, axis=axis)
def _gelu(x):
    return jax.nn.gelu(x, approximate=True)
def _silu(x):
    return jax.nn.silu(x)
def _sigmoid(x):
    return jax.nn.sigmoid(x)
def _layernorm(x, axis=-1, eps=1e-5):
    m = jnp.mean(x, axis=axis, keepdims=True)
    v = jnp.var(x, axis=axis, keepdims=True)
    return (x - m) / jnp.sqrt(v + eps)
def _scatter_add(tgt, idx, src, axis=0):
    return tgt.at[idx].add(src)
def _segment_sum(src, seg, n):
    return jax.ops.segment_sum(src, seg, n)
class _Rng:
    def __init__(self, key):
        self._k = key
    def _next(self):
        self._k, sub = jax.random.split(self._k)
        return sub
    def normal(self, shape):
        return jax.random.normal(self._next(), shape, dtype=jnp.bfloat16)
    def randint(self, lo, hi, shape):
        return jax.random.randint(self._next(), shape, lo, hi, dtype=jnp.int32)
    def uniform(self, shape, lo=0.0, hi=1.0):
        return jax.random.uniform(self._next(), shape, jnp.bfloat16, lo, hi)
    def permutation(self, n):
        return jax.random.permutation(self._next(), n)


kernel_name = 'interleave_layers__sliding_block__moe_arch_mod__prompt'

def setup_inputs():
    _rng = _Rng(jax.random.key(int.from_bytes(__import__("os").urandom(4), "little")))
    _w = (lambda a: (lambda t: t.astype(jnp.bfloat16) if jnp.issubdtype(t.dtype, jnp.floating) else t)(jnp.asarray(a)))
    def _A_setup():
        B, S, D = 1, 2048, 1024
        return {
            "x": _w((lambda *s: _rng.normal(s) * 0.05)(B, S, D)),
            "wqkv": _w((lambda *s: _rng.normal(s) * 0.05)(D, 3 * D)),
            "wo": _w((lambda *s: _rng.normal(s) * 0.05)(D, D)),
        }
    _A_in = _A_setup()

    def _B_setup():
        B, S, D, F, C = 1, 2048, 1024, 3584, 1
        return {
            "x": _w((lambda *s: _rng.normal(s) * 0.05)(B, S, D)),
            "w_r": _w((lambda *s: _rng.normal(s) * 0.05)(D)),
            "w_gate": _w((lambda *s: _rng.normal(s) * 0.05)(D, F)),
            "w_up": _w((lambda *s: _rng.normal(s) * 0.05)(D, F)),
            "w_down": _w((lambda *s: _rng.normal(s) * 0.05)(F, D)),
        }
    _B_in = _B_setup()

    return {
        "A_x": _A_in["x"],
        "A_wqkv": _A_in["wqkv"],
        "A_wo": _A_in["wo"],
        "B_x": _B_in["x"],
        "B_w_r": _B_in["w_r"],
        "B_w_gate": _B_in["w_gate"],
        "B_w_up": _B_in["w_up"],
        "B_w_down": _B_in["w_down"],
    }

def reference(A_x, A_wqkv, A_wo, B_x, B_w_r, B_w_gate, B_w_up, B_w_down):
    def _A_ref(x, wqkv, wo):
        B, S, D = x.shape
        H = 32; Dh = D // H; W = 256
        qkv = (lambda x, *d: x.transpose(*d))((x @ wqkv).reshape(B, S, 3, H, Dh), 2, 0, 3, 1, 4)
        q, k, v = qkv[0], qkv[1], qkv[2]
        scores = jnp.einsum("bhqd,bhkd->bhqk", q, k) * (Dh ** -0.5)
        idx = jnp.arange(S)
        mask = (idx[:, None] - idx[None, :] >= 0) & (idx[:, None] - idx[None, :] < W)
        scores = jnp.where(mask[None, None], scores, -1e9)
        p = _softmax(scores, axis=-1)
        o = jnp.einsum("bhqk,bhkd->bhqd", p, v)
        return (lambda x, *d: x.transpose(*d))(o, 0, 2, 1, 3).reshape(B, S, D) @ wo

    def _B_ref(x, w_r, w_gate, w_up, w_down):
        B, S, D = x.shape
        C = 1
        r = x @ w_r
        idx = jnp.argsort(-r, axis=-1)[:, :C]
        idx_e = jnp.repeat(idx.reshape(B, C, 1), D, axis=2)
        x_sel = jnp.take_along_axis(x, idx_e, axis=1)
        g = _silu(x_sel @ w_gate)
        u = x_sel @ w_up
        y = (g * u) @ w_down
        r_sel = _sigmoid(jnp.take_along_axis(r, idx, axis=1))
        y = y * r_sel.reshape(B, C, 1)
        b_off = (jnp.arange(B) * S).reshape(B, 1)
        flat_idx = (idx + b_off).reshape(B * C)
        zero = (x * 0.0).reshape(B * S, D)
        upd = _scatter_add(zero, flat_idx, y.reshape(B * C, D), axis=0)
        return x + upd.reshape(B, S, D)

    x = A_x
    x = x + _A_ref(_layernorm(x, axis=-1), A_wqkv, A_wo)
    x = x + _B_ref(_layernorm(x, axis=-1), B_w_r, B_w_gate, B_w_up, B_w_down)
    x = x + _A_ref(_layernorm(x, axis=-1), A_wqkv, A_wo)
    x = x + _B_ref(_layernorm(x, axis=-1), B_w_r, B_w_gate, B_w_up, B_w_down)
    return x
```

```python
import jax
import jax.numpy as jnp
import numpy as np
from jax import lax
import jax.experimental.pallas as pl
import jax.experimental.pallas.tpu as pltpu

S, D, F = 2048, 1024, 3584
NHG = 8
NQB = S // 128
TM = 256
NC = S // TM
FC = 512
BF, F32 = jnp.bfloat16, jnp.float32
NEG = -1e9

_bf = lambda v: float(np.asarray(v, dtype=jnp.bfloat16).astype(np.float32))
QSCALE = _bf(32 ** -0.5) * float(np.log2(np.e))
EPS = _bf(1e-5)


def _rb(x):
    return x.astype(BF).astype(F32)


def _ln(x):
    m = jnp.mean(x, axis=1, keepdims=True)
    xc = x - m
    v = jnp.mean(xc * xc, axis=1, keepdims=True)
    sd = _rb(jnp.sqrt(_rb(_rb(v) + EPS)))
    return xc * (1.0 / sd)


def _nt(a, b):
    return lax.dot_general(a, b, (((1,), (1,)), ((), ())), preferred_element_type=F32)


def _nn(a, b):
    return jnp.dot(a, b, preferred_element_type=F32)


def _kernel(wr_ref, x_hbm, wqkv_hbm, wo_hbm, wg_hbm, wu_hbm, wd_hbm, out_hbm,
            x_s, h_s, x1_s, o_s, w_s, wo_s, wg_s, wu_s, wd_s, wt_s, qt_s, k_s, vt_s,
            x_sem, w_sem, f_sem, o_sem):
    def x_copy(c):
        rows = pl.ds(c * TM, TM)
        return pltpu.make_async_copy(x_hbm.at[rows], x_s.at[rows], x_sem.at[c])

    def w_copy(j, g):
        col = pl.multiple_of(j * D + g * 128, 128)
        return pltpu.make_async_copy(wqkv_hbm.at[:, pl.ds(col, 128)], w_s.at[j, g], w_sem.at[j, g])

    def o_copy(c):
        rows = pl.ds(pl.multiple_of(c * TM, TM), TM)
        return pltpu.make_async_copy(x_s.at[rows], out_hbm.at[rows], o_sem.at[c])

    f_copies = [pltpu.make_async_copy(a, b, f_sem.at[i]) for i, (a, b) in enumerate(
        ((wo_hbm, wo_s), (wg_hbm, wg_s), (wu_hbm, wu_s), (wd_hbm, wd_s)))]

    x_copy(0).start()
    for j in range(3):
        w_copy(j, 0).start()
    for c in range(1, NC):
        x_copy(c).start()
    for g in range(1, NHG):
        for j in range(3):
            w_copy(j, g).start()
    for cp in f_copies:
        cp.start()

    row = lax.broadcasted_iota(jnp.int32, (128, 128), 0)
    col = lax.broadcasted_iota(jnp.int32, (128, 128), 1)
    tri = row <= col

    def prep_w(g):
        wt_s[0:128, :] = w_s[0, g].T
        wt_s[128:256, :] = w_s[2, g].T

    def qkv(g, slot, c):
        rows = pl.ds(c * TM, TM)
        h = h_s[rows, :]
        qv = _nt(wt_s[...], h)
        qt_s[slot, :, rows] = (qv[:128] * QSCALE).astype(BF)
        vt_s[slot, :, rows] = qv[128:].astype(BF)
        k_s[slot, rows, :] = _nn(h, w_s[1, g]).astype(BF)

    def qk(slot, b):
        q0 = b * 128
        if b >= 2:
            pieces = []
            for i in range(0, 128, 16):
                pieces += [k_s[slot, q0 - 256 + i:q0 - 240 + i, :], k_s[slot, q0 + i:q0 + i + 16, :]]
            pieces.append(k_s[slot, q0 - 128:q0, :])
            kb = jnp.concatenate(pieces, 0)
        else:
            kb = k_s[slot, 0:q0 + 128, :]
        ws = []
        for h in range(4):
            parts = [qt_s[slot, h * 32:(h + 1) * 32, q0:q0 + 128]]
            if h > 0:
                parts = [jnp.zeros((32 * h, 128), BF)] + parts
            if h < 3:
                parts = parts + [jnp.zeros((96 - 32 * h, 128), BF)]
            ws.append(jnp.concatenate(parts, 0))
        sall = _nn(kb, jnp.concatenate(ws, 1))
        res = []
        for h in range(4):
            s = sall[:, h * 128:(h + 1) * 128]
            if b >= 2:
                first = jnp.concatenate([s[2 * i:2 * i + 16] for i in range(0, 128, 16)], 0)
                last = jnp.concatenate([s[2 * i + 16:2 * i + 32] for i in range(0, 128, 16)], 0)
                s = jnp.concatenate([jnp.where(tri, last, first), s[256:]], 0)
            elif b == 1:
                s = jnp.concatenate([jnp.where(tri, s[128:], NEG), s[:128]], 0)
            else:
                s = jnp.where(tri, s, NEG)
            res.append((s, jnp.max(s, axis=0, keepdims=True)))
        return res

    def softmax_pv(g, slot, b, res):
        q0 = b * 128
        outs = []
        for h, (s, m) in enumerate(res):
            p = jnp.exp2(s - m)
            l = jnp.sum(p, axis=0, keepdims=True)
            last = jnp.where(tri, p[:128], 0.0)
            if b >= 2:
                pp = jnp.concatenate([jnp.where(tri, 0.0, p[:128]), p[128:], last], 0)
            elif b == 1:
                pp = jnp.concatenate([p[128:], last], 0)
            else:
                pp = last
            oh = _nn(vt_s[slot, h * 32:(h + 1) * 32, max(q0 - 256, 0):q0 + 128], pp.astype(BF))
            outs.append(oh * (1.0 / l))
        o_s[g, q0:q0 + 128, :] = jnp.concatenate(outs, 0).T.astype(BF)

    def layer(li, carry):
        first = li == 0

        @pl.when(first)
        def _():
            for j in range(3):
                w_copy(j, 0).wait()
            x_copy(0).wait()

        prep_w(0)
        h_s[0:TM, :] = _ln(x_s[0:TM, :].astype(F32)).astype(BF)

        def p1(c, _):
            @pl.when(first)
            def _():
                rows = pl.ds(pl.multiple_of((c + 1) * TM, TM), TM)
                pltpu.make_async_copy(x_hbm.at[rows], x_s.at[rows], x_sem.at[c + 1]).wait()

            rows = pl.ds(pl.multiple_of(c * TM, TM), TM)
            nrows = pl.ds(pl.multiple_of((c + 1) * TM, TM), TM)
            h = h_s[rows, :]
            qv = _nt(wt_s[...], h)
            kk = _nn(h, w_s[1, 0])
            h_s[nrows, :] = _ln(x_s[nrows, :].astype(F32)).astype(BF)
            qt_s[0, :, rows] = (qv[:128] * QSCALE).astype(BF)
            vt_s[0, :, rows] = qv[128:].astype(BF)
            k_s[0, rows, :] = kk.astype(BF)
            return _

        lax.fori_loop(0, NC - 1, p1, None)
        qkv(0, 0, NC - 1)

        def attn(g, slot, with_proj):
            nxt = qk(slot, 0)
            for b in range(NQB):
                cur = nxt
                if b + 1 < NQB:
                    nxt = qk(slot, b + 1)
                if with_proj and b % 2 == 0:
                    qkv(g + 1, 1 - slot, b // 2)
                softmax_pv(g, slot, b, cur)

        def p2(g, _):
            @pl.when(first)
            def _():
                for j in range(3):
                    w_copy(j, g + 1).wait()

            prep_w(g + 1)
            attn(g, g % 2, True)
            return _

        lax.fori_loop(0, NHG - 1, p2, None)
        attn(NHG - 1, (NHG - 1) % 2, False)

        @pl.when(first)
        def _():
            f_copies[0].wait()

        wr = wr_ref[...].astype(F32)

        def oproj(c):
            rows = pl.ds(pl.multiple_of(c * TM, TM), TM)
            o = jnp.concatenate([o_s[g, rows, :] for g in range(NHG)], 1)
            x1_s[rows, :] = (x_s[rows, :].astype(F32) + _nn(o, wo_s[...])).astype(BF)

        def post(c, best):
            bv, bi = best
            rows = pl.ds(pl.multiple_of(c * TM, TM), TM)
            x1 = x1_s[rows, :].astype(F32)
            hb = _ln(x1).astype(BF)
            h_s[rows, :] = hb
            h = hb.astype(F32)
            x_s[rows, :] = (x1 + h).astype(BF)
            r = _rb(jnp.sum(h * wr, axis=1, keepdims=True))
            better = r > bv
            return jnp.where(better, r, bv), jnp.where(better, c, bi)

        def start_out(c):
            @pl.when(li == 1)
            def _():
                o_copy(c).start()

        oproj(0)

        def p4(c, best):
            best = post(c, best)
            oproj(c + 1)
            start_out(c)
            return best

        best = (jnp.full((TM, 1), -jnp.inf, F32), jnp.zeros((TM, 1), jnp.int32))
        best = lax.fori_loop(0, NC - 1, p4, best)
        bv, bi = post(NC - 1, best)
        start_out(NC - 1)
        rmax = jnp.max(bv, axis=0, keepdims=True)
        tok = bi * TM + lax.broadcasted_iota(jnp.int32, (TM, 1), 0)
        idx = jnp.min(jnp.where(bv == rmax, tok, S - 1))
        base = pl.multiple_of((idx // 16) * 16, 16)
        blk = pl.ds(base, 16)

        @pl.when(first)
        def _():
            for cp in f_copies[1:]:
                cp.wait()

        hs = h_s[blk, :]

        def ffn(j, y):
            cols = pl.ds(pl.multiple_of(j * FC, FC), FC)
            gt = _rb(_nn(hs, wg_s[:, cols]))
            up = _rb(_nn(hs, wu_s[:, cols]))
            a = (_rb(gt * jax.nn.sigmoid(gt)) * up).astype(BF)
            return y + _nn(a, wd_s[cols, :])

        y = lax.fori_loop(0, F // FC, ffn, jnp.zeros((16, D), F32))
        y = _rb(_rb(y) * _rb(jax.nn.sigmoid(rmax)))
        sel = lax.broadcasted_iota(jnp.int32, (16, D), 0) == idx - base
        upd = jnp.where(sel, y, 0.0)

        @pl.when(li == 1)
        def _():
            for c in range(NC):
                o_copy(c).wait()

        x_s[blk, :] = (x1_s[blk, :].astype(F32) + _rb(hs.astype(F32) + upd)).astype(BF)

        @pl.when(li == 1)
        def _():
            cp = pltpu.make_async_copy(x_s.at[blk], out_hbm.at[blk], o_sem.at[0])
            cp.start()
            cp.wait()

        return carry

    lax.fori_loop(0, 2, layer, None)


@jax.jit
def pallas_interleave_layers__sliding_block__moe_arch_mod__prompt_kernel(
    A_x: jax.Array,
    A_wqkv: jax.Array,
    A_wo: jax.Array,
    B_x: jax.Array,
    B_w_r: jax.Array,
    B_w_gate: jax.Array,
    B_w_up: jax.Array,
    B_w_down: jax.Array,
):
    del B_x
    hbm = pl.BlockSpec(memory_space=pl.ANY)
    out = pl.pallas_call(
        _kernel,
        out_shape=jax.ShapeDtypeStruct((S, D), BF),
        in_specs=[pl.BlockSpec(memory_space=pltpu.VMEM)] + [hbm] * 6,
        out_specs=hbm,
        scratch_shapes=[
            pltpu.VMEM((S, D), BF),
            pltpu.VMEM((S, D), BF),
            pltpu.VMEM((S, D), BF),
            pltpu.VMEM((NHG, S, 128), BF),
            pltpu.VMEM((3, NHG, D, 128), BF),
            pltpu.VMEM((D, D), BF),
            pltpu.VMEM((D, F), BF),
            pltpu.VMEM((D, F), BF),
            pltpu.VMEM((F, D), BF),
            pltpu.VMEM((256, D), BF),
            pltpu.VMEM((2, 128, S), BF),
            pltpu.VMEM((2, S, 128), BF),
            pltpu.VMEM((2, 128, S), BF),
            pltpu.SemaphoreType.DMA((NC,)),
            pltpu.SemaphoreType.DMA((3, NHG)),
            pltpu.SemaphoreType.DMA((4,)),
            pltpu.SemaphoreType.DMA((NC,)),
        ],
        compiler_params=pltpu.CompilerParams(vmem_limit_bytes=100 * 1024 * 1024),
    )(B_w_r.reshape(1, D), A_x.reshape(S, D), A_wqkv, A_wo, B_w_gate, B_w_up, B_w_down)
    return out.reshape(1, S, D)
```

```python
import functools

import jax
import jax.numpy as jnp
import numpy as np
from jax import lax
import jax.experimental.pallas as pl
import jax.experimental.pallas.tpu as pltpu

S, D, F = 2048, 1024, 3584
NHG = 8
NQB = S // 128
TM = 256
NC = S // TM
RB = TM // 8
FC = 512
BF, F32, I32 = jnp.bfloat16, jnp.float32, jnp.int32
NEG = -1e9

_bf = lambda v: float(np.asarray(v, dtype=jnp.bfloat16).astype(np.float32))
QSCALE = _bf(32 ** -0.5) * float(np.log2(np.e))
EPS = _bf(1e-5)


def _rb(x):
    return x.astype(BF).astype(F32)


def _ln(x):
    m = jnp.mean(x, axis=1, keepdims=True)
    xc = x - m
    v = jnp.mean(xc * xc, axis=1, keepdims=True)
    sd = _rb(jnp.sqrt(_rb(_rb(v) + EPS)))
    return xc * (1.0 / sd)


def _nt(a, b):
    return lax.dot_general(a, b, (((1,), (1,)), ((), ())), preferred_element_type=F32)


def _nn(a, b):
    return jnp.dot(a, b, preferred_element_type=F32)


def _pack(lo, hi):
    return pltpu.bitcast(pltpu.pack_elementwise([lo, hi], packed_dtype=BF), I32)


def _ds(start, size):
    return pl.ds(start if isinstance(start, int) else pl.multiple_of(start, size), size)


def _spread(slots, pieces, lo, hi):
    for i, f in enumerate(pieces):
        slots[lo + i * (hi - lo) // len(pieces)].append(f)


def _kernel(wr_ref, x_hbm, wqkv_hbm, wo_hbm, wg_hbm, wu_hbm, wd_hbm, out_hbm,
            x_s, x1_s, h_s, o_s, w_s, wo_s, wg_s, wu_s, wd_s, wt_s, qt_s, vt_s, kf_s, kp_s, kr_s,
            s_s, p_s,
            x_sem, w_sem, wo_sem, f_sem, o_sem):
    h_w, o_w, w_w, wo_w, wt_w, qt_w, vt_w = (
        r.bitcast(I32) for r in (h_s, o_s, w_s, wo_s, wt_s, qt_s, vt_s))

    def x_copy(c):
        rows = _ds(c * TM, TM)
        return pltpu.make_async_copy(x_hbm.at[rows], x_s.at[rows], x_sem.at[c])

    def w_copy(j, g):
        cols = pl.ds(j * D + g * 128, 128)
        return pltpu.make_async_copy(wqkv_hbm.at[:, cols], w_s.at[j, g], w_sem.at[j * NHG + g])

    def wo_copy(g):
        return pltpu.make_async_copy(wo_hbm.at[:, pl.ds(g * 128, 128)], wo_s.at[g], wo_sem.at[g])

    def o_copy(c):
        rows = _ds(c * TM, TM)
        return pltpu.make_async_copy(x_s.at[rows], out_hbm.at[rows], o_sem.at[c])

    f_copies = [pltpu.make_async_copy(a, b, f_sem.at[i]) for i, (a, b) in enumerate(
        ((wg_hbm, wg_s), (wu_hbm, wu_s), (wd_hbm, wd_s)))]

    def iota(shape, d):
        return lax.broadcasted_iota(I32, shape, d)

    r32, c32 = iota((32, 128), 0), iota((32, 128), 1)
    tri32 = jnp.where(r32 < 16, 2 * r32, 2 * r32 - 31) <= c32 % 32
    grp32 = c32 // 32
    grp = iota((16, 128), 1) // 32
    odd, high = grp % 2 == 1, grp >= 2
    r64, c64 = iota((64, 128), 0), iota((64, 128), 1)
    triw = jnp.where(2 * r64 <= c64, 0xFFFF, 0) | jnp.where(2 * r64 + 1 <= c64, -65536, 0)

    def wide(ref_w, b):
        rows = _ds(b * 64, 64)
        return jnp.concatenate([pltpu.bitcast(ref_w[i, rows, :], BF) for i in range(8)], 1)

    def ln_in(c, j):
        rows = _ds(c * TM + j * RB, RB)
        h = _ln(x_s[rows, :].astype(F32)).astype(BF)
        for i in range(8):
            h_s[i, rows, :] = h[:, i * 128:(i + 1) * 128]

    def prep_w(j, g):
        for i in range(8):
            wt_s[j, g, i] = w_s[2 * j, g, i * 128:(i + 1) * 128, :].T

    def proj_t(j, g, b):
        wt = jnp.concatenate([pltpu.bitcast(wt_w[j, g, i], BF) for i in range(8)], 1)
        y = _nt(wt, wide(h_w, b))
        if j == 0:
            qt_s[b, g] = (y * QSCALE).astype(BF)
        else:
            vt_s[b, g] = y.astype(BF)

    def proj_k(g, b, half):
        kf_s[g, half] = _nn(wide(h_w, b), pltpu.bitcast(w_w[1, g], BF))

    def k_rep(g, c):
        blocks = [kp_s[g, _ds((c * 8 + i) * 16, 16), :] for i in range(3)]
        for i in range(8):
            ld = lambda o: kf_s[g, i // 4, pl.ds((i % 4) * 32 + o, 8, stride=4), :]
            blocks.append(jnp.concatenate([_pack(ld(0), ld(2)), _pack(ld(1), ld(3))], 0))
        for i in range(8, 11):
            kp_s[g, _ds((c * 8 + i) * 16, 16), :] = blocks[i]
        for j in range(8):
            r = [blocks[j]] + [pltpu.roll(blocks[j + s], 32 * s, 1) for s in (1, 2, 3)]
            y = [jnp.where(odd, r[(m + 1) % 4], r[m]) for m in range(4)]
            for h in range(4):
                kr_s[g * 4 + h, _ds((c * 8 + j) * 16, 16), :] = jnp.where(
                    high, y[(2 - h) % 4], y[-h % 4])

    def qk(g, b, slot):
        lo = max(5 - 4 * b, 0) if isinstance(b, int) else 0
        order = ([8] if lo else [0, 8]) + list(range(max(lo, 1), 8))
        res = []
        for h in range(4):
            q = qt_w[b, g, h * 16:(h + 1) * 16, :]
            w = jnp.concatenate([jnp.where(grp == (p - h) % 4, q, 0) for p in range(4)], 0)
            k = jnp.concatenate(
                [kr_s[g * 4 + h, _ds((4 * b - 5 + i) * 16, 16), :] for i in order], 0)
            s = _nn(pltpu.bitcast(k, BF), pltpu.bitcast(w, BF))
            s = {i: s[n * 32:(n + 1) * 32] for n, i in enumerate(order)}
            s[0] = jnp.where(tri32, s.pop(8), NEG if lo else s[0])
            for i in range(lo, lo + 3 if lo else 0):
                s[i] = jnp.where(grp32 >= lo + 3 - i, s[i], NEG)
            m = functools.reduce(jnp.maximum, s.values())
            for i, v in s.items():
                s_s[slot, h, i] = v
            res.append((sorted(s), jnp.max(m, axis=0, keepdims=True)))
        return res

    def softmax(slot, h, live, m):
        p = {i: jnp.exp2(s_s[slot, h, i] - m) for i in live}
        l = jnp.sum(functools.reduce(jnp.add, p.values()), axis=0, keepdims=True)
        zero = jnp.zeros((16, 128), I32)
        u = [_pack(p[i][:16], p[i][16:]) if i in p else zero for i in range(8)]
        u = [jnp.where(odd, u[(i - 1) % 8], u[i]) for i in range(8)]
        u = [jnp.where(high, u[(i - 2) % 8], u[i]) for i in range(8)]
        edge = jnp.concatenate(u[:4], 0)
        p_s[h, 0:64] = edge & ~triw
        p_s[h, 64:128] = jnp.concatenate(u[4:], 0)
        p_s[h, 128:192] = edge & triw
        return 1.0 / l

    def pv(g, b, sm):
        n = min(b + 1, 3) if isinstance(b, int) else 3
        outs = []
        for h, linv in enumerate(sm):
            v = jnp.concatenate([pltpu.bitcast(vt_w[b - i, g, h * 16:(h + 1) * 16, :], BF)
                                 for i in range(n - 1, -1, -1)], 1)
            outs.append(_nn(v, pltpu.bitcast(p_s[h, 192 - 64 * n:], BF)) * linv)
        o_s[g, _ds(b * 128, 128), :] = jnp.concatenate(outs, 0).T.astype(BF)

    def oproj(b, j):
        rows, cols = _ds(b * 128, 128), slice(j * 128, (j + 1) * 128)
        y = _nn(wide(o_w, b), pltpu.bitcast(wo_w[j], BF))
        x1_s[rows, cols] = (x_s[rows, cols].astype(F32) + y).astype(BF)

    def post(c, j, best):
        rows = _ds(c * TM + j * RB, RB)
        x1 = x1_s[rows, :].astype(F32)
        h = _rb(_ln(x1))
        x_s[rows, :] = (x1 + h).astype(BF)
        r = _rb(jnp.sum(h * wr_ref[...].astype(F32), axis=1, keepdims=True))
        better = r > best[0]
        best[:] = jnp.where(better, r, best[0]), jnp.where(better, c * TM + j * RB, best[1])

    P = functools.partial

    def qkv_pieces(c, g):
        return ([P(proj_k, g, 2 * c + i, i) for i in range(2)]
                + [P(proj_t, j, g, 2 * c + i) for j in range(2) for i in range(2)])

    def stage(t, best, do_out, do_qkv):
        best = list(best)
        slots = [[] for _ in range(64)]
        nd = (16 if do_qkv else 32) if do_out else 8
        if do_qkv:
            _spread(slots, [P(ln_in, t + 1, j) for j in range(TM // RB)], 0, nd - 2)
            _spread(slots, [P(k_rep, g, t + 1) for g in range(NHG)], nd + 4, 68)
        if do_out:
            _spread(slots, [P(post, t - 1, j, best) for j in range(TM // RB)], nd, 64)
            _spread(slots, [P(oproj, 2 * t - 2 + i, j) for i in range(2) for j in range(8)], 0, nd)
        if do_qkv:
            _spread(slots, [f for g in range(NHG) for f in qkv_pieces(t + 1, g)], nd, 64)
        quads = [(g, 2 * t + i) for i in range(2) for g in range(NHG)]
        nxt = qk(*quads[0], 0)
        for n, quad in enumerate(quads):
            cur = nxt
            if n + 1 < len(quads):
                nxt = qk(*quads[n + 1], (n + 1) % 2)
            sm = []
            for h in range(4):
                sm.append(softmax(n % 2, h, *cur[h]))
                for f in slots[4 * n + h]:
                    f()
            pv(*quad, sm)
        return tuple(best)

    def first_chunk(load):
        for j in range(TM // RB):
            ln_in(0, j)
        for g in range(NHG):
            pieces = qkv_pieces(0, g)
            if load:
                for j in range(3):
                    w_copy(j, g).wait()
                    if g + 2 < NHG:
                        w_copy(j, g + 2).start()
                if g == NHG - 2:
                    x_copy(1).start()
                    for j in range(NHG):
                        wo_copy(j).start()
                pieces.insert(1, P(prep_w, 0, g))
                pieces.insert(3, P(prep_w, 1, g))
            pieces.insert(len(pieces) - 1, P(k_rep, g, 0))
            for f in pieces:
                f()

    x_copy(0).start()
    for g in range(2):
        for j in range(3):
            w_copy(j, g).start()
    kp_s[:, 0:48, :] = jnp.zeros((NHG, 48, 128), I32)
    x_copy(0).wait()
    first_chunk(True)
    for c in range(2, NC):
        x_copy(c).start()
    x_copy(1).wait()

    def layer(li, carry):
        first, last = li == 0, li == 1
        best = (jnp.full((RB, 1), -jnp.inf, F32), jnp.zeros((RB, 1), I32))
        best = stage(0, best, False, True)

        @pl.when(first)
        def _():
            for j in range(NHG):
                wo_copy(j).wait()
            for c in range(2, NC):
                x_copy(c).wait()
            for cp in f_copies:
                cp.start()

        def body(t, best):
            best = stage(t, best, True, True)

            @pl.when(last)
            def _():
                o_copy(t - 1).start()

            return best

        best = lax.fori_loop(1, NC - 1, body, best)
        best = list(stage(NC - 1, best, True, False))
        for j in range(8):
            oproj(2 * NC - 2, j)
        for j in range(8):
            oproj(2 * NC - 1, j)
            if j % 2 == 1:
                post(NC - 1, j // 2, best)
        for j in range(4, 8):
            post(NC - 1, j, best)

        @pl.when(last)
        def _():
            o_copy(NC - 2).start()
            o_copy(NC - 1).start()

        bv, bi = best
        rmax = jnp.max(bv, axis=0, keepdims=True)
        idx = jnp.min(jnp.where(bv == rmax, bi + iota((RB, 1), 0), S - 1))
        base = (idx // 16) * 16
        blk = _ds(base, 16)

        @pl.when(first)
        def _():
            for cp in f_copies:
                cp.wait()

        x1 = x1_s[blk, :].astype(F32)
        hs = _ln(x1).astype(BF)
        acts = []
        for j in range(F // FC):
            cols = slice(j * FC, (j + 1) * FC)
            gt = _rb(_nn(hs, wg_s[:, cols]))
            up = _rb(_nn(hs, wu_s[:, cols]))
            acts.append((_rb(gt * jax.nn.sigmoid(gt)) * up).astype(BF))
        y = _nn(jnp.concatenate(acts, 1), wd_s[...])
        y = _rb(_rb(y) * _rb(jax.nn.sigmoid(rmax)))
        upd = jnp.where(iota((16, D), 0) == idx - base, y, 0.0)

        @pl.when(last)
        def _():
            for c in range(NC):
                o_copy(c).wait()

        x_s[blk, :] = (x1 + _rb(hs.astype(F32) + upd)).astype(BF)

        @pl.when(last)
        def _():
            cp = pltpu.make_async_copy(x_s.at[blk], out_hbm.at[blk], o_sem.at[0])
            cp.start()
            cp.wait()

        @pl.when(first)
        def _():
            first_chunk(False)

        return carry

    lax.fori_loop(0, 2, layer, None)


@jax.jit
def pallas_interleave_layers__sliding_block__moe_arch_mod__prompt_kernel(
    A_x: jax.Array,
    A_wqkv: jax.Array,
    A_wo: jax.Array,
    B_x: jax.Array,
    B_w_r: jax.Array,
    B_w_gate: jax.Array,
    B_w_up: jax.Array,
    B_w_down: jax.Array,
):
    del B_x
    hbm = pl.BlockSpec(memory_space=pl.ANY)
    out = pl.pallas_call(
        _kernel,
        out_shape=jax.ShapeDtypeStruct((S, D), BF),
        in_specs=[pl.BlockSpec(memory_space=pltpu.VMEM)] + [hbm] * 6,
        out_specs=hbm,
        scratch_shapes=[
            pltpu.VMEM((S, D), BF),
            pltpu.VMEM((S, D), BF),
            pltpu.VMEM((8, S, 128), BF),
            pltpu.VMEM((NHG, S, 128), BF),
            pltpu.VMEM((3, NHG, D, 128), BF),
            pltpu.VMEM((8, D, 128), BF),
            pltpu.VMEM((D, F), BF),
            pltpu.VMEM((D, F), BF),
            pltpu.VMEM((F, D), BF),
            pltpu.VMEM((2, NHG, 8, 128, 128), BF),
            pltpu.VMEM((NQB, NHG, 128, 128), BF),
            pltpu.VMEM((NQB, NHG, 128, 128), BF),
            pltpu.VMEM((NHG, 2, 128, 128), F32),
            pltpu.VMEM((NHG, 67 * 16, 128), I32),
            pltpu.VMEM((32, 64 * 16, 128), I32),
            pltpu.VMEM((2, 4, 8, 32, 128), F32),
            pltpu.VMEM((4, 192, 128), I32),
            pltpu.SemaphoreType.DMA((NC,)),
            pltpu.SemaphoreType.DMA((3 * NHG,)),
            pltpu.SemaphoreType.DMA((NHG,)),
            pltpu.SemaphoreType.DMA((3,)),
            pltpu.SemaphoreType.DMA((NC,)),
        ],
        compiler_params=pltpu.CompilerParams(vmem_limit_bytes=110 * 1024 * 1024),
    )(B_w_r.reshape(1, D), A_x.reshape(S, D), A_wqkv, A_wo, B_w_gate, B_w_up, B_w_down)
    return out.reshape(1, S, D)
```

```python
import functools

import jax
import jax.numpy as jnp
import numpy as np
from jax import lax
import jax.experimental.pallas as pl
import jax.experimental.pallas.tpu as pltpu

S, D, F = 2048, 1024, 3584
NHG = 8
NQB = S // 128
TM = 256
NC = S // TM
RB = TM // 8
FC = 512
BF, F32, I32 = jnp.bfloat16, jnp.float32, jnp.int32
NEG = -1e9
LAG = 1

_bf = lambda v: float(np.asarray(v, dtype=jnp.bfloat16).astype(np.float32))
QSCALE = _bf(32 ** -0.5) * float(np.log2(np.e))
EPS = _bf(1e-5)


def _rb(x):
    return x.astype(BF).astype(F32)


def _ln(x):
    m = jnp.mean(x, axis=1, keepdims=True)
    xc = x - m
    v = jnp.mean(xc * xc, axis=1, keepdims=True)
    sd = _rb(jnp.sqrt(_rb(_rb(v) + EPS)))
    return xc * (1.0 / sd)


def _nt(a, b):
    return lax.dot_general(a, b, (((1,), (1,)), ((), ())), preferred_element_type=F32)


def _nn(a, b):
    return jnp.dot(a, b, preferred_element_type=F32)


def _pack(lo, hi):
    return pltpu.bitcast(pltpu.pack_elementwise([lo, hi], packed_dtype=BF), I32)


def _bf16(words, axis):
    return jnp.concatenate([pltpu.bitcast(w, BF) for w in words], axis)


def _lhs_terms(a11, a12, a21, a22):
    return [a11 + a22, a21 + a22, a11, a22, a11 + a12, a21 - a11, a12 - a22]


def _rhs_terms(b11, b12, b21, b22):
    return [b11 + b22, b11, b12 - b22, b21 - b11, b22, b11 + b12, b21 + b22]


def _on_words(fn, words):
    lo, hi = (fn(*[pltpu.unpack_elementwise(w, index=i, packed_dtype=BF, unpacked_dtype=F32)
                   for w in words]) for i in range(2))
    return [_pack(a, b) for a, b in zip(lo, hi)]


def _ds(start, size):
    return pl.ds(start if isinstance(start, int) else pl.multiple_of(start, size), size)


def _spread(slots, pieces, lo, hi):
    for i, f in enumerate(pieces):
        slots[lo + i * (hi - lo) // len(pieces)].append(f)


def _kernel(wr_ref, x_hbm, wqkv_hbm, wo_hbm, wg_hbm, wu_hbm, wd_hbm, out_hbm,
            x_s, x1_s, ha_s, oa_s, o_s, w_s, wo_s, wg_s, wu_s, wd_s, wt_s, ws_s, c_s, qt_s, vt_s, kf_s, kp_s, kr_s,
            s0_s, s1_s, p_s, z_s,
            x_sem, w_sem, wo_sem, f_sem, o_sem):
    ha_w, o_w, w_w, wo_w, wt_w, qt_w, vt_w = (
        r.bitcast(I32) for r in (ha_s, o_s, w_s, wo_s, wt_s, qt_s, vt_s))

    s_s = (s0_s, s1_s)

    def x_copy(c):
        rows = _ds(c * TM, TM)
        return pltpu.make_async_copy(x_hbm.at[rows], x_s.at[rows], x_sem.at[c])

    def w_copy(j, g):
        cols = pl.ds(j * D + g * 128, 128)
        return pltpu.make_async_copy(wqkv_hbm.at[:, cols], w_s.at[j, g], w_sem.at[j * NHG + g])

    def wo_copy(g):
        return pltpu.make_async_copy(wo_hbm.at[:, pl.ds(g * 128, 128)], wo_s.at[g], wo_sem.at[g])

    def o_copy(c):
        rows = _ds(c * TM, TM)
        return pltpu.make_async_copy(x_s.at[rows], out_hbm.at[rows], o_sem.at[c])

    f_copies = [pltpu.make_async_copy(a, b, f_sem.at[i]) for i, (a, b) in enumerate(
        ((wg_hbm, wg_s), (wu_hbm, wu_s), (wd_hbm, wd_s)))]

    def iota(shape, d):
        return lax.broadcasted_iota(I32, shape, d)

    r32, c32 = iota((32, 128), 0), iota((32, 128), 1)
    tri32 = jnp.where(r32 < 16, 2 * r32, 2 * r32 - 31) <= c32 % 32
    grp32 = c32 // 32
    grp = iota((16, 128), 1) // 32
    odd, high = grp % 2 == 1, grp >= 2
    r64, c64 = iota((64, 128), 0), iota((64, 128), 1)
    triw = jnp.where(2 * r64 <= c64, 0xFFFF, 0) | jnp.where(2 * r64 + 1 <= c64, -65536, 0)

    def ln_in(c, j):
        h = [_ln(x_s[_ds(z_s[0] + c * TM + i * 128 + j * 16, 16), :].astype(F32)) for i in range(2)]
        for i in range(4):
            lo, hi = slice(i * 128, (i + 1) * 128), slice((i + 4) * 128, (i + 5) * 128)
            for m, a in enumerate(_lhs_terms(h[0][:, lo], h[0][:, hi], h[1][:, lo], h[1][:, hi])):
                ha_s[m, i, j * 16:(j + 1) * 16, :] = a.astype(BF)
        return jnp.concatenate([h[0][:, D - 128:], h[1][:, D - 128:]], 0)

    def prep_o(c, i):
        words = [o_w[g, _ds((2 * c + b) * 64, 64), :] for b in range(2) for g in (i, i + 4)]
        for m, a in enumerate(_on_words(_lhs_terms, words)):
            oa_s[m, i] = a

    def prep_w(kind, u, i):
        if kind in (0, 2):
            for n in range(4):
                rows = pl.ds((i + 4 * (n // 2)) * 128, 128)
                wt_s[kind // 2, i, n] = w_s[kind, 2 * u + n % 2, rows, :].T
            words = [wt_w[kind // 2, i, n] for n in range(4)]
        else:
            src = w_w.at[1] if kind == 1 else wo_w
            words = [src[2 * u + n % 2, pl.ds((i + 4 * (n // 2)) * 64, 64), :] for n in range(4)]
        for m, a in enumerate(_on_words(_rhs_terms, words)):
            ws_s[kind * 4 + u, m, i] = a

    def emit(kind, c, b, g, y):
        if kind == 0:
            qt_s[2 * c + b, g] = (y * QSCALE).astype(BF)
        elif kind == 1:
            kf_s[g, b] = y
        elif kind == 2:
            vt_s[2 * c + b, g] = y.astype(BF)
        else:
            rows, cols = _ds((2 * c + b) * 128, 128), slice(g * 128, (g + 1) * 128)
            x1_s[rows, cols] = (x_s[rows, cols].astype(F32) + y).astype(BF)

    def proj(kind, c, u, m):
        a = _bf16([(oa_s if kind == 3 else ha_w)[m, i] for i in range(4)], 1)
        w = [ws_s[kind * 4 + u, m, i] for i in range(4)]
        y = _nt(_bf16(w, 1), a) if kind in (0, 2) else _nn(a, _bf16(w, 0))
        if m == 6:
            c_s[0] = y
        elif m == 4:
            c_s[0] -= y
            c_s[1] = y
        elif m == 2:
            emit(kind, c, 0, 2 * u + 1, c_s[1] + y)
            c_s[3] = y
        elif m == 0:
            c_s[0] += y
            c_s[3] += y
        elif m == 3:
            emit(kind, c, 0, 2 * u, c_s[0] + y)
            c_s[2] = y
        elif m == 1:
            emit(kind, c, 1, 2 * u, c_s[2] + y)
            c_s[3] -= y
        else:
            emit(kind, c, 1, 2 * u + 1, c_s[3] + y)
        return y

    def k_rep(g, c):
        blocks = [kp_s[g, _ds((c * 8 + i) * 16, 16), :] for i in range(3)]
        for i in range(8):
            ld = lambda o: kf_s[g, i // 4, pl.ds((i % 4) * 32 + o, 8, stride=4), :]
            blocks.append(jnp.concatenate([_pack(ld(0), ld(2)), _pack(ld(1), ld(3))], 0))
        for i in range(8, 11):
            kp_s[g, _ds((c * 8 + i) * 16, 16), :] = blocks[i]
        for j in range(8):
            r = [blocks[j]] + [pltpu.roll(blocks[j + s], 32 * s, 1) for s in (1, 2, 3)]
            y = [jnp.where(odd, r[(m + 1) % 4], r[m]) for m in range(4)]
            for h in range(4):
                kr_s[g * 4 + h, _ds((c * 8 + j) * 16, 16), :] = jnp.where(
                    high, y[(2 - h) % 4], y[-h % 4])

    def qk(g, b, slot):
        lo = max(5 - 4 * b, 0) if isinstance(b, int) else 0
        order = ([8] if lo else [0, 8]) + list(range(max(lo, 1), 8))
        res = []
        for h in range(4):
            q = qt_w[b, g, h * 16:(h + 1) * 16, :]
            w = jnp.concatenate([jnp.where(grp == (p - h) % 4, q, 0) for p in range(4)], 0)
            k = jnp.concatenate(
                [kr_s[g * 4 + h, _ds((4 * b - 5 + i) * 16, 16), :] for i in order], 0)
            s = _nn(pltpu.bitcast(k, BF), pltpu.bitcast(w, BF))
            s = {i: s[n * 32:(n + 1) * 32] for n, i in enumerate(order)}
            s[0] = jnp.where(tri32, s.pop(8), NEG if lo else s[0])
            for i in range(lo, lo + 3 if lo else 0):
                s[i] = jnp.where(grp32 >= lo + 3 - i, s[i], NEG)
            m = functools.reduce(jnp.maximum, s.values())
            for i, v in s.items():
                s_s[slot][h, i] = v
            res.append((sorted(s), jnp.max(m, axis=0, keepdims=True)))
        return res

    def softmax(slot, h, live, m):
        p = {i: jnp.exp2(s_s[slot][z_s[0] + h, i] - m) for i in live}
        l = jnp.sum(functools.reduce(jnp.add, p.values()), axis=0, keepdims=True)
        zero = jnp.zeros((16, 128), I32)
        u = [_pack(p[i][:16], p[i][16:]) if i in p else zero for i in range(8)]
        u = [jnp.where(odd, u[(i - 1) % 8], u[i]) for i in range(8)]
        u = [jnp.where(high, u[(i - 2) % 8], u[i]) for i in range(8)]
        edge = jnp.concatenate(u[:4], 0)
        z = (slot * 4 + h) * 3
        p_s[z] = edge & ~triw
        p_s[z + 1] = jnp.concatenate(u[4:], 0)
        p_s[z + 2] = edge & triw
        return 1.0 / l

    def pv(g, b, slot, sm):
        n = min(b + 1, 3) if isinstance(b, int) else 3
        outs = []
        for h, linv in enumerate(sm):
            v = jnp.concatenate([pltpu.bitcast(vt_w[b - i, g, h * 16:(h + 1) * 16, :], BF)
                                 for i in range(n - 1, -1, -1)], 1)
            outs.append(_nn(v, _bf16([p_s[(slot * 4 + h) * 3 + i] for i in range(3 - n, 3)], 0)) * linv)
        o_s[g, _ds(b * 128, 128), :] = jnp.concatenate(outs, 0).T.astype(BF)

    def post(c, j, best):
        rows = _ds(c * TM + j * RB, RB)
        x1 = x1_s[_ds(z_s[0] + c * TM + j * RB, RB), :].astype(F32)
        h = _rb(_ln(x1))
        x_s[rows, :] = (x1 + h).astype(BF)
        r = _rb(jnp.sum(h * wr_ref[...].astype(F32).reshape(1, D), axis=1, keepdims=True))
        better = jnp.where(c < NC, r, -jnp.inf) > best[0]
        best[:] = jnp.where(better, r, best[0]), jnp.where(better, c * TM + j * RB, best[1])
        return jnp.broadcast_to(r, (RB, 128))

    P = functools.partial

    def pieces(kind, c, u):
        return [P(proj, kind, c, u, m) for m in (6, 4, 2, 0, 3, 1, 5)]

    def stage(t, best, qkv=True, out=True, ln=True, fin=True):
        best = list(best)
        slots = [[] for _ in range(64)]
        nq = (48 if out else 56) if qkv else 8
        if ln:
            _spread(slots, [P(ln_in, t + 2, j) for j in range(8)], nq, 64)
        if fin:
            _spread(slots, [P(post, jnp.where(t >= 2, t - 2, NC), j, best) for j in range(8)], 8, nq if ln else 64)
        if out:
            _spread(slots, [P(prep_o, t - 1, i) for i in range(4)], 0, 8)
        if qkv:
            _spread(slots, [P(k_rep, g, t + 1) for g in range(NHG)], nq // 3, nq)
            _spread(slots, [f for kind in (1, 0, 2) for u in range(4)
                            for f in pieces(kind, t + 1, u)], 0, nq)
        if out:
            _spread(slots, [f for u in range(4) for f in pieces(3, t - 1, u)], nq, 64)
        quads = [(g, 2 * t + i) for i in range(2) for g in range(NHG)]
        due = {}
        nxt = qk(*quads[0], 0)
        for n, quad in enumerate(quads):
            cur = nxt
            if n + 1 < len(quads):
                nxt = qk(*quads[n + 1], (n + 1) % 2)
            sm, y = [], None
            for h in range(4):
                sm.append(softmax(n % 2, h, *cur[h]))
                i = 4 * n + h
                for f in slots[i]:
                    if f.func in (post, ln_in):
                        due[i + LAG] = f()
                    elif f.func is proj:
                        y = f()
                    else:
                        f()
                if i in due and i < 63:
                    s_s[(i + 1) // 4 % 2][4, 1] = due.pop(i)
                if y is not None and i < 63:
                    s_s[(i + 1) // 4 % 2][4, 0, 0:8] = y[:8]
                    follow = [f.func for f in slots[i + 1]]
                    pad = _ds(S + TM, 16)
                    if post in follow:
                        x1_s[pad, 0:128] = y[:16].astype(BF)
                    if ln_in in follow:
                        x_s[pad, 0:128] = y[:16].astype(BF)
            pv(*quad, n % 2, sm)
        return tuple(best)

    def first_chunk(load):
        todo = [(kind, u) for kind in (1, 0, 2) for u in range(4)]

        def fetch(n):
            return [w_copy(todo[n][0], 2 * todo[n][1] + e) for e in range(2)] if n < 12 else []

        def prep(n):
            for cp in fetch(n):
                cp.wait()
            for cp in fetch(n + 3) + ([x_copy(1)] if n == 6 else []):
                cp.start()
            return [P(prep_w, *todo[n], i) for i in range(4)]

        if load:
            for cp in [x_copy(0)] + fetch(0):
                cp.start()
            z_s[0] = 0
            x_s[S:S + TM, :] = jnp.zeros((TM, D), BF)
            x1_s[S:S + TM, :] = jnp.zeros((TM, D), BF)
            kp_s[:, 0:48, :] = jnp.zeros((NHG, 48, 128), I32)
            x_copy(0).wait()
            for cp in fetch(1) + fetch(2):
                cp.start()
        for j in range(8):
            ln_in(0, j)
        for f in prep(0) if load else []:
            f()
        for n, (kind, u) in enumerate(todo):
            side = prep(n + 1) if load and n < 11 else []
            if n >= 4:
                side.append(P(k_rep, n - 4, 0))
            for f in pieces(kind, 0, u):
                f()
                if side:
                    side.pop(0)()
        if load:
            for cp in [wo_copy(j) for j in range(NHG)] + [x_copy(c) for c in range(2, NC)]:
                cp.start()
            x_copy(1).wait()
        for j in range(8):
            ln_in(1, j)
        if load:
            x_copy(2).wait()

    def layer(li):
        first, last = li == 0, li == 1
        first_chunk(first)
        best = (jnp.full((RB, 1), -jnp.inf, F32), jnp.zeros((RB, 1), I32))
        best = stage(0, best, out=False, fin=False)
        if first:
            for cp in [wo_copy(j) for j in range(NHG)] + [x_copy(c) for c in range(3, NC)]:
                cp.wait()
            for cp in f_copies:
                cp.start()
            for u in range(4):
                for i in range(4):
                    prep_w(3, u, i)

        def body(t, best):
            best = stage(t, best)
            if last:
                pl.when(t >= 2)(lambda: o_copy(t - 2).start())
            return best

        best = lax.fori_loop(1, NC - 1, body, best)
        best = list(stage(NC - 1, best, qkv=False, ln=False))
        if last:
            o_copy(NC - 3).start()
        for i in range(4):
            prep_o(NC - 1, i)
        for u in range(4):
            for f in pieces(3, NC - 1, u):
                f()
            post(NC - 2, 2 * u, best)
            post(NC - 2, 2 * u + 1, best)
        for j in range(8):
            post(NC - 1, j, best)
        if last:
            o_copy(NC - 2).start()
            o_copy(NC - 1).start()

        bv, bi = best
        rmax = jnp.max(bv, axis=0, keepdims=True)
        idx = jnp.min(jnp.where(bv == rmax, bi + iota((RB, 1), 0), S - 1))
        base = (idx // 16) * 16
        blk = _ds(base, 16)

        @pl.when(first)
        def _():
            for cp in f_copies:
                cp.wait()

        x1 = x1_s[blk, :].astype(F32)
        hs = _ln(x1).astype(BF)
        acts = []
        for j in range(F // FC):
            cols = slice(j * FC, (j + 1) * FC)
            gt = _rb(_nn(hs, wg_s[:, cols]))
            up = _rb(_nn(hs, wu_s[:, cols]))
            acts.append((_rb(gt * jax.nn.sigmoid(gt)) * up).astype(BF))
        y = _nn(jnp.concatenate(acts, 1), wd_s[...])
        y = _rb(_rb(y) * _rb(jax.nn.sigmoid(rmax)))
        upd = jnp.where(iota((16, D), 0) == idx - base, y, 0.0)

        @pl.when(last)
        def _():
            for c in range(NC):
                o_copy(c).wait()

        x_s[blk, :] = (x1 + _rb(hs.astype(F32) + upd)).astype(BF)

        @pl.when(last)
        def _():
            cp = pltpu.make_async_copy(x_s.at[blk], out_hbm.at[blk], o_sem.at[0])
            cp.start()
            cp.wait()

    layer(0)
    layer(1)


@jax.jit
def pallas_interleave_layers__sliding_block__moe_arch_mod__prompt_kernel(
    A_x: jax.Array,
    A_wqkv: jax.Array,
    A_wo: jax.Array,
    B_x: jax.Array,
    B_w_r: jax.Array,
    B_w_gate: jax.Array,
    B_w_up: jax.Array,
    B_w_down: jax.Array,
):
    del B_x
    hbm = pl.BlockSpec(memory_space=pl.ANY)
    out = pl.pallas_call(
        _kernel,
        out_shape=jax.ShapeDtypeStruct((S, D), BF),
        in_specs=[pl.BlockSpec(memory_space=pltpu.VMEM)] + [hbm] * 6,
        out_specs=hbm,
        scratch_shapes=[
            pltpu.VMEM((S + TM + 16, D), BF),
            pltpu.VMEM((S + TM + 16, D), BF),
            pltpu.VMEM((7, 4, 128, 128), BF),
            pltpu.VMEM((7, 4, 64, 128), I32),
            pltpu.VMEM((NHG, S, 128), BF),
            pltpu.VMEM((3, NHG, D, 128), BF),
            pltpu.VMEM((8, D, 128), BF),
            pltpu.VMEM((D, F), BF),
            pltpu.VMEM((D, F), BF),
            pltpu.VMEM((F, D), BF),
            pltpu.VMEM((2, 4, 4, 128, 128), BF),
            pltpu.VMEM((16, 7, 4, 64, 128), I32),
            pltpu.VMEM((4, 128, 128), F32),
            pltpu.VMEM((NQB, NHG, 128, 128), BF),
            pltpu.VMEM((NQB, NHG, 128, 128), BF),
            pltpu.VMEM((NHG, 2, 128, 128), F32),
            pltpu.VMEM((NHG, 67 * 16, 128), I32),
            pltpu.VMEM((32, 64 * 16, 128), I32),
            pltpu.VMEM((5, 8, 32, 128), F32),
            pltpu.VMEM((5, 8, 32, 128), F32),
            pltpu.VMEM((24, 64, 128), I32),
            pltpu.SMEM((1,), I32),
            pltpu.SemaphoreType.DMA((NC,)),
            pltpu.SemaphoreType.DMA((3 * NHG,)),
            pltpu.SemaphoreType.DMA((NHG,)),
            pltpu.SemaphoreType.DMA((3,)),
            pltpu.SemaphoreType.DMA((NC,)),
        ],
        compiler_params=pltpu.CompilerParams(vmem_limit_bytes=110 * 1024 * 1024),
    )(B_w_r, A_x.reshape(S, D), A_wqkv, A_wo, B_w_gate, B_w_up, B_w_down)
    return out.reshape(1, S, D)
```

```python
import functools

import jax
import jax.numpy as jnp
import numpy as np
from jax import lax
import jax.experimental.pallas as pl
import jax.experimental.pallas.tpu as pltpu

S, D, F = 2048, 1024, 3584
NHG = 8
NQB = S // 128
TM = 256
NC = S // TM
RB = TM // 8
FC = 512
BF, F32, I32 = jnp.bfloat16, jnp.float32, jnp.int32
NEG = -1e9
LAG = 2
Q0 = 65
Q7 = 12
KP = 0
T1 = 17
E1 = 65
L0 = 1
L1 = 64
K0 = 0
K1 = 48

_bf = lambda v: float(np.asarray(v, dtype=jnp.bfloat16).astype(np.float32))
QSCALE = _bf(32 ** -0.5) * float(np.log2(np.e))
EPS = _bf(1e-5)


def _rb(x):
    return x.astype(BF).astype(F32)


def _stats(x):
    m = jnp.mean(x, axis=1, keepdims=True)
    xc = x - m
    v = jnp.mean(xc * xc, axis=1, keepdims=True)
    return m, xc, 1.0 / _rb(jnp.sqrt(_rb(_rb(v) + EPS)))


def _ln(x):
    _, xc, inv = _stats(x)
    return xc * inv


def _nt(a, b):
    return lax.dot_general(a, b, (((1,), (1,)), ((), ())), preferred_element_type=F32)


def _nn(a, b):
    return jnp.dot(a, b, preferred_element_type=F32)


def _pack(lo, hi):
    return pltpu.bitcast(pltpu.pack_elementwise([lo, hi], packed_dtype=BF), I32)


def _bf16(words, axis):
    return jnp.concatenate([pltpu.bitcast(w, BF) for w in words], axis)


def _lhs_terms(a11, a12, a21, a22):
    return [a11 + a22, a21 + a22, a11, a22, a11 + a12, a21 - a11, a12 - a22]


def _rhs_terms(b11, b12, b21, b22):
    return [b11 + b22, b11, b12 - b22, b21 - b11, b22, b11 + b12, b21 + b22]


def _on_words(fn, words):
    lo, hi = (fn(*[pltpu.unpack_elementwise(w, index=i, packed_dtype=BF, unpacked_dtype=F32)
                   for w in words]) for i in range(2))
    return [_pack(a, b) for a, b in zip(lo, hi)]


def _ds(start, size):
    return pl.ds(start if isinstance(start, int) else pl.multiple_of(start, size), size)


def _spread(slots, pieces, lo, hi):
    for i, f in enumerate(pieces):
        slots[lo + i * (hi - lo) // len(pieces)].append(f)


def _kernel(wr_ref, x_hbm, wqkv_hbm, wo_hbm, wg_hbm, wu_hbm, wd_hbm, out_hbm,
            x_s, x1_s, ha_s, hb_s, oa_s, o_s, w_s, wo_s, wg_s, wu_s, wd_s, wt_s, ws_s, c_s, qt_s, vt_s, kf_s, kp_s, kr_s,
            s0_s, s1_s, p_s, tri_s, wr_s, r_s, st_s, z_s,
            x_sem, w_sem, wo_sem, f_sem, o_sem):
    ha_w, hb_w, o_w, w_w, wo_w, wt_w, qt_w, vt_w, wd_w = (
        r.bitcast(I32) for r in (ha_s, hb_s, o_s, w_s, wo_s, wt_s, qt_s, vt_s, wd_s))

    s_s = (s0_s, s1_s)

    def x_copy(c):
        rows = _ds(c * TM, TM)
        return pltpu.make_async_copy(x_hbm.at[rows], x_s.at[rows], x_sem.at[c])

    def w_copy(j, g):
        cols = pl.ds(j * D + g * 128, 128)
        return pltpu.make_async_copy(wqkv_hbm.at[:, cols], w_s.at[j, g], w_sem.at[j * NHG + g])

    def wo_copy(g):
        return pltpu.make_async_copy(wo_hbm.at[:, pl.ds(g * 128, 128)], wo_s.at[g], wo_sem.at[g])

    def o_copy(c):
        rows = _ds(c * TM, TM)
        return pltpu.make_async_copy(x_s.at[rows], out_hbm.at[rows], o_sem.at[c])

    f_copies = [pltpu.make_async_copy(a, b, f_sem.at[i]) for i, (a, b) in enumerate(
        [(wg_hbm, wg_s), (wu_hbm, wu_s)]
        + [(wd_hbm.at[:, pl.ds(g * 128, 128)], wd_s.at[g]) for g in range(8)])]

    def iota(shape, d):
        return lax.broadcasted_iota(I32, shape, d)

    r32, c32 = iota((32, 128), 0), iota((32, 128), 1)
    tri32 = jnp.where(r32 < 16, 2 * r32, 2 * r32 - 31) <= c32 % 32
    grp32 = c32 // 32
    grp = iota((16, 128), 1) // 32
    odd, high = grp % 2 == 1, grp >= 2
    r64, c64 = iota((64, 128), 0), iota((64, 128), 1)
    triw = jnp.where(2 * r64 <= c64, 0xFFFF, 0) | jnp.where(2 * r64 + 1 <= c64, -65536, 0)
    tri_s[0], tri_s[1] = ~triw, triw
    wr_s[...] = jnp.broadcast_to(wr_ref[...].astype(F32).reshape(1, D), (RB, D))

    def static(c):
        return isinstance(c, int)

    def hide(c):
        return z_s[0] if static(c) else 0

    def ln_stats(c, j):
        m, _, inv = _stats(x_s[_ds(z_s[0] + c * TM + j * RB, RB), :].astype(F32))
        inv = jnp.broadcast_to(inv, (RB, 128))
        st_s[0, _ds(j * RB, RB)] = jnp.broadcast_to(m, (RB, 128))
        st_s[1, _ds(j * RB, RB)] = inv
        return inv

    def ln_in(c, j):
        def h(b, i):
            r = b * 128 + j * 16
            x = x_s[_ds(z_s[0] + c * TM + r, 16), i * 128:(i + 1) * 128].astype(F32)
            return (x - st_s[0, _ds(r, 16)]) * st_s[1, _ds(r, 16)]

        for i in range(4):
            terms = _lhs_terms(h(0, i), h(0, i + 4), h(1, i), h(1, i + 4))
            for m, a in enumerate(terms):
                (hb_s if static(c) and c == 1 else ha_s)[m, i, _ds(j * 16, 16), :] = a.astype(BF)
        return jnp.concatenate(terms[:2], 0)

    def prep_o(c, i):
        words = [o_w[g, _ds((2 * c + b) * 64, 64), :] for b in range(2) for g in (i, i + 4)]
        for m, a in enumerate(_on_words(_lhs_terms, words)):
            oa_s[m, i] = a

    def prep_w(kind, u, i):
        if kind in (0, 2):
            for n in range(4):
                rows = pl.ds((i + 4 * (n // 2)) * 128, 128)
                wt_s[kind // 2, i, n] = w_s[kind, 2 * u + n % 2, rows, :].T
            words = [wt_w[kind // 2, i, n] for n in range(4)]
        else:
            src = w_w.at[1] if kind == 1 else wo_w
            words = [src[2 * u + n % 2, pl.ds((i + 4 * (n // 2)) * 64, 64), :] for n in range(4)]
        for m, a in enumerate(_on_words(_rhs_terms, words)):
            ws_s[kind * 4 + u, m, i] = a

    def emit(kind, c, b, g, y):
        if kind == 0:
            qt_s[2 * c + b, g] = (y * QSCALE).astype(BF)
        elif kind == 1:
            kf_s[g, b] = y
        elif kind == 2:
            vt_s[2 * c + b, g] = y.astype(BF)
        else:
            rows, cols = _ds((2 * c + b) * 128, 128), slice(g * 128, (g + 1) * 128)
            x1_s[rows, cols] = (x_s[rows, cols].astype(F32) + y).astype(BF)

    def proj(kind, c, u, m):
        src = oa_s if kind == 3 else hb_w if static(c) and c == 1 else ha_w
        a = _bf16([src[hide(c) + m, i] for i in range(4)], 1)
        w = [ws_s[kind * 4 + u, m, i] for i in range(4)]
        y = _nt(_bf16(w, 1), a) if kind in (0, 2) else _nn(a, _bf16(w, 0))
        if m == 6:
            c_s[0] = y
        elif m == 4:
            c_s[0] -= y
            c_s[1] = y
        elif m == 2:
            emit(kind, c, 0, 2 * u + 1, c_s[1] + y)
            c_s[3] = y
        elif m == 0:
            c_s[0] += y
            c_s[3] += y
        elif m == 3:
            emit(kind, c, 0, 2 * u, c_s[0] + y)
            c_s[2] = y
        elif m == 1:
            emit(kind, c, 1, 2 * u, c_s[2] + y)
            c_s[3] -= y
        else:
            emit(kind, c, 1, 2 * u + 1, c_s[3] + y)
        return y

    def k_rep(g, c):
        blocks = [kp_s[g, _ds(hide(c) + (c * 8 + i) * 16, 16), :] for i in range(3)]
        for i in range(8):
            ld = lambda o: kf_s[(z_s[0] if KP else hide(c)) + g, i // 4, pl.ds((i % 4) * 32 + o, 8, stride=4), :]
            blocks.append(jnp.concatenate([_pack(ld(0), ld(2)), _pack(ld(1), ld(3))], 0))
        for i in range(8, 11):
            kp_s[g, _ds((c * 8 + i) * 16, 16), :] = blocks[i]
        for j in range(8):
            r = [blocks[j]] + [pltpu.roll(blocks[j + s], 32 * s, 1) for s in (1, 2, 3)]
            y = [jnp.where(odd, r[(m + 1) % 4], r[m]) for m in range(4)]
            for h in range(4):
                kr_s[g * 4 + h, _ds((c * 8 + j) * 16, 16), :] = jnp.where(
                    high, y[(2 - h) % 4], y[-h % 4])

    def qk(g, b, slot):
        lo = max(5 - 4 * b, 0) if isinstance(b, int) else 0
        order = ([8] if lo else [0, 8]) + list(range(max(lo, 1), 8))
        res = []
        for h in range(4):
            q = qt_w[b, g, h * 16:(h + 1) * 16, :]
            w = jnp.concatenate([jnp.where(grp == (p - h) % 4, q, 0) for p in range(4)], 0)
            k = jnp.concatenate(
                [kr_s[g * 4 + h, _ds(hide(b) + (4 * b - 5 + i) * 16, 16), :] for i in order], 0)
            s = _nn(pltpu.bitcast(k, BF), pltpu.bitcast(w, BF))
            s = {i: s[n * 32:(n + 1) * 32] for n, i in enumerate(order)}
            s[0] = jnp.where(tri32, s.pop(8), NEG if lo else s[0])
            for i in range(lo, lo + 3 if lo else 0):
                s[i] = jnp.where(grp32 >= lo + 3 - i, s[i], NEG)
            m = functools.reduce(jnp.maximum, s.values())
            for i, v in s.items():
                s_s[slot][h, i] = v
            s_s[slot][h, 8, 0:8] = jnp.broadcast_to(jnp.max(m, axis=0, keepdims=True), (8, 128))
            res.append(sorted(s))
        return res

    def softmax(slot, h, live):
        m = jnp.concatenate([s_s[slot][z_s[0] + h, 8, 0:8]] * 4, 0)
        p = {i: jnp.exp2(s_s[slot][z_s[0] + h, i] - m) for i in live}
        l = jnp.sum(functools.reduce(jnp.add, p.values()), axis=0, keepdims=True)
        zero = jnp.zeros((16, 128), I32)
        u = [_pack(p[i][:16], p[i][16:]) if i in p else zero for i in range(8)]
        u = [jnp.where(odd, u[(i - 1) % 8], u[i]) for i in range(8)]
        u = [jnp.where(high, u[(i - 2) % 8], u[i]) for i in range(8)]
        edge = jnp.concatenate(u[:4], 0)
        z = (slot * 4 + h) * 3
        p_s[z] = edge & tri_s[0]
        p_s[z + 1] = jnp.concatenate(u[4:], 0)
        p_s[z + 2] = edge & tri_s[1]
        return 1.0 / l

    def pv(g, b, slot, sm):
        n = min(b + 1, 3) if isinstance(b, int) else 3
        outs = []
        for h, linv in enumerate(sm):
            v = jnp.concatenate([pltpu.bitcast(vt_w[b - i, g, h * 16:(h + 1) * 16, :], BF)
                                 for i in range(n - 1, -1, -1)], 1)
            outs.append(_nn(v, _bf16([p_s[(slot * 4 + h) * 3 + i] for i in range(3 - n, 3)], 0)) * linv)
        o_s[g, _ds(b * 128, 128), :] = jnp.concatenate(outs, 0).T.astype(BF)

    def post(c, j):
        rows = _ds(c * TM + j * RB, RB)
        x1 = x1_s[_ds(z_s[0] + c * TM + j * RB, RB), :].astype(F32)
        h = _rb(_ln(x1))
        x_s[rows, :] = (x1 + h).astype(BF)
        r = _rb(jnp.sum(h * wr_s[...], axis=1, keepdims=True))
        r = jnp.broadcast_to(r, (RB, 128))
        r_s[rows, :] = r
        return r

    P = functools.partial

    def pieces(kind, c, u):
        return [P(proj, kind, c, u, m) for m in (6, 4, 2, 0, 3, 1, 5)]

    def release(y, follow):
        follow = [f.func for f in follow]
        pad = _ds(S + TM, 16)
        if post in follow:
            x1_s[pad, 0:128] = y[:16].astype(BF)
        if ln_in in follow or ln_stats in follow:
            x_s[pad, :] = jnp.concatenate([y[:16]] * 8, 1).astype(BF)
        if k_rep in follow:
            kf_s[NHG, 0, 0:8] = y[:8]

    def stage(t, qkv=True, out=True, ln=True, fin=True):
        slots = [[] for _ in range(65)]
        nq = (48 if out else Q0) if qkv else Q7
        if ln:
            _spread(slots, [P(ln_stats, t + 2, j) for j in range(8)], 1, T1)
            _spread(slots, [P(ln_in, t + 2, j) for j in range(8)], *((nq + 1, 64) if out else (T1, 40)))
        if fin:
            _spread(slots, [P(post, jnp.where(t >= 2, t - 2, NC), j) for j in range(8)], T1 if ln else 8, nq if ln else 64)
        if out:
            _spread(slots, [P(prep_o, t - 1, i) for i in range(4)], 0, min(nq, 8))
        if qkv:
            _spread(slots, [P(k_rep, g, t + 1) for g in range(NHG)], nq // 3 + K0, K1)
            _spread(slots, [f for kind in (1, 0, 2) for u in range(4)
                            for f in pieces(kind, t + 1, u)], 0, nq)
        if out:
            _spread(slots, [f for u in range(4) for f in pieces(3, t - 1, u)], nq, E1)
        quads = [(g, 2 * t + i) for i in range(2) for g in range(NHG)]
        due = {}
        nxt = qk(*quads[0], 0)
        for n, quad in enumerate(quads):
            cur = nxt
            if n + 1 < len(quads):
                nxt = qk(*quads[n + 1], (n + 1) % 2)
            sm, y = [], None
            for h in range(4):
                sm.append(softmax(n % 2, h, cur[h]))
                i = 4 * n + h
                for f in slots[i]:
                    if f.func in (post, ln_in, ln_stats):
                        due[i + LAG] = f()
                    elif f.func is proj:
                        y = f()
                    else:
                        f()
                if i in due and i < 63:
                    s_s[(i + 1) // 4 % 2][4, 1] = due.pop(i)
                if y is not None and i < 63:
                    s_s[(i + 1) // 4 % 2][4, 0, 0:8] = y[:8]
                    release(y, slots[i + 1])
            pv(*quad, n % 2, sm)
        for f in slots[64]:
            f()

    def norm_first():
        for j in range(8):
            ln_stats(0, j)
        for j in range(8):
            ln_in(0, j)

    def first_chunk(load):
        todo = [(kind, u) for kind in (1, 0, 2) for u in range(4)]

        def fetch(n):
            return [w_copy(todo[n][0], 2 * todo[n][1] + e) for e in range(2)] if n < 12 else []

        def prep(n):
            for cp in fetch(n) + ([x_copy(1)] if n == 5 else []):
                cp.wait()
            for cp in fetch(n + 3) + ([x_copy(n)] if n in (1, 2) else []):
                cp.start()
            return [P(prep_w, *todo[n], i) for i in range(4)]

        if load:
            for cp in [x_copy(0)] + fetch(0):
                cp.start()
            z_s[0] = 0
            x_s[S:S + TM, :] = jnp.zeros((TM, D), BF)
            x1_s[S:S + TM, :] = jnp.zeros((TM, D), BF)
            kp_s[:, 0:48, :] = jnp.zeros((NHG, 48, 128), I32)
            x_copy(0).wait()
            for cp in fetch(1) + fetch(2):
                cp.start()
            norm_first()
        for f in prep(0) if load else []:
            f()
        for n, (kind, u) in enumerate(todo):
            side = prep(n + 1) if load and n < 11 else []
            if n >= 4:
                side += [P(k_rep, n - 4, 0), ]
                side += [P(ln_in if n >= 8 else ln_stats, 1, 2 * (n % 4) + j) for j in range(2)]
            for f in pieces(kind, 0, u):
                y = f()
                if side:
                    release(y, side[:1])
                    side.pop(0)()
        if load:
            for cp in [wo_copy(j) for j in range(NHG)] + [x_copy(c) for c in range(3, NC)]:
                cp.start()
        if load:
            x_copy(2).wait()

    def layer(li):
        first, last = li == 0, li == 1
        first_chunk(first)
        stage(0, out=False, fin=False)
        if first:
            for cp in [wo_copy(j) for j in range(NHG)] + [x_copy(c) for c in range(3, NC)]:
                cp.wait()
            for cp in f_copies:
                cp.start()
            for u in range(4):
                for i in range(4):
                    prep_w(3, u, i)

        def body(t, _):
            stage(t)
            if last:
                pl.when(t >= 2)(lambda: o_copy(t - 2).start())

        lax.fori_loop(1, NC - 1, body, None)
        if first:
            for cp in f_copies:
                cp.wait()
        stage(NC - 1, qkv=False, ln=False)
        for i in range(4):
            prep_o(NC - 1, i)
        for u in range(4):
            for n, f in enumerate(pieces(3, NC - 1, u)):
                y = f()
                if n in (0, 3):
                    release(y, [P(post)])
                    post(NC - 2, 2 * u + n // 3)

        def argmax(lo, hi):
            r = r_s[lo:hi, :]
            top = jnp.max(r, axis=0, keepdims=True)
            at = jnp.min(jnp.where(r == top, iota(r.shape, 0) + lo, S - 1), axis=0, keepdims=True)
            return top[:, 0:1], at[:, 0:1]

        top0, at0 = argmax(0, S - 2 * TM)
        for j in range(8):
            post(NC - 1, j)
        top1, at1 = argmax(S - 2 * TM, S)
        rmax = jnp.maximum(top0, top1)
        idx = jnp.min(jnp.where(top1 > top0, at1, at0))
        base = (idx // 16) * 16
        blk = _ds(base, 16)

        x1 = x1_s[blk, :].astype(F32)
        hs = _ln(x1).astype(BF)
        acts = []
        for j in range(F // FC):
            cols = slice(j * FC, (j + 1) * FC)
            gt = _rb(_nn(hs, wg_s[:, cols]))
            up = _rb(_nn(hs, wu_s[:, cols]))
            acts.append((_rb(gt * jax.nn.sigmoid(gt)) * up).astype(BF))
            if last and j == 2:
                for c in range(NC - 3, NC):
                    o_copy(c).start()
        if first:
            norm_first()
        a = jnp.concatenate(acts, 1)
        y = _nn(a, _bf16([wd_w[g] for g in range(8)], 1))
        y = _rb(_rb(y) * _rb(jax.nn.sigmoid(rmax)))
        upd = jnp.where(iota((16, D), 0) == idx - base, y, 0.0)
        new = (x1 + _rb(hs.astype(F32) + upd)).astype(BF)
        if first:
            x_s[blk, :] = new
            ln_stats(0, base % TM // RB)
            ln_in(0, base % 128 // 16)
        else:
            for c in range(NC):
                o_copy(c).wait()
            x_s[blk, :] = new
            cp = pltpu.make_async_copy(x_s.at[blk], out_hbm.at[blk], o_sem.at[0])
            cp.start()
            cp.wait()

    layer(0)
    layer(1)


@jax.jit
def pallas_interleave_layers__sliding_block__moe_arch_mod__prompt_kernel(
    A_x: jax.Array,
    A_wqkv: jax.Array,
    A_wo: jax.Array,
    B_x: jax.Array,
    B_w_r: jax.Array,
    B_w_gate: jax.Array,
    B_w_up: jax.Array,
    B_w_down: jax.Array,
):
    del B_x
    hbm = pl.BlockSpec(memory_space=pl.ANY)
    out = pl.pallas_call(
        _kernel,
        out_shape=jax.ShapeDtypeStruct((S, D), BF),
        in_specs=[pl.BlockSpec(memory_space=pltpu.VMEM)] + [hbm] * 6,
        out_specs=hbm,
        scratch_shapes=[
            pltpu.VMEM((S + TM + 16, D), BF),
            pltpu.VMEM((S + TM + 16, D), BF),
            pltpu.VMEM((7, 4, 128, 128), BF),
            pltpu.VMEM((7, 4, 128, 128), BF),
            pltpu.VMEM((7, 4, 64, 128), I32),
            pltpu.VMEM((NHG, S, 128), BF),
            pltpu.VMEM((3, NHG, D, 128), BF),
            pltpu.VMEM((8, D, 128), BF),
            pltpu.VMEM((D, F), BF),
            pltpu.VMEM((D, F), BF),
            pltpu.VMEM((8, F, 128), BF),
            pltpu.VMEM((2, 4, 4, 128, 128), BF),
            pltpu.VMEM((16, 7, 4, 64, 128), I32),
            pltpu.VMEM((4, 128, 128), F32),
            pltpu.VMEM((NQB, NHG, 128, 128), BF),
            pltpu.VMEM((NQB, NHG, 128, 128), BF),
            pltpu.VMEM((NHG + 1, 2, 128, 128), F32),
            pltpu.VMEM((NHG, 67 * 16, 128), I32),
            pltpu.VMEM((32, 64 * 16, 128), I32),
            pltpu.VMEM((5, 9, 32, 128), F32),
            pltpu.VMEM((5, 9, 32, 128), F32),
            pltpu.VMEM((24, 64, 128), I32),
            pltpu.VMEM((2, 64, 128), I32),
            pltpu.VMEM((RB, D), F32),
            pltpu.VMEM((S + TM, 128), F32),
            pltpu.VMEM((2, TM, 128), F32),
            pltpu.SMEM((1,), I32),
            pltpu.SemaphoreType.DMA((NC,)),
            pltpu.SemaphoreType.DMA((3 * NHG,)),
            pltpu.SemaphoreType.DMA((NHG,)),
            pltpu.SemaphoreType.DMA((10,)),
            pltpu.SemaphoreType.DMA((NC,)),
        ],
        compiler_params=pltpu.CompilerParams(vmem_limit_bytes=110 * 1024 * 1024),
    )(B_w_r, A_x.reshape(S, D), A_wqkv, A_wo, B_w_gate, B_w_up, B_w_down)
    return out.reshape(1, S, D)
```

```python
import functools

import jax
import jax.numpy as jnp
import numpy as np
from jax import lax
import jax.experimental.pallas as pl
import jax.experimental.pallas.tpu as pltpu

S, D, F = 2048, 1024, 3584
NHG = 8
NQB = S // 128
TM = 256
NC = S // TM
RB = TM // 8
FC = 512
BF, F32, I32 = jnp.bfloat16, jnp.float32, jnp.int32
NEG = -1e9
LAG = 2
Q0 = 65
Q7 = 12
KP = 0
T1 = 17
E1 = 65
L0 = 1
L1 = 64
K0 = 0
K1 = 48

_bf = lambda v: float(np.asarray(v, dtype=jnp.bfloat16).astype(np.float32))
QSCALE = _bf(32 ** -0.5) * float(np.log2(np.e))
EPS = _bf(1e-5)


def _rb(x):
    return x.astype(BF).astype(F32)


def _stats(x):
    m = jnp.mean(x, axis=1, keepdims=True)
    xc = x - m
    v = jnp.mean(xc * xc, axis=1, keepdims=True)
    return m, xc, 1.0 / _rb(jnp.sqrt(_rb(_rb(v) + EPS)))


def _ln(x):
    _, xc, inv = _stats(x)
    return xc * inv


def _nt(a, b):
    return lax.dot_general(a, b, (((1,), (1,)), ((), ())), preferred_element_type=F32)


def _nn(a, b):
    return jnp.dot(a, b, preferred_element_type=F32)


def _pack(lo, hi):
    return pltpu.bitcast(pltpu.pack_elementwise([lo, hi], packed_dtype=BF), I32)


def _bf16(words, axis):
    return jnp.concatenate([pltpu.bitcast(w, BF) for w in words], axis)


def _lhs_terms(a11, a12, a21, a22):
    return [a11 + a22, a21 + a22, a11, a22, a11 + a12, a21 - a11, a12 - a22]


def _rhs_terms(b11, b12, b21, b22):
    return [b11 + b22, b11, b12 - b22, b21 - b11, b22, b11 + b12, b21 + b22]


def _on_words(fn, words):
    lo, hi = (fn(*[pltpu.unpack_elementwise(w, index=i, packed_dtype=BF, unpacked_dtype=F32)
                   for w in words]) for i in range(2))
    return [_pack(a, b) for a, b in zip(lo, hi)]


def _ds(start, size):
    return pl.ds(start if isinstance(start, int) else pl.multiple_of(start, size), size)


def _spread(slots, pieces, lo, hi):
    for i, f in enumerate(pieces):
        slots[lo + i * (hi - lo) // len(pieces)].append(f)


def _kernel(wr_ref, x_hbm, wqkv_hbm, wo_hbm, wg_hbm, wu_hbm, wd_hbm, out_hbm,
            x_s, x1_s, ha_s, hb_s, oa_s, o_s, w_s, wo_s, wg_s, wu_s, wd_s, ws_s, c_s, qt_s, vt_s, kf_s, kp_s, kr_s,
            s0_s, s1_s, p_s, tri_s, wr_s, r_s, st_s, z_s,
            x_sem, w_sem, wo_sem, f_sem, o_sem):
    ha_w, hb_w, o_w, w_w, wo_w, qt_w, vt_w, wd_w = (
        r.bitcast(I32) for r in (ha_s, hb_s, o_s, w_s, wo_s, qt_s, vt_s, wd_s))

    s_s = (s0_s, s1_s)

    def x_copy(c):
        rows = _ds(c * TM, TM)
        return pltpu.make_async_copy(x_hbm.at[rows], x_s.at[rows], x_sem.at[c])

    def w_copy(j, g):
        cols = pl.ds(j * D + g * 128, 128)
        return pltpu.make_async_copy(wqkv_hbm.at[:, cols], w_s.at[j, g], w_sem.at[j * NHG + g])

    def wo_copy(g):
        return pltpu.make_async_copy(wo_hbm.at[:, pl.ds(g * 128, 128)], wo_s.at[g], wo_sem.at[g])

    def o_copy(c):
        rows = _ds(c * TM, TM)
        return pltpu.make_async_copy(x_s.at[rows], out_hbm.at[rows], o_sem.at[c])

    f_copies = [pltpu.make_async_copy(a, b, f_sem.at[i]) for i, (a, b) in enumerate(
        [(wg_hbm, wg_s), (wu_hbm, wu_s)]
        + [(wd_hbm.at[:, pl.ds(g * 128, 128)], wd_s.at[g]) for g in range(8)])]

    late_copies = [x_copy(2)] + [wo_copy(j) for j in range(NHG)]

    def iota(shape, d):
        return lax.broadcasted_iota(I32, shape, d)

    r32, c32 = iota((32, 128), 0), iota((32, 128), 1)
    tri32 = jnp.where(r32 < 16, 2 * r32, 2 * r32 - 31) <= c32 % 32
    grp32 = c32 // 32
    grp = iota((16, 128), 1) // 32
    odd, high = grp % 2 == 1, grp >= 2
    r64, c64 = iota((64, 128), 0), iota((64, 128), 1)
    triw = jnp.where(2 * r64 <= c64, 0xFFFF, 0) | jnp.where(2 * r64 + 1 <= c64, -65536, 0)

    def setup():
        tri_s[0], tri_s[1] = ~triw, triw
        wr_s[...] = jnp.broadcast_to(wr_ref[...].astype(F32).reshape(1, D), (RB, D))
        z_s[0] = 0
        x_s[S:S + TM, :] = jnp.zeros((TM, D), BF)
        x1_s[S:S + TM, :] = jnp.zeros((TM, D), BF)
        kp_s[:, 0:48, :] = jnp.zeros((NHG, 48, 128), I32)

    def static(c):
        return isinstance(c, int)

    def hide(c):
        return z_s[0] if static(c) else 0

    def ln_stats(c, j):
        m, _, inv = _stats(x_s[_ds(z_s[0] + c * TM + j * RB, RB), :].astype(F32))
        inv = jnp.broadcast_to(inv, (RB, 128))
        st_s[0, _ds(j * RB, RB)] = jnp.broadcast_to(m, (RB, 128))
        st_s[1, _ds(j * RB, RB)] = inv
        return inv

    def ln_in(c, j):
        def h(b, i):
            r = b * 128 + j * 16
            x = x_s[_ds(z_s[0] + c * TM + r, 16), i * 128:(i + 1) * 128].astype(F32)
            return (x - st_s[0, _ds(r, 16)]) * st_s[1, _ds(r, 16)]

        for i in range(4):
            terms = _lhs_terms(h(0, i), h(0, i + 4), h(1, i), h(1, i + 4))
            for m, a in enumerate(terms):
                (hb_s if static(c) and c == 1 else ha_s)[m, i, _ds(j * 16, 16), :] = a.astype(BF)
        return jnp.concatenate(terms[:2], 0)

    def prep_o(c, i):
        words = [o_w[g, _ds((2 * c + b) * 64, 64), :] for b in range(2) for g in (i, i + 4)]
        for m, a in enumerate(_on_words(_lhs_terms, words)):
            oa_s[m, i] = a

    def prep_w(kind, u, i):
        src = wo_w if kind == 3 else w_w.at[kind]
        z = z_s[0] if kind == 3 else 0
        words = [src[z + 2 * u + n % 2, pl.ds((i + 4 * (n // 2)) * 64, 64), :] for n in range(4)]
        if kind in (0, 2):
            words = [pltpu.bitcast(pltpu.bitcast(w, BF).T, I32) for w in words]
        for m, a in enumerate(_on_words(_rhs_terms, words)):
            ws_s[kind * 4 + u, m, i] = a
        return pltpu.bitcast(a[32:], F32)

    def emit(kind, c, b, g, y):
        if kind == 0:
            qt_s[2 * c + b, g] = (y * QSCALE).astype(BF)
        elif kind == 1:
            kf_s[g, b] = y
        elif kind == 2:
            vt_s[2 * c + b, g] = y.astype(BF)
        else:
            rows, cols = _ds((2 * c + b) * 128, 128), slice(g * 128, (g + 1) * 128)
            x1_s[rows, cols] = (x_s[rows, cols].astype(F32) + y).astype(BF)

    def proj(kind, c, u, m):
        src = oa_s if kind == 3 else hb_w if static(c) and c == 1 else ha_w
        a = _bf16([src[hide(c) + m, i] for i in range(4)], 1)
        w = [ws_s[kind * 4 + u, m, i] for i in range(4)]
        y = _nt(_bf16(w, 1), a) if kind in (0, 2) else _nn(a, _bf16(w, 0))
        if m == 6:
            c_s[0] = y
        elif m == 4:
            c_s[0] -= y
            c_s[1] = y
        elif m == 2:
            emit(kind, c, 0, 2 * u + 1, c_s[1] + y)
            c_s[3] = y
        elif m == 0:
            c_s[0] += y
            c_s[3] += y
        elif m == 3:
            emit(kind, c, 0, 2 * u, c_s[0] + y)
            c_s[2] = y
        elif m == 1:
            emit(kind, c, 1, 2 * u, c_s[2] + y)
            c_s[3] -= y
        else:
            emit(kind, c, 1, 2 * u + 1, c_s[3] + y)
        return y

    def k_rep(g, c):
        blocks = [kp_s[g, _ds(hide(c) + (c * 8 + i) * 16, 16), :] for i in range(3)]
        for i in range(8):
            ld = lambda o: kf_s[(z_s[0] if KP else hide(c)) + g, i // 4, pl.ds((i % 4) * 32 + o, 8, stride=4), :]
            blocks.append(jnp.concatenate([_pack(ld(0), ld(2)), _pack(ld(1), ld(3))], 0))
        for i in range(8, 11):
            kp_s[g, _ds((c * 8 + i) * 16, 16), :] = blocks[i]
        for j in range(8):
            r = [blocks[j]] + [pltpu.roll(blocks[j + s], 32 * s, 1) for s in (1, 2, 3)]
            y = [jnp.where(odd, r[(m + 1) % 4], r[m]) for m in range(4)]
            for h in range(4):
                kr_s[g * 4 + h, _ds((c * 8 + j) * 16, 16), :] = jnp.where(
                    high, y[(2 - h) % 4], y[-h % 4])

    def qk(g, b, slot):
        lo = max(5 - 4 * b, 0) if isinstance(b, int) else 0
        order = ([8] if lo else [0, 8]) + list(range(max(lo, 1), 8))
        res = []
        for h in range(4):
            q = qt_w[b, g, h * 16:(h + 1) * 16, :]
            w = jnp.concatenate([jnp.where(grp == (p - h) % 4, q, 0) for p in range(4)], 0)
            k = jnp.concatenate(
                [kr_s[g * 4 + h, _ds(hide(b) + (4 * b - 5 + i) * 16, 16), :] for i in order], 0)
            s = _nn(pltpu.bitcast(k, BF), pltpu.bitcast(w, BF))
            s = {i: s[n * 32:(n + 1) * 32] for n, i in enumerate(order)}
            s[0] = jnp.where(tri32, s.pop(8), NEG if lo else s[0])
            for i in range(lo, lo + 3 if lo else 0):
                s[i] = jnp.where(grp32 >= lo + 3 - i, s[i], NEG)
            m = functools.reduce(jnp.maximum, s.values())
            for i, v in s.items():
                s_s[slot][h, i] = v
            s_s[slot][h, 8, 0:8] = jnp.broadcast_to(jnp.max(m, axis=0, keepdims=True), (8, 128))
            res.append(sorted(s))
        return res

    def softmax(slot, h, live):
        m = jnp.concatenate([s_s[slot][z_s[0] + h, 8, 0:8]] * 4, 0)
        p = {i: jnp.exp2(s_s[slot][z_s[0] + h, i] - m) for i in live}
        l = jnp.sum(functools.reduce(jnp.add, p.values()), axis=0, keepdims=True)
        zero = jnp.zeros((16, 128), I32)
        u = [_pack(p[i][:16], p[i][16:]) if i in p else zero for i in range(8)]
        u = [jnp.where(odd, u[(i - 1) % 8], u[i]) for i in range(8)]
        u = [jnp.where(high, u[(i - 2) % 8], u[i]) for i in range(8)]
        edge = jnp.concatenate(u[:4], 0)
        z = (slot * 4 + h) * 3
        p_s[z] = edge & tri_s[0]
        p_s[z + 1] = jnp.concatenate(u[4:], 0)
        p_s[z + 2] = edge & tri_s[1]
        return 1.0 / l

    def pv(g, b, slot, sm):
        n = min(b + 1, 3) if isinstance(b, int) else 3
        outs = []
        for h, linv in enumerate(sm):
            v = jnp.concatenate([pltpu.bitcast(vt_w[b - i, g, h * 16:(h + 1) * 16, :], BF)
                                 for i in range(n - 1, -1, -1)], 1)
            outs.append(_nn(v, _bf16([p_s[(slot * 4 + h) * 3 + i] for i in range(3 - n, 3)], 0)) * linv)
        o_s[g, _ds(b * 128, 128), :] = jnp.concatenate(outs, 0).T.astype(BF)

    def post(c, j):
        rows = _ds(c * TM + j * RB, RB)
        x1 = x1_s[_ds(z_s[0] + c * TM + j * RB, RB), :].astype(F32)
        h = _rb(_ln(x1))
        x_s[rows, :] = (x1 + h).astype(BF)
        r = _rb(jnp.sum(h * wr_s[...], axis=1, keepdims=True))
        r = jnp.broadcast_to(r, (RB, 128))
        r_s[rows, :] = r
        return r

    P = functools.partial

    def pieces(kind, c, u):
        return [P(proj, kind, c, u, m) for m in (6, 4, 2, 0, 3, 1, 5)]

    def release(y, follow):
        follow = [f.func for f in follow]
        pad = _ds(S + TM, 16)
        if post in follow:
            x1_s[pad, 0:128] = y[:16].astype(BF)
        if ln_in in follow or ln_stats in follow:
            x_s[pad, :] = jnp.concatenate([y[:16]] * 8, 1).astype(BF)
        if k_rep in follow:
            kf_s[NHG, 0, 0:8] = y[:8]
        if prep_w in follow:
            wo_s[8, 0:16] = y[:16].astype(BF)

    def stage(t, qkv=True, out=True, ln=True, fin=True, load=False):
        slots = [[] for _ in range(65)]
        nq = (48 if out else Q0) if qkv else Q7
        if load:
            slots[11] += [P(cp.wait) for cp in late_copies]
            _spread(slots, [P(prep_w, 3, u, i) for u in range(4) for i in range(4)], 12, 44)
        if ln:
            _spread(slots, [P(ln_stats, t + 2, j) for j in range(8)], *((1, T1) if out else (13, 45)))
            _spread(slots, [P(ln_in, t + 2, j) for j in range(8)], *((nq + 1, 64) if out else (45, 61)))
        if fin:
            _spread(slots, [P(post, jnp.where(t >= 2, t - 2, NC), j) for j in range(8)], T1 if ln else 8, nq if ln else 64)
        if out:
            _spread(slots, [P(prep_o, t - 1, i) for i in range(4)], 0, min(nq, 8))
        if qkv:
            _spread(slots, [P(k_rep, g, t + 1) for g in range(NHG)], nq // 3 + K0, K1)
            _spread(slots, [f for kind in (1, 0, 2) for u in range(4)
                            for f in pieces(kind, t + 1, u)], 0, nq)
        if out:
            _spread(slots, [f for u in range(4) for f in pieces(3, t - 1, u)], nq, E1)
        quads = [(g, 2 * t + i) for i in range(2) for g in range(NHG)]
        due = {}
        nxt = qk(*quads[0], 0)
        for n, quad in enumerate(quads):
            cur = nxt
            if n + 1 < len(quads):
                nxt = qk(*quads[n + 1], (n + 1) % 2)
            sm, y = [], None
            for h in range(4):
                sm.append(softmax(n % 2, h, cur[h]))
                i = 4 * n + h
                for f in slots[i]:
                    if f.func in (post, ln_in, ln_stats, prep_w):
                        due[i + LAG] = f()
                    elif f.func is proj:
                        y = f()
                    else:
                        f()
                if i in due and i < 63:
                    s_s[(i + 1) // 4 % 2][4, 1] = due.pop(i)
                if y is not None and i < 63:
                    s_s[(i + 1) // 4 % 2][4, 0, 0:8] = y[:8]
                    release(y, slots[i + 1])
            pv(*quad, n % 2, sm)
        for f in slots[64]:
            f()

    def norm_first():
        for j in range(8):
            ln_stats(0, j)
        for j in range(8):
            ln_in(0, j)

    def first_chunk(load):
        todo = [(kind, u) for kind in (1, 0, 2) for u in range(4)]

        def fetch(*ns):
            return [w_copy(todo[n][0], 2 * todo[n][1] + e) for n in ns for e in range(2)]

        groups = [fetch(0), fetch(1, 2), fetch(3, 4) + [x_copy(1)], fetch(5, 6), fetch(7, 8),
                  fetch(9, 10, 11), late_copies, [x_copy(c) for c in range(3, NC)]]

        def prep(n):
            if n in (0, 1, 3, 5, 7, 9):
                for cp in groups[(n + 1) // 2]:
                    cp.wait()
                for cp in groups[(n + 1) // 2 + 2]:
                    cp.start()
            return [P(prep_w, *todo[n], i) for i in range(4)]

        if load:
            for cp in [x_copy(0)] + groups[0]:
                cp.start()
            setup()
            x_copy(0).wait()
            for cp in groups[1]:
                cp.start()
            norm_first()
            for f in prep(0):
                f()
        for n, (kind, u) in enumerate(todo):
            side = prep(n + 1) if load and n < 11 else []
            if n >= 4:
                side += [P(k_rep, n - 4, 0), ]
                side += [P(ln_in if n >= 8 else ln_stats, 1, 2 * (n % 4) + j) for j in range(2)]
            for f in pieces(kind, 0, u):
                y = f()
                if side:
                    release(y, side[:1])
                    side.pop(0)()

    def layer(li):
        first, last = li == 0, li == 1
        first_chunk(first)
        stage(0, out=False, fin=False, load=first)
        if first:
            for c in range(3, NC):
                x_copy(c).wait()
            for cp in f_copies:
                cp.start()

        def body(t, _):
            stage(t)
            if last:
                pl.when(t >= 2)(lambda: o_copy(t - 2).start())

        lax.fori_loop(1, NC - 1, body, None)
        if first:
            for cp in f_copies:
                cp.wait()
        stage(NC - 1, qkv=False, ln=False)
        for i in range(4):
            prep_o(NC - 1, i)
        for u in range(4):
            for n, f in enumerate(pieces(3, NC - 1, u)):
                y = f()
                if n in (0, 3):
                    release(y, [P(post)])
                    post(NC - 2, 2 * u + n // 3)

        def argmax(lo, hi):
            r = r_s[lo:hi, :]
            top = jnp.max(r, axis=0, keepdims=True)
            at = jnp.min(jnp.where(r == top, iota(r.shape, 0) + lo, S - 1), axis=0, keepdims=True)
            return top[:, 0:1], at[:, 0:1]

        top0, at0 = argmax(0, S - 2 * TM)
        for j in range(8):
            post(NC - 1, j)
        top1, at1 = argmax(S - 2 * TM, S)
        rmax = jnp.maximum(top0, top1)
        idx = jnp.min(jnp.where(top1 > top0, at1, at0))
        base = (idx // 16) * 16
        blk = _ds(base, 16)

        x1 = x1_s[blk, :].astype(F32)
        hs = _ln(x1).astype(BF)
        acts = []
        for j in range(F // FC):
            cols = slice(j * FC, (j + 1) * FC)
            gt = _rb(_nn(hs, wg_s[:, cols]))
            up = _rb(_nn(hs, wu_s[:, cols]))
            acts.append((_rb(gt * jax.nn.sigmoid(gt)) * up).astype(BF))
            if last and j == 2:
                for c in range(NC - 3, NC):
                    o_copy(c).start()
        if first:
            norm_first()
        a = jnp.concatenate(acts, 1)
        y = _nn(a, _bf16([wd_w[g] for g in range(8)], 1))
        y = _rb(_rb(y) * _rb(jax.nn.sigmoid(rmax)))
        upd = jnp.where(iota((16, D), 0) == idx - base, y, 0.0)
        new = (x1 + _rb(hs.astype(F32) + upd)).astype(BF)
        if first:
            x_s[blk, :] = new
            ln_stats(0, base % TM // RB)
            ln_in(0, base % 128 // 16)
        else:
            for c in range(NC):
                o_copy(c).wait()
            x_s[blk, :] = new
            cp = pltpu.make_async_copy(x_s.at[blk], out_hbm.at[blk], o_sem.at[0])
            cp.start()
            cp.wait()

    layer(0)
    layer(1)


@jax.jit
def pallas_interleave_layers__sliding_block__moe_arch_mod__prompt_kernel(
    A_x: jax.Array,
    A_wqkv: jax.Array,
    A_wo: jax.Array,
    B_x: jax.Array,
    B_w_r: jax.Array,
    B_w_gate: jax.Array,
    B_w_up: jax.Array,
    B_w_down: jax.Array,
):
    del B_x
    hbm = pl.BlockSpec(memory_space=pl.ANY)
    out = pl.pallas_call(
        _kernel,
        out_shape=jax.ShapeDtypeStruct((S, D), BF),
        in_specs=[pl.BlockSpec(memory_space=pltpu.VMEM)] + [hbm] * 6,
        out_specs=hbm,
        scratch_shapes=[
            pltpu.VMEM((S + TM + 16, D), BF),
            pltpu.VMEM((S + TM + 16, D), BF),
            pltpu.VMEM((7, 4, 128, 128), BF),
            pltpu.VMEM((7, 4, 128, 128), BF),
            pltpu.VMEM((7, 4, 64, 128), I32),
            pltpu.VMEM((NHG, S, 128), BF),
            pltpu.VMEM((3, NHG, D, 128), BF),
            pltpu.VMEM((9, D, 128), BF),
            pltpu.VMEM((D, F), BF),
            pltpu.VMEM((D, F), BF),
            pltpu.VMEM((8, F, 128), BF),
            pltpu.VMEM((16, 7, 4, 64, 128), I32),
            pltpu.VMEM((4, 128, 128), F32),
            pltpu.VMEM((NQB, NHG, 128, 128), BF),
            pltpu.VMEM((NQB, NHG, 128, 128), BF),
            pltpu.VMEM((NHG + 1, 2, 128, 128), F32),
            pltpu.VMEM((NHG, 67 * 16, 128), I32),
            pltpu.VMEM((32, 64 * 16, 128), I32),
            pltpu.VMEM((5, 9, 32, 128), F32),
            pltpu.VMEM((5, 9, 32, 128), F32),
            pltpu.VMEM((24, 64, 128), I32),
            pltpu.VMEM((2, 64, 128), I32),
            pltpu.VMEM((RB, D), F32),
            pltpu.VMEM((S + TM, 128), F32),
            pltpu.VMEM((2, TM, 128), F32),
            pltpu.SMEM((1,), I32),
            pltpu.SemaphoreType.DMA((NC,)),
            pltpu.SemaphoreType.DMA((3 * NHG,)),
            pltpu.SemaphoreType.DMA((NHG,)),
            pltpu.SemaphoreType.DMA((10,)),
            pltpu.SemaphoreType.DMA((NC,)),
        ],
        compiler_params=pltpu.CompilerParams(vmem_limit_bytes=110 * 1024 * 1024),
    )(B_w_r, A_x.reshape(S, D), A_wqkv, A_wo, B_w_gate, B_w_up, B_w_down)
    return out.reshape(1, S, D)
```

```python
import functools

import jax
import jax.numpy as jnp
import numpy as np
from jax import lax
import jax.experimental.pallas as pl
import jax.experimental.pallas.tpu as pltpu

S, D, F = 2048, 1024, 3584
NHG = 8
NQB = S // 128
TM = 256
NC = S // TM
RB = TM // 8
FC = 512
BF, F32, I32 = jnp.bfloat16, jnp.float32, jnp.int32
NEG = -1e9
LAG = 2
T0 = 1
P0 = 16
P1 = 48
O0 = 2
O1 = 34
Q0 = 65
Q7 = 12
KP = 0
T1 = 16
E1 = 65
L0 = 1
L1 = 64
K0 = 0
K1 = 48

_bf = lambda v: float(np.asarray(v, dtype=jnp.bfloat16).astype(np.float32))
QSCALE = _bf(32 ** -0.5) * float(np.log2(np.e))
EPS = _bf(1e-5)


def _rb(x):
    return x.astype(BF).astype(F32)


def _stats(x):
    m = jnp.mean(x, axis=1, keepdims=True)
    xc = x - m
    v = jnp.mean(xc * xc, axis=1, keepdims=True)
    return m, xc, 1.0 / _rb(jnp.sqrt(_rb(_rb(v) + EPS)))


def _ln(x):
    _, xc, inv = _stats(x)
    return xc * inv


def _nt(a, b):
    return lax.dot_general(a, b, (((1,), (1,)), ((), ())), preferred_element_type=F32)


def _nn(a, b):
    return jnp.dot(a, b, preferred_element_type=F32)


def _pack(lo, hi):
    return pltpu.bitcast(pltpu.pack_elementwise([lo, hi], packed_dtype=BF), I32)


def _bf16(words, axis):
    return jnp.concatenate([pltpu.bitcast(w, BF) for w in words], axis)


def _lhs_terms(a11, a12, a21, a22):
    return [a11 + a22, a21 + a22, a11, a22, a11 + a12, a21 - a11, a12 - a22]


def _rhs_terms(b11, b12, b21, b22):
    return [b11 + b22, b11, b12 - b22, b21 - b11, b22, b11 + b12, b21 + b22]


def _on_words(fn, words):
    lo, hi = (fn(*[pltpu.unpack_elementwise(w, index=i, packed_dtype=BF, unpacked_dtype=F32)
                   for w in words]) for i in range(2))
    return [_pack(a, b) for a, b in zip(lo, hi)]


def _ds(start, size):
    return pl.ds(start if isinstance(start, int) else pl.multiple_of(start, size), size)


def _spread(slots, pieces, lo, hi):
    for i, f in enumerate(pieces):
        slots[lo + i * (hi - lo) // len(pieces)].append(f)


def _kernel(wr_ref, x_hbm, wqkv_hbm, wo_hbm, wg_hbm, wu_hbm, wd_hbm, out_hbm,
            x_s, x1_s, ha_s, hb_s, oa_s, o_s, w_s, wo_s, wg_s, wu_s, wd_s, ws_s, c_s, qt_s, vt_s, kf_s, kp_s, kr_s,
            s0_s, s1_s, p_s, tri_s, wr_s, top_s, at_s, st_s, z_s, y_s,
            sem):
    ha_w, hb_w, o_w, w_w, wo_w, qt_w, vt_w, wg_w, wu_w, wd_w = (
        r.bitcast(I32) for r in (ha_s, hb_s, o_s, w_s, wo_s, qt_s, vt_s, wg_s, wu_s, wd_s))

    s_s = (s0_s, s1_s)

    todo = [(kind, u) for kind in (1, 0, 2) for u in range(4)]

    def x_in(*cs):
        return [(x_hbm.at[_ds(c * TM, TM)], x_s.at[_ds(c * TM, TM)]) for c in cs]

    def w_in(*ns):
        tiles = [(todo[n][0], 2 * todo[n][1] + e) for n in ns for e in range(2)]
        return [(wqkv_hbm.at[:, pl.ds(j * D + g * 128, 128)], w_s.at[j, g]) for j, g in tiles]

    def slabs(src, dst):
        return [(src.at[:, pl.ds(g * 128, 128)], dst.at[g]) for g in range(src.shape[1] // 128)]

    groups = [x_in(0), w_in(0), w_in(1, 2), w_in(3, 4) + x_in(1), w_in(5, 6), w_in(7, 8),
              w_in(9, 10, 11), x_in(2) + slabs(wo_hbm, wo_s), x_in(*range(3, NC)),
              slabs(wg_hbm, wg_s) + slabs(wu_hbm, wu_s) + slabs(wd_hbm, wd_s)]

    def start(n):
        for src, dst in groups[n]:
            pltpu.make_async_copy(src, dst, sem.at[n]).start()

    def wait(n):
        for src, dst in groups[n]:
            pltpu.make_async_copy(src, dst, sem.at[n]).wait()

    def out_copy(row, size):
        rows = _ds(row, size)
        return pltpu.make_async_copy(x_s.at[rows], out_hbm.at[rows], sem.at[len(groups)])

    def iota(shape, d):
        return lax.broadcasted_iota(I32, shape, d)

    r32, c32 = iota((32, 128), 0), iota((32, 128), 1)
    tri32 = jnp.where(r32 < 16, 2 * r32, 2 * r32 - 31) <= c32 % 32
    grp32 = c32 // 32
    grp = iota((16, 128), 1) // 32
    odd, high = grp % 2 == 1, grp >= 2
    r64, c64 = iota((64, 128), 0), iota((64, 128), 1)
    triw = jnp.where(2 * r64 <= c64, 0xFFFF, 0) | jnp.where(2 * r64 + 1 <= c64, -65536, 0)

    def setup():
        tri_s[0], tri_s[1] = ~triw, triw
        wr_s[...] = jnp.broadcast_to(wr_ref[...].astype(F32).reshape(1, D), (RB, D))
        z_s[0] = 0
        x_s[S:S + TM, :] = jnp.zeros((TM, D), BF)
        x1_s[S:S + TM, :] = jnp.zeros((TM, D), BF)
        kp_s[:, 0:48, :] = jnp.zeros((NHG, 48, 128), I32)

    def static(c):
        return isinstance(c, int)

    def hide(c):
        return z_s[0] if static(c) else 0

    def ln_stats(c, j):
        m, _, inv = _stats(x_s[_ds(z_s[0] + c * TM + j * RB, RB), :].astype(F32))
        inv = jnp.broadcast_to(inv, (RB, 128))
        st_s[0, _ds(j * RB, RB)] = jnp.broadcast_to(m, (RB, 128))
        st_s[1, _ds(j * RB, RB)] = inv
        return inv

    def ln_in(c, j):
        def h(b, i):
            r = b * 128 + j * 16
            x = x_s[_ds(z_s[0] + c * TM + r, 16), i * 128:(i + 1) * 128].astype(F32)
            return (x - st_s[0, _ds(r, 16)]) * st_s[1, _ds(r, 16)]

        for i in range(4):
            terms = _lhs_terms(h(0, i), h(0, i + 4), h(1, i), h(1, i + 4))
            for m, a in enumerate(terms):
                (hb_s if static(c) and c == 1 else ha_s)[m, i, _ds(j * 16, 16), :] = a.astype(BF)
        return jnp.concatenate(terms[:2], 0)

    def prep_o(c, i, e):
        words = [o_w[g, _ds((2 * c + b) * 64 + e * 32, 32), :] for b in range(2) for g in (i, i + 4)]
        for m, a in enumerate(_on_words(_lhs_terms, words)):
            oa_s[m, i, e * 32:(e + 1) * 32] = a
        return pltpu.bitcast(a, F32)

    def prep_w(kind, u, i):
        src = wo_w if kind == 3 else w_w.at[kind]
        z = z_s[0] if kind == 3 else 0
        words = [src[z + 2 * u + n % 2, pl.ds((i + 4 * (n // 2)) * 64, 64), :] for n in range(4)]
        if kind in (0, 2):
            words = [pltpu.bitcast(pltpu.bitcast(w, BF).T, I32) for w in words]
        for m, a in enumerate(_on_words(_rhs_terms, words)):
            ws_s[kind * 4 + u, m, i] = a
        return pltpu.bitcast(a[32:], F32)

    def emit(kind, c, b, g, y):
        if kind == 0:
            qt_s[2 * c + b, g] = (y * QSCALE).astype(BF)
        elif kind == 1:
            kf_s[g, b] = y
        elif kind == 2:
            vt_s[2 * c + b, g] = y.astype(BF)
        else:
            rows, cols = _ds((2 * c + b) * 128, 128), slice(g * 128, (g + 1) * 128)
            x1_s[rows, cols] = (x_s[rows, cols].astype(F32) + y).astype(BF)

    def proj(kind, c, u, m):
        src = oa_s if kind == 3 else hb_w if static(c) and c == 1 else ha_w
        a = _bf16([src[hide(c) + m, i] for i in range(4)], 1)
        w = [ws_s[kind * 4 + u, m, i] for i in range(4)]
        y = _nt(_bf16(w, 1), a) if kind in (0, 2) else _nn(a, _bf16(w, 0))
        if m == 6:
            c_s[0] = y
        elif m == 4:
            c_s[0] -= y
            c_s[1] = y
        elif m == 2:
            emit(kind, c, 0, 2 * u + 1, c_s[1] + y)
            c_s[3] = y
        elif m == 0:
            c_s[0] += y
            c_s[3] += y
        elif m == 3:
            emit(kind, c, 0, 2 * u, c_s[0] + y)
            c_s[2] = y
        elif m == 1:
            emit(kind, c, 1, 2 * u, c_s[2] + y)
            c_s[3] -= y
        else:
            emit(kind, c, 1, 2 * u + 1, c_s[3] + y)
        return y

    def k_rep(g, c):
        blocks = [kp_s[g, _ds(hide(c) + (c * 8 + i) * 16, 16), :] for i in range(3)]
        for i in range(8):
            ld = lambda o: kf_s[(z_s[0] if KP else hide(c)) + g, i // 4, pl.ds((i % 4) * 32 + o, 8, stride=4), :]
            blocks.append(jnp.concatenate([_pack(ld(0), ld(2)), _pack(ld(1), ld(3))], 0))
        for i in range(8, 11):
            kp_s[g, _ds((c * 8 + i) * 16, 16), :] = blocks[i]
        for j in range(8):
            r = [blocks[j]] + [pltpu.roll(blocks[j + s], 32 * s, 1) for s in (1, 2, 3)]
            y = [jnp.where(odd, r[(m + 1) % 4], r[m]) for m in range(4)]
            for h in range(4):
                kr_s[g * 4 + h, _ds((c * 8 + j) * 16, 16), :] = jnp.where(
                    high, y[(2 - h) % 4], y[-h % 4])

    def qk(g, b, slot):
        lo = max(5 - 4 * b, 0) if isinstance(b, int) else 0
        order = ([8] if lo else [0, 8]) + list(range(max(lo, 1), 8))
        res = []
        for h in range(4):
            q = qt_w[b, g, h * 16:(h + 1) * 16, :]
            w = jnp.concatenate([jnp.where(grp == (p - h) % 4, q, 0) for p in range(4)], 0)
            k = jnp.concatenate(
                [kr_s[g * 4 + h, _ds(hide(b) + (4 * b - 5 + i) * 16, 16), :] for i in order], 0)
            s = _nn(pltpu.bitcast(k, BF), pltpu.bitcast(w, BF))
            s = {i: s[n * 32:(n + 1) * 32] for n, i in enumerate(order)}
            s[0] = jnp.where(tri32, s.pop(8), NEG if lo else s[0])
            for i in range(lo, lo + 3 if lo else 0):
                s[i] = jnp.where(grp32 >= lo + 3 - i, s[i], NEG)
            m = functools.reduce(jnp.maximum, s.values())
            for i, v in s.items():
                s_s[slot][h, i] = v
            s_s[slot][h, 8, 0:8] = jnp.broadcast_to(jnp.max(m, axis=0, keepdims=True), (8, 128))
            res.append(sorted(s))
        return res

    def softmax(slot, h, live):
        m = jnp.concatenate([s_s[slot][z_s[0] + h, 8, 0:8]] * 4, 0)
        p = {i: jnp.exp2(s_s[slot][z_s[0] + h, i] - m) for i in live}
        l = jnp.sum(functools.reduce(jnp.add, p.values()), axis=0, keepdims=True)
        zero = jnp.zeros((16, 128), I32)
        u = [_pack(p[i][:16], p[i][16:]) if i in p else zero for i in range(8)]
        u = [jnp.where(odd, u[(i - 1) % 8], u[i]) for i in range(8)]
        u = [jnp.where(high, u[(i - 2) % 8], u[i]) for i in range(8)]
        edge = jnp.concatenate(u[:4], 0)
        z = (slot * 4 + h) * 3
        p_s[z] = edge & tri_s[0]
        p_s[z + 1] = jnp.concatenate(u[4:], 0)
        p_s[z + 2] = edge & tri_s[1]
        return 1.0 / l

    def pv(g, b, slot, sm):
        n = min(b + 1, 3) if isinstance(b, int) else 3
        outs = []
        for h, linv in enumerate(sm):
            v = jnp.concatenate([pltpu.bitcast(vt_w[b - i, g, h * 16:(h + 1) * 16, :], BF)
                                 for i in range(n - 1, -1, -1)], 1)
            outs.append(_nn(v, _bf16([p_s[(slot * 4 + h) * 3 + i] for i in range(3 - n, 3)], 0)) * linv)
        o_s[g, _ds(b * 128, 128), :] = jnp.concatenate(outs, 0).T.astype(BF)

    def post(c, j):
        rows = _ds(c * TM + j * RB, RB)
        x1 = x1_s[_ds(z_s[0] + c * TM + j * RB, RB), :].astype(F32)
        h = _rb(_ln(x1))
        x_s[rows, :] = (x1 + h).astype(BF)
        r = _rb(jnp.sum(h * wr_s[...], axis=1, keepdims=True))
        r = jnp.broadcast_to(r, (RB, 128))
        top, at = top_s[...], at_s[...]
        for i in range(0, RB, 8):
            better = jnp.where(c < NC, r[i:i + 8], -jnp.inf) > top
            top = jnp.where(better, r[i:i + 8], top)
            at = jnp.where(better, c * TM + j * RB + i + iota((8, 128), 0), at)
        top_s[...], at_s[...] = top, at
        return r

    P = functools.partial

    def pieces(kind, c, u):
        return [P(proj, kind, c, u, m) for m in (6, 4, 2, 0, 3, 1, 5)]

    def release(y, follow):
        follow = [f.func for f in follow]
        pad = _ds(S + TM, 16)
        if post in follow:
            x1_s[pad, 0:128] = y[:16].astype(BF)
        if ln_in in follow or ln_stats in follow:
            x_s[pad, :] = jnp.concatenate([y[:16]] * 8, 1).astype(BF)
        if k_rep in follow:
            kf_s[NHG, 0, 0:8] = y[:8]
        if prep_w in follow:
            wo_s[8, 0:16] = y[:16].astype(BF)

    def stage(t, qkv=True, out=True, ln=True, fin=True, load=False):
        slots = [[] for _ in range(65)]
        nq = (48 if out else Q0) if qkv else Q7
        if load:
            slots[11].append(P(wait, 7))
            _spread(slots, [P(prep_w, 3, u, i) for u in range(4) for i in range(4)], 12, 44)
        if ln:
            _spread(slots, [P(ln_stats, t + 2, j) for j in range(8)], *((T0, T1) if out else (13, 45)))
            _spread(slots, [P(ln_in, t + 2, j) for j in range(8)], *((nq + L0, L1) if out else (45, 61)))
        if fin:
            _spread(slots, [P(post, jnp.where(t >= 2, t - 2, NC), j) for j in range(8)], *((P0, P1) if ln else (8, 64)))
        if out:
            _spread(slots, [P(prep_o, t - 1, i, e) for i in range(4) for e in range(2)],
                    *((O0, O1) if qkv else (0, 8)))
        if qkv:
            _spread(slots, [P(k_rep, g, t + 1) for g in range(NHG)], nq // 3 + K0, K1)
            _spread(slots, [f for kind in (1, 0, 2) for u in range(4)
                            for f in pieces(kind, t + 1, u)], 0, nq)
        if out:
            _spread(slots, [f for u in range(4) for f in pieces(3, t - 1, u)], nq, 65)
        quads = [(g, 2 * t + i) for i in range(2) for g in range(NHG)]
        due = {}
        nxt = qk(*quads[0], 0)
        for n, quad in enumerate(quads):
            cur = nxt
            if n + 1 < len(quads):
                nxt = qk(*quads[n + 1], (n + 1) % 2)
            sm, y = [], None
            for h in range(4):
                sm.append(softmax(n % 2, h, cur[h]))
                i = 4 * n + h
                for f in slots[i]:
                    if f.func in (post, ln_in, ln_stats, prep_w, prep_o):
                        due.setdefault(i + LAG, []).append(f())
                    elif f.func is proj:
                        y = f()
                    else:
                        f()
                for e, v in enumerate(due.pop(i, []) if i < 63 else []):
                    s_s[(i + 1) // 4 % 2][4, 1 + e] = v
                if y is not None and i < 63:
                    s_s[(i + 1) // 4 % 2][4, 0, 0:8] = y[:8]
                    release(y, slots[i + 1])
            pv(*quad, n % 2, sm)
        for f in slots[64]:
            f()

    def norm_first():
        for j in range(8):
            ln_stats(0, j)
        for j in range(8):
            ln_in(0, j)

    def first_chunk(load):
        def prep(n):
            if n in (0, 1, 3, 5, 7, 9):
                wait((n + 3) // 2)
                start((n + 7) // 2)
            return [P(prep_w, *todo[n], i) for i in range(4)]

        if load:
            start(0)
            start(1)
            setup()
            wait(0)
            start(2)
            norm_first()
            for f in prep(0):
                f()
        for n, (kind, u) in enumerate(todo):
            side = prep(n + 1) if load and n < 11 else []
            if n >= 4:
                side += [P(k_rep, n - 4, 0), ]
                side += [P(ln_in if n >= 8 else ln_stats, 1, 2 * (n % 4) + j) for j in range(2)]
            for f in pieces(kind, 0, u):
                y = f()
                if side:
                    release(y, side[:1])
                    side.pop(0)()

    def argmax():
        top = jnp.max(top_s[...], axis=0, keepdims=True)
        return top[:, 0:1], jnp.min(jnp.where(top_s[...] == top, at_s[...], S - 1)[:, 0:1])

    def glu(hs, t0, n):
        gate, up = (_rb(_nn(hs, _bf16([w[t0 + i] for i in range(n)], 1))) for w in (wg_w, wu_w))
        return gate, (_rb(gate * jax.nn.sigmoid(gate)) * up).astype(BF)

    def layer(li):
        first, last = li == 0, li == 1
        first_chunk(first)
        top_s[...] = jnp.full((8, 128), -jnp.inf, F32)
        at_s[...] = iota((8, 128), 0)
        stage(0, out=False, fin=False, load=first)
        if first:
            wait(8)
            start(9)

        def body(t, _):
            stage(t)
            if last:
                pl.when(t >= 2)(lambda: out_copy((t - 2) * TM, TM).start())

        lax.fori_loop(1, NC - 1, body, None)
        if first:
            wait(9)
        stage(NC - 1, qkv=False, ln=False)
        for i in range(4):
            prep_o(NC - 1, i, 0)
            prep_o(NC - 1, i, 1)
        for n, f in enumerate([f for u in range(4) for f in pieces(3, NC - 1, u)]):
            y = f()
            if n % 5 in (0, 2) and n < 20:
                release(y, [P(post)])
                post(NC - 2, n // 5 * 2 + n % 5 // 2)

        guess = argmax()[1] // 16 * 16
        hs = _ln(x1_s[_ds(guess, 16), :].astype(F32)).astype(BF)
        acts = []
        post(NC - 1, 0)
        post(NC - 1, 1)
        for j in range(7):
            gate, a = glu(hs, 4 * j, 4)
            acts.append(a)
            if j < 6:
                release(gate[:, 0:128], [P(post)])
                post(NC - 1, j + 2)
        rmax, idx = argmax()
        base = (idx // 16) * 16
        blk = _ds(base, 16)
        if last:
            for c in range(NC - 3, NC):
                out_copy(c * TM, TM).start()
        a = jnp.concatenate(acts, 1)
        for e in range(2):
            if first:
                release(gate[:, 0:128], [P(ln_in)])
                for j in range(8):
                    (ln_in if e else ln_stats)(0, j)
            gate = _nn(a, _bf16([wd_w[4 * e + g] for g in range(4)], 1))
            y_s[:, e * 512:(e + 1) * 512] = gate
        x1 = x1_s[blk, :].astype(F32)
        hs = _ln(x1).astype(BF)

        def redo(j, _):
            a = glu(hs, 2 * j, 2)[1]
            y = _nn(a, _bf16([wd_w[g, _ds(j * 128, 128)] for g in range(8)], 1))
            y_s[...] = jnp.where(j == 0, y, y_s[...] + y)

        lax.fori_loop(0, jnp.where(base == guess, 0, F // 256), redo, None)
        y = _rb(_rb(y_s[...]) * _rb(jax.nn.sigmoid(rmax)))
        upd = jnp.where(iota((16, D), 0) == idx - base, y, 0.0)
        new = (x1 + _rb(hs.astype(F32) + upd)).astype(BF)
        if first:
            x_s[blk, :] = new
            ln_stats(0, base % TM // RB)
            ln_in(0, base % 128 // 16)
        else:
            for c in range(NC):
                out_copy(c * TM, TM).wait()
            x_s[blk, :] = new
            out_copy(base, 16).start()
            out_copy(base, 16).wait()

    layer(0)
    layer(1)


@jax.jit
def pallas_interleave_layers__sliding_block__moe_arch_mod__prompt_kernel(
    A_x: jax.Array,
    A_wqkv: jax.Array,
    A_wo: jax.Array,
    B_x: jax.Array,
    B_w_r: jax.Array,
    B_w_gate: jax.Array,
    B_w_up: jax.Array,
    B_w_down: jax.Array,
):
    del B_x
    hbm = pl.BlockSpec(memory_space=pl.ANY)
    out = pl.pallas_call(
        _kernel,
        out_shape=jax.ShapeDtypeStruct((S, D), BF),
        in_specs=[pl.BlockSpec(memory_space=pltpu.VMEM)] + [hbm] * 6,
        out_specs=hbm,
        scratch_shapes=[
            pltpu.VMEM((S + TM + 16, D), BF),
            pltpu.VMEM((S + TM + 16, D), BF),
            pltpu.VMEM((7, 4, 128, 128), BF),
            pltpu.VMEM((7, 4, 128, 128), BF),
            pltpu.VMEM((7, 4, 64, 128), I32),
            pltpu.VMEM((NHG, S, 128), BF),
            pltpu.VMEM((3, NHG, D, 128), BF),
            pltpu.VMEM((9, D, 128), BF),
            pltpu.VMEM((F // 128, D, 128), BF),
            pltpu.VMEM((F // 128, D, 128), BF),
            pltpu.VMEM((8, F, 128), BF),
            pltpu.VMEM((16, 7, 4, 64, 128), I32),
            pltpu.VMEM((4, 128, 128), F32),
            pltpu.VMEM((NQB, NHG, 128, 128), BF),
            pltpu.VMEM((NQB, NHG, 128, 128), BF),
            pltpu.VMEM((NHG + 1, 2, 128, 128), F32),
            pltpu.VMEM((NHG, 67 * 16, 128), I32),
            pltpu.VMEM((32, 64 * 16, 128), I32),
            pltpu.VMEM((5, 9, 32, 128), F32),
            pltpu.VMEM((5, 9, 32, 128), F32),
            pltpu.VMEM((24, 64, 128), I32),
            pltpu.VMEM((2, 64, 128), I32),
            pltpu.VMEM((RB, D), F32),
            pltpu.VMEM((8, 128), F32),
            pltpu.VMEM((8, 128), I32),
            pltpu.VMEM((2, TM, 128), F32),
            pltpu.SMEM((1,), I32),
            pltpu.VMEM((16, D), F32),
            pltpu.SemaphoreType.DMA((11,)),
        ],
        compiler_params=pltpu.CompilerParams(vmem_limit_bytes=110 * 1024 * 1024),
    )(B_w_r, A_x.reshape(S, D), A_wqkv, A_wo, B_w_gate, B_w_up, B_w_down)
    return out.reshape(1, S, D)
```

```python
import functools

import jax
import jax.numpy as jnp
import numpy as np
from jax import lax
import jax.experimental.pallas as pl
import jax.experimental.pallas.tpu as pltpu

S, D, F = 2048, 1024, 3584
NHG = 8
NQB = S // 128
TM = 256
NC = S // TM
RB = TM // 8
FC = 512
BF, F32, I32 = jnp.bfloat16, jnp.float32, jnp.int32
NEG = -1e9
LAG = 2
RC = 0
MZ = 1
KP = 1
K0 = 26
K1 = 58
D7 = 32
L0 = 0
L1 = 12
T0 = 13
T1 = 29
P0 = 28
P1 = 60
O0 = 19
O1 = 4
E1 = 3

_bf = lambda v: float(np.asarray(v, dtype=jnp.bfloat16).astype(np.float32))
QSCALE = _bf(32 ** -0.5) * float(np.log2(np.e))
EPS = _bf(1e-5)


def _rb(x):
    return x.astype(BF).astype(F32)


def _stats(x):
    m = jnp.mean(x, axis=1, keepdims=True)
    xc = x - m
    v = jnp.mean(xc * xc, axis=1, keepdims=True)
    return m, xc, 1.0 / _rb(jnp.sqrt(_rb(_rb(v) + EPS)))


def _ln(x):
    _, xc, inv = _stats(x)
    return xc * inv


def _nt(a, b):
    return lax.dot_general(a, b, (((1,), (1,)), ((), ())), preferred_element_type=F32)


def _nn(a, b):
    return jnp.dot(a, b, preferred_element_type=F32)


def _pack(lo, hi):
    return pltpu.bitcast(pltpu.pack_elementwise([lo, hi], packed_dtype=BF), I32)


def _bf16(words, axis):
    return jnp.concatenate([pltpu.bitcast(w, BF) for w in words], axis)


def _lhs_terms(a11, a12, a21, a22):
    return [a11 + a22, a21 + a22, a11, a22, a11 + a12, a21 - a11, a12 - a22]


def _rhs_terms(b11, b12, b21, b22):
    return [b11 + b22, b11, b12 - b22, b21 - b11, b22, b11 + b12, b21 + b22]


def _unpack(w, i):
    return pltpu.unpack_elementwise(w, index=i, packed_dtype=BF, unpacked_dtype=F32)


def _rb2(x):
    w = _pack(x[:x.shape[0] // 2], x[x.shape[0] // 2:])
    return jnp.concatenate([_unpack(w, 0), _unpack(w, 1)], 0)


def _on_words(fn, words):
    lo, hi = (fn(*[_unpack(w, i) for w in words]) for i in range(2))
    return [_pack(a, b) for a, b in zip(lo, hi)]


def _ds(start, size):
    return pl.ds(start if isinstance(start, int) else pl.multiple_of(start, size), size)


def _spread(slots, pieces, lo, hi):
    for i, f in enumerate(pieces):
        slots[lo + i * (hi - lo) // len(pieces)].append(f)


def _kernel(wr_ref, x_hbm, wqkv_hbm, wo_hbm, wg_hbm, wu_hbm, wd_hbm, out_hbm,
            x_s, x1_s, ha_s, hb_s, oa_s, o_s, w_s, wo_s, wg_s, wu_s, wd_s, ws_s, c_s, qt_s, vt_s, kf_s, kp_s, kr_s,
            s0_s, s1_s, p_s, tri_s, wr_s, top_s, at_s, st_s, z_s, y_s,
            sem):
    x_w, x1_w, o_w, w_w, wo_w, qt_w, vt_w, wg_w, wu_w, wd_w = (
        r.bitcast(I32) for r in (x_s, x1_s, o_s, w_s, wo_s, qt_s, vt_s, wg_s, wu_s, wd_s))

    s_s = (s0_s, s1_s)

    todo = [(kind, u) for kind in (1, 0, 2) for u in range(4)]

    def x_in(lo, hi):
        rows = pl.ds(lo * TM, (hi - lo) * TM)
        return [(x_hbm.at[rows, pl.ds(g * 128, 128)], x_s.at[g, rows]) for g in range(8)]

    def w_in(*ns):
        tiles = [(todo[n][0], 2 * todo[n][1] + e) for n in ns for e in range(2)]
        return [(wqkv_hbm.at[:, pl.ds(j * D + g * 128, 128)], w_s.at[j, g]) for j, g in tiles]

    def slabs(src, dst):
        return [(src.at[:, pl.ds(g * 128, 128)], dst.at[g]) for g in range(src.shape[1] // 128)]

    groups = [x_in(0, 1), w_in(0), w_in(1, 2), w_in(3, 4) + x_in(1, 2), w_in(5, 6), w_in(7, 8),
              w_in(9, 10, 11), x_in(2, 3) + slabs(wo_hbm, wo_s), x_in(3, NC),
              slabs(wg_hbm, wg_s) + slabs(wu_hbm, wu_s) + slabs(wd_hbm, wd_s)]

    def start(n):
        for src, dst in groups[n]:
            pltpu.make_async_copy(src, dst, sem.at[n]).start()

    def wait(n):
        for src, dst in groups[n]:
            pltpu.make_async_copy(src, dst, sem.at[n]).wait()

    def out_copies(rows):
        return [pltpu.make_async_copy(x_s.at[g, rows], out_hbm.at[rows, pl.ds(g * 128, 128)],
                                      sem.at[len(groups)]) for g in range(8)]

    def iota(shape, d):
        return lax.broadcasted_iota(I32, shape, d)

    mk = {}

    def make_masks():
        row, col = iota((32, 128), 0) + z_s[0], iota((32, 128), 1) + (z_s[0] if MZ else 0)
        mk["tri"] = jnp.where(row < 16, 2 * row, 2 * row - 31) <= (col & 31)
        mk["grp"] = col >> 5
        mk["odd"], mk["high"] = (col[:16] & 32) != 0, col[:16] >= 64

    r64, c64 = iota((64, 128), 0), iota((64, 128), 1)
    triw = jnp.where(2 * r64 <= c64, 0xFFFF, 0) | jnp.where(2 * r64 + 1 <= c64, -65536, 0)

    def setup():
        tri_s[0], tri_s[1] = ~triw, triw
        wr_s[...] = jnp.broadcast_to(wr_ref[...].astype(F32).reshape(1, D), (RB, D))
        z_s[0] = 0
        kp_s[:, 0:48, :] = jnp.zeros((NHG, 48, 128), I32)

    def static(c):
        return isinstance(c, int)

    def hide(c):
        return z_s[0] if static(c) else 0

    def terms(kind, c):
        if static(c) and c == (NC - 1 if kind == 3 else 1):
            return hb_s
        return oa_s if kind == 3 else ha_s

    def tokens(ref_w, c, j):
        rows = _ds(z_s[0] + c * (TM // 2) + j * 16, 16)
        w = jnp.concatenate([ref_w[g, rows, :] for g in range(8)], 1)
        return jnp.concatenate([_unpack(w, 0), _unpack(w, 1)], 0)

    def ln_stats(c, j):
        m, _, inv = _stats(tokens(x_w, c, j))
        m, inv = jnp.broadcast_to(m, (RB, 128)), jnp.broadcast_to(inv, (RB, 128))
        for e in range(2):
            st_s[0, e, _ds(j * 16, 16)] = m[e * 16:(e + 1) * 16]
            st_s[1, e, _ds(j * 16, 16)] = inv[e * 16:(e + 1) * 16]
        return inv

    def ln_in(c, j):
        dst = terms(0, c)
        for i in range(4):
            h = [[], []]
            for b in range(2):
                r = b * 64 + j * 8
                for g in (i, i + 4):
                    w = x_w[g, _ds(z_s[0] + c * (TM // 2) + r, 8), :]
                    for e in range(2):
                        h[e].append((_unpack(w, e) - st_s[0, e, _ds(r, 8)]) * st_s[1, e, _ds(r, 8)])
            lo, hi = _lhs_terms(*h[0]), _lhs_terms(*h[1])
            for m in range(7):
                dst[m, i, _ds(j * 8, 8)] = _pack(lo[m], hi[m])
        return jnp.concatenate(lo[:2] + hi[:2], 0)

    def prep_o(c, i, e):
        words = [o_w[g, _ds((2 * c + b) * 64 + e * 32, 32), :] for b in range(2) for g in (i, i + 4)]
        for m, a in enumerate(_on_words(_lhs_terms, words)):
            terms(3, c)[m, i, e * 32:(e + 1) * 32] = a
        return pltpu.bitcast(a, F32)

    def prep_w(kind, u, i):
        src = wo_w if kind == 3 else w_w.at[kind]
        z = z_s[0] if kind == 3 else 0
        words = [src[z + 2 * u + n % 2, pl.ds((i + 4 * (n // 2)) * 64, 64), :] for n in range(4)]
        if kind in (0, 2):
            words = [pltpu.bitcast(pltpu.bitcast(w, BF).T, I32) for w in words]
        for m, a in enumerate(_on_words(_rhs_terms, words)):
            ws_s[kind * 4 + u, m, i] = a
        return pltpu.bitcast(a[32:], F32)

    def emit(kind, c, b, g, y):
        if kind == 0:
            qt_s[2 * c + b, g] = (y * QSCALE).astype(BF)
        elif kind == 1:
            kf_s[g, b] = y
        elif kind == 2:
            vt_s[2 * c + b, g] = y.astype(BF)
        else:
            x = pltpu.bitcast(x_w[g, _ds((2 * c + b) * 64, 64), :], BF).astype(F32)
            x1_s[g, _ds((2 * c + b) * 128, 128), :] = (x + y).astype(BF)

    def proj(kind, c, u, m):
        src = terms(kind, c)
        a = _bf16([src[hide(c) + m, i] for i in range(4)], 1)
        w = [ws_s[kind * 4 + u, m, i] for i in range(4)]
        y = _nt(_bf16(w, 1), a) if kind in (0, 2) else _nn(a, _bf16(w, 0))
        if m == 6:
            c_s[0] = y
        elif m == 4:
            c_s[0] -= y
            c_s[1] = y
        elif m == 2:
            emit(kind, c, 0, 2 * u + 1, c_s[1] + y)
            c_s[3] = y
        elif m == 0:
            c_s[0] += y
            c_s[3] += y
        elif m == 3:
            emit(kind, c, 0, 2 * u, c_s[0] + y)
            c_s[2] = y
        elif m == 1:
            emit(kind, c, 1, 2 * u, c_s[2] + y)
            c_s[3] -= y
        else:
            emit(kind, c, 1, 2 * u + 1, c_s[3] + y)
        return y

    def k_rep(g, c):
        blocks = [kp_s[g, _ds(hide(c) + (c * 8 + i) * 16, 16), :] for i in range(3)]
        for i in range(8):
            ld = lambda o: kf_s[(z_s[0] if KP else hide(c)) + g, i // 4, pl.ds((i % 4) * 32 + o, 8, stride=4), :]
            blocks.append(jnp.concatenate([_pack(ld(0), ld(2)), _pack(ld(1), ld(3))], 0))
        for i in range(8, 11):
            kp_s[g, _ds((c * 8 + i) * 16, 16), :] = blocks[i]
        for j in range(8):
            r = [blocks[j]] + [pltpu.roll(blocks[j + s], 32 * s, 1) for s in (1, 2, 3)]
            y = [jnp.where(mk["odd"], r[(m + 1) % 4], r[m]) for m in range(4)]
            for h in range(4):
                kr_s[g * 4 + h, _ds((c * 8 + j) * 16, 16), :] = jnp.where(
                    mk["high"], y[(2 - h) % 4], y[-h % 4])

    def qk(g, b, slot):
        lo = max(5 - 4 * b, 0) if isinstance(b, int) else 0
        order = ([8] if lo else [0, 8]) + list(range(max(lo, 1), 8))
        res = []
        for h in range(4):
            q = qt_w[b, g, h * 16:(h + 1) * 16, :]
            w = jnp.concatenate([jnp.where(mk["grp"][:16] == (p - h) % 4, q, 0) for p in range(4)], 0)
            k = jnp.concatenate(
                [kr_s[g * 4 + h, _ds(hide(b) + (4 * b - 5 + i) * 16, 16), :] for i in order], 0)
            s = _nn(pltpu.bitcast(k, BF), pltpu.bitcast(w, BF))
            s = {i: s[n * 32:(n + 1) * 32] for n, i in enumerate(order)}
            s[0] = jnp.where(mk["tri"], s.pop(8), NEG if lo else s[0])
            for i in range(lo, lo + 3 if lo else 0):
                s[i] = jnp.where(mk["grp"] >= lo + 3 - i, s[i], NEG)
            m = functools.reduce(jnp.maximum, s.values())
            for i, v in s.items():
                s_s[slot][h, i] = v
            s_s[slot][h, 8, 0:8] = jnp.broadcast_to(jnp.max(m, axis=0, keepdims=True), (8, 128))
            res.append(sorted(s))
        return res

    def softmax(slot, h, live):
        m = jnp.concatenate([s_s[slot][z_s[0] + h, 8, 0:8]] * 4, 0)
        p = {i: jnp.exp2(s_s[slot][z_s[0] + h, i] - m) for i in live}
        l = jnp.sum(functools.reduce(jnp.add, p.values()), axis=0, keepdims=True)
        zero = jnp.zeros((16, 128), I32)
        u = [_pack(p[i][:16], p[i][16:]) if i in p else zero for i in range(8)]
        u = [jnp.where(mk["odd"], u[(i - 1) % 8], u[i]) for i in range(8)]
        u = [jnp.where(mk["high"], u[(i - 2) % 8], u[i]) for i in range(8)]
        edge = jnp.concatenate(u[:4], 0)
        z = (slot * 4 + h) * 3
        p_s[z] = edge & tri_s[0]
        p_s[z + 1] = jnp.concatenate(u[4:], 0)
        p_s[z + 2] = edge & tri_s[1]
        return pl.reciprocal(l, full_range=False) if RC else 1.0 / l

    def pv(g, b, slot, sm):
        n = min(b + 1, 3) if isinstance(b, int) else 3
        outs = []
        for h, linv in enumerate(sm):
            v = jnp.concatenate([pltpu.bitcast(vt_w[b - i, g, h * 16:(h + 1) * 16, :], BF)
                                 for i in range(n - 1, -1, -1)], 1)
            outs.append(_nn(v, _bf16([p_s[(slot * 4 + h) * 3 + i] for i in range(3 - n, 3)], 0)) * linv)
        o_s[g, _ds(b * 128, 128), :] = jnp.concatenate(outs, 0).T.astype(BF)

    def post(c, j):
        x1 = tokens(x1_w, c, j)
        h = _rb2(_ln(x1))
        x = x1 + h
        x = _pack(x[:16], x[16:])
        for g in range(8):
            x_w[g, _ds(c * (TM // 2) + j * 16, 16), :] = x[:, g * 128:(g + 1) * 128]
        r = _rb(jnp.sum(h * wr_s[...], axis=1, keepdims=True))
        r = jnp.broadcast_to(r, (RB, 128))
        top, at = top_s[...], at_s[...]
        for i in (0, 16, 8, 24):
            better = r[i:i + 8] > top
            top = jnp.where(better, r[i:i + 8], top)
            at = jnp.where(better, c * TM + j * RB + i % 16 * 2 + i // 16 + 2 * (iota((8, 128), 0) + z_s[0]), at)
        top_s[...], at_s[...] = top, at
        return r

    P = functools.partial

    def pieces(kind, c, u):
        return [P(proj, kind, c, u, m) for m in (6, 4, 2, 0, 3, 1, 5)]

    def release(y, follow):
        follow = [f.func for f in follow]
        for ref, users in ((x1_w, [post]), (x_w, [ln_in, ln_stats])):
            for g in range(8) if any(f in follow for f in users) else []:
                ref[g, S // 2:] = pltpu.bitcast(y[:8], I32)
        if k_rep in follow:
            kf_s[NHG, 0, 0:8] = y[:8]
        if prep_w in follow:
            wo_s[8, 0:16] = y[:16].astype(BF)

    def stage(t, qkv=True, out=True, load=False):
        make_masks()
        slots = [[] for _ in range(65)]
        nd = 16 if qkv and out else 0
        if load:
            slots[11].append(P(wait, 7))
            _spread(slots, [P(prep_w, 3, u, i) for u in range(4) for i in range(4)], 12, 44)
        if qkv and out:
            _spread(slots, [P(ln_in, t + 1, j) for j in range(8)], L0, L1)
        if qkv:
            c = 2 if static(t) else jnp.minimum(t + 2, NC - 1)
            _spread(slots, [P(ln_stats, c, j) for j in range(8)], T0, T1)
            _spread(slots, [P(k_rep, g, t + 1) for g in range(NHG)], K0, K1)
        if out and qkv:
            _spread(slots, [P(post, t - 1, j) for j in range(8)], P0, P1)
        for i in range(4):
            for e in range(2):
                slots[min(16 * i + O0 + O1 * e, 64)].append(P(prep_o, t, i, e))
        fs = [f for u in range(4) for f in pieces(3, t - 1, u)] if out else []
        if qkv:
            _spread(slots, fs, 0, nd)
            fs = [f for kind, u in todo for f in pieces(kind, t + 1, u)]
        _spread(slots, fs[:-E1], nd, 64)
        slots[64] += fs[-E1:]
        quads = [(i + g, 2 * t + b) for i in range(4) for g in (0, 4) for b in range(2)]
        due = {}
        nxt = qk(*quads[0], 0)
        for n, quad in enumerate(quads):
            cur = nxt
            if n + 1 < len(quads):
                nxt = qk(*quads[n + 1], (n + 1) % 2)
            sm, y = [], None
            for h in range(4):
                sm.append(softmax(n % 2, h, cur[h]))
                i = 4 * n + h
                for f in slots[i]:
                    if f.func in (post, ln_in, ln_stats, prep_w, prep_o):
                        due.setdefault(i + LAG, []).append(f())
                    elif f.func is proj:
                        y = f()
                    else:
                        f()
                for e, v in enumerate(due.pop(i, []) if i < 63 else []):
                    s_s[(i + 1) // 4 % 2][4, 1 + e] = v
                if y is not None and i < 63:
                    s_s[(i + 1) // 4 % 2][4, 0, 0:8] = y[:8]
                    release(y, slots[i + 1])
            pv(*quad, n % 2, sm)
        for f in slots[64]:
            f()

    def norm_first():
        for j in range(8):
            ln_stats(0, j)
        for j in range(8):
            ln_in(0, j)

    def first_chunk(load):
        def prep(n):
            if n in (0, 1, 3, 5, 7, 9):
                wait((n + 3) // 2)
                start((n + 7) // 2)
            return [P(prep_w, *todo[n], i) for i in range(4)]

        if load:
            start(0)
            start(1)
            setup()
            wait(0)
            start(2)
            norm_first()
            for f in prep(0):
                f()
        make_masks()
        for n, (kind, u) in enumerate(todo):
            side = prep(n + 1) if load and n < 11 else []
            if n >= 4:
                side += [P(k_rep, n - 4, 0), ]
                side += [P(ln_in if n >= 8 else ln_stats, 1, 2 * (n % 4) + j) for j in range(2)]
            for f in pieces(kind, 0, u):
                y = f()
                if side:
                    release(y, side[:1])
                    side.pop(0)()

    def overlap(main, side, pad, lag):
        due = {}
        for n, f in enumerate(main):
            for e, v in enumerate(due.pop(n, [])):
                pad[e % 2 * 32:e % 2 * 32 + 32] = pltpu.bitcast(v, I32)
            y = f()[:, 0:128]
            release(y, side.get(n, []))
            due[n + lag] = [g() for g in side.get(n, [])]

    def argmax():
        top = jnp.max(top_s[...], axis=0, keepdims=True)
        return top[:, 0:1], jnp.min(jnp.where(top_s[...] == top, at_s[...], S - 1)[:, 0:1])

    def block(row):
        return jnp.concatenate([x1_s[g, _ds(row, 16), :] for g in range(8)], 1).astype(F32)

    def glu(hs, t0, n):
        gate, up = (_rb(_nn(hs, _bf16([w[t0 + i] for i in range(n)], 1))) for w in (wg_w, wu_w))
        return gate, (_rb(gate * jax.nn.sigmoid(gate)) * up).astype(BF)

    def layer(li):
        first, last = li == 0, li == 1
        first_chunk(first)
        top_s[...] = jnp.full((8, 128), -jnp.inf, F32)
        at_s[...] = 2 * iota((8, 128), 0)
        stage(0, out=False, load=first)
        if first:
            wait(8)
            start(9)

        def body(t, _):
            stage(t)
            if last:
                for cp in out_copies(_ds((t - 1) * TM, TM)):
                    cp.start()

        lax.fori_loop(1, NC - 1, body, None)
        if first:
            wait(9)
        stage(NC - 1, qkv=False)
        post(NC - 2, 0)
        overlap([f for u in range(4) for f in pieces(3, NC - 1, u)],
                {j * 5 // 2 - 1: [P(post, NC - 2, j)] for j in range(1, 8)}, hb_s.at[7, 0], 7)

        guess = argmax()[1] // 16 * 16
        hs = _ln(block(guess)).astype(BF)
        acts = []
        post(NC - 1, 0)
        post(NC - 1, 1)

        def up(j):
            gate, a = glu(hs, z_s[0] + 4 * j, 4)
            acts.append(a)
            return gate

        def down(j):
            y = _nn(acts[j], _bf16([wd_w[z_s[0] + g, j * 256:(j + 1) * 256] for g in range(8)], 1))
            y_s[...] = y_s[...] + y if j else y
            return y

        overlap([P(up, j) for j in range(7)],
                {j: [P(post, NC - 1, j + 2)] for j in range(6)}, wg_w.at[F // 128], 2)
        rmax, idx = argmax()
        base = (idx // 16) * 16
        blk = _ds(base, 16)
        if last:
            for cp in out_copies(pl.ds(S - 2 * TM, 2 * TM)):
                cp.start()
        side = {}
        if first:
            for j in range(2):
                ln_stats(0, j)
            side = {n: [P(ln_stats, 0, 2 * n + 2 + e) for e in range(2)] for n in range(3)}
            side.update({n: [P(ln_in, 0, j) for j in range(3 * n - 9, min(3 * n - 6, 8))]
                         for n in range(3, 6)})
        overlap([P(down, j) for j in range(7)], side, wd_w.at[8], 4)
        x1 = block(base)
        hs = _ln(x1).astype(BF)

        def redo(j, _):
            a = glu(hs, 2 * j, 2)[1]
            y = _nn(a, _bf16([wd_w[g, _ds(j * 128, 128)] for g in range(8)], 1))
            y_s[...] = jnp.where(j == 0, y, y_s[...] + y)

        lax.fori_loop(0, jnp.where(base == guess, 0, F // 256), redo, None)
        y = _rb(_rb(y_s[...]) * _rb(jax.nn.sigmoid(rmax)))
        upd = jnp.where(iota((16, D), 0) == idx - base, y, 0.0)
        new = (x1 + _rb(hs.astype(F32) + upd)).astype(BF)
        if last:
            for rows in [_ds(c * TM, TM) for c in range(NC - 2)] + [pl.ds(S - 2 * TM, 2 * TM)]:
                for cp in out_copies(rows):
                    cp.wait()
        for g in range(8):
            x_s[g, blk, :] = new[:, g * 128:(g + 1) * 128]
        if first:
            ln_stats(0, base % TM // RB)
            ln_in(0, base % 128 // 16)
        else:
            for cp in out_copies(blk):
                cp.start()
            for cp in out_copies(blk):
                cp.wait()

    layer(0)
    layer(1)


@jax.jit
def pallas_interleave_layers__sliding_block__moe_arch_mod__prompt_kernel(
    A_x: jax.Array,
    A_wqkv: jax.Array,
    A_wo: jax.Array,
    B_x: jax.Array,
    B_w_r: jax.Array,
    B_w_gate: jax.Array,
    B_w_up: jax.Array,
    B_w_down: jax.Array,
):
    del B_x
    hbm = pl.BlockSpec(memory_space=pl.ANY)
    out = pl.pallas_call(
        _kernel,
        out_shape=jax.ShapeDtypeStruct((S, D), BF),
        in_specs=[pl.BlockSpec(memory_space=pltpu.VMEM)] + [hbm] * 6,
        out_specs=hbm,
        scratch_shapes=[
            pltpu.VMEM((8, S + 16, 128), BF),
            pltpu.VMEM((8, S + 16, 128), BF),
            pltpu.VMEM((7, 4, 64, 128), I32),
            pltpu.VMEM((8, 4, 64, 128), I32),
            pltpu.VMEM((7, 4, 64, 128), I32),
            pltpu.VMEM((NHG, S, 128), BF),
            pltpu.VMEM((3, NHG, D, 128), BF),
            pltpu.VMEM((9, D, 128), BF),
            pltpu.VMEM((F // 128 + 1, D, 128), BF),
            pltpu.VMEM((F // 128, D, 128), BF),
            pltpu.VMEM((9, F, 128), BF),
            pltpu.VMEM((16, 7, 4, 64, 128), I32),
            pltpu.VMEM((4, 128, 128), F32),
            pltpu.VMEM((NQB, NHG, 128, 128), BF),
            pltpu.VMEM((NQB, NHG, 128, 128), BF),
            pltpu.VMEM((NHG + 1, 2, 128, 128), F32),
            pltpu.VMEM((NHG, 67 * 16, 128), I32),
            pltpu.VMEM((32, 64 * 16, 128), I32),
            pltpu.VMEM((5, 9, 32, 128), F32),
            pltpu.VMEM((5, 9, 32, 128), F32),
            pltpu.VMEM((24, 64, 128), I32),
            pltpu.VMEM((2, 64, 128), I32),
            pltpu.VMEM((RB, D), F32),
            pltpu.VMEM((8, 128), F32),
            pltpu.VMEM((8, 128), I32),
            pltpu.VMEM((2, 2, 128, 128), F32),
            pltpu.SMEM((1,), I32),
            pltpu.VMEM((16, D), F32),
            pltpu.SemaphoreType.DMA((11,)),
        ],
        compiler_params=pltpu.CompilerParams(vmem_limit_bytes=110 * 1024 * 1024),
    )(B_w_r, A_x.reshape(S, D), A_wqkv, A_wo, B_w_gate, B_w_up, B_w_down)
    return out.reshape(1, S, D)
```

```python
import functools

import jax
import jax.numpy as jnp
import numpy as np
from jax import lax
import jax.experimental.pallas as pl
import jax.experimental.pallas.tpu as pltpu

S, D, F = 2048, 1024, 3584
NHG = 8
NQB = S // 128
TM = 256
NC = S // TM
RB = TM // 8
FC = 512
BF, F32, I32 = jnp.bfloat16, jnp.float32, jnp.int32
NEG = -1e9
LAG = 2
RC = 0
MZ = 1
KP = 1
K0 = 26
K1 = 58
D7 = 32
L0 = 0
L1 = 12
T0 = 13
T1 = 29
P0 = 28
P1 = 60
O0 = 19
O1 = 4
E1 = 3

_bf = lambda v: float(np.asarray(v, dtype=jnp.bfloat16).astype(np.float32))
QSCALE = _bf(32 ** -0.5) * float(np.log2(np.e))
EPS = _bf(1e-5)


def _rb(x):
    return x.astype(BF).astype(F32)


def _stats(x):
    m = jnp.mean(x, axis=1, keepdims=True)
    xc = x - m
    v = jnp.mean(xc * xc, axis=1, keepdims=True)
    return m, xc, 1.0 / _rb(jnp.sqrt(_rb(_rb(v) + EPS)))


def _ln(x):
    _, xc, inv = _stats(x)
    return xc * inv


def _nt(a, b):
    return lax.dot_general(a, b, (((1,), (1,)), ((), ())), preferred_element_type=F32)


def _nn(a, b):
    return jnp.dot(a, b, preferred_element_type=F32)


def _pack(lo, hi):
    return pltpu.bitcast(pltpu.pack_elementwise([lo, hi], packed_dtype=BF), I32)


def _bf16(words, axis):
    return jnp.concatenate([pltpu.bitcast(w, BF) for w in words], axis)


def _lhs_terms(a11, a12, a21, a22):
    return [a11 + a22, a21 + a22, a11, a22, a11 + a12, a21 - a11, a12 - a22]


def _rhs_terms(b11, b12, b21, b22):
    return [b11 + b22, b11, b12 - b22, b21 - b11, b22, b11 + b12, b21 + b22]


def _unpack(w, i):
    return pltpu.unpack_elementwise(w, index=i, packed_dtype=BF, unpacked_dtype=F32)


def _rb2(x):
    w = _pack(x[:x.shape[0] // 2], x[x.shape[0] // 2:])
    return jnp.concatenate([_unpack(w, 0), _unpack(w, 1)], 0)


def _on_words(fn, words):
    lo, hi = (fn(*[_unpack(w, i) for w in words]) for i in range(2))
    return [_pack(a, b) for a, b in zip(lo, hi)]


def _ds(start, size):
    return pl.ds(start if isinstance(start, int) else pl.multiple_of(start, size), size)


def _spread(slots, pieces, lo, hi):
    for i, f in enumerate(pieces):
        slots[lo + i * (hi - lo) // len(pieces)].append(f)


def _kernel(wr_ref, x_hbm, wqkv_hbm, wo_hbm, wg_hbm, wu_hbm, wd_hbm, out_hbm,
            x_s, x1_s, ha_s, hb_s, oa_s, o_s, w_s, wo_s, wg_s, wu_s, wd_s, ws_s, c_s, qt_s, vt_s, kf_s, kp_s, kr_s,
            s0_s, s1_s, p_s, tri_s, wr_s, top_s, at_s, st_s, z_s, y_s,
            sem):
    ha_w, hb_w, x1_w, o_w, w_w, wo_w, qt_w, vt_w, wg_w, wu_w, wd_w = (
        r.bitcast(I32) for r in (ha_s, hb_s, x1_s, o_s, w_s, wo_s, qt_s, vt_s, wg_s, wu_s, wd_s))

    s_s = (s0_s, s1_s)

    todo = [(kind, u) for kind in (1, 0, 2) for u in range(4)]

    def x_in(lo, hi):
        rows = pl.ds(lo * TM, (hi - lo) * TM)
        return [(x_hbm.at[rows], x_s.at[rows])]

    def w_in(*ns):
        tiles = [(todo[n][0], 2 * todo[n][1] + e) for n in ns for e in range(2)]
        return [(wqkv_hbm.at[:, pl.ds(j * D + g * 128, 128)], w_s.at[j, g]) for j, g in tiles]

    def slabs(src, dst):
        return [(src.at[:, pl.ds(g * 128, 128)], dst.at[g]) for g in range(src.shape[1] // 128)]

    groups = [x_in(0, 1), w_in(0, 1), w_in(2, 3), w_in(4, 5), w_in(6, 7) + x_in(1, 2), w_in(8, 9),
              w_in(10, 11), x_in(2, 3) + slabs(wo_hbm, wo_s), x_in(3, NC),
              slabs(wg_hbm, wg_s) + slabs(wu_hbm, wu_s) + slabs(wd_hbm, wd_s)]

    def start(n):
        for src, dst in groups[n]:
            pltpu.make_async_copy(src, dst, sem.at[n]).start()

    def wait(n):
        for src, dst in groups[n]:
            pltpu.make_async_copy(src, dst, sem.at[n]).wait()

    def out_copies(rows):
        return [pltpu.make_async_copy(x_s.at[rows], out_hbm.at[rows], sem.at[len(groups)])]

    def iota(shape, d):
        return lax.broadcasted_iota(I32, shape, d)

    mk = {}

    def make_masks():
        row, col = iota((32, 128), 0) + z_s[0], iota((32, 128), 1) + (z_s[0] if MZ else 0)
        mk["tri"] = jnp.where(row < 16, 2 * row, 2 * row - 31) <= (col & 31)
        mk["grp"] = col >> 5
        mk["odd"], mk["high"] = (col[:16] & 32) != 0, col[:16] >= 64

    r64, c64 = iota((64, 128), 0), iota((64, 128), 1)
    triw = jnp.where(2 * r64 <= c64, 0xFFFF, 0) | jnp.where(2 * r64 + 1 <= c64, -65536, 0)

    def setup():
        tri_s[0], tri_s[1] = ~triw, triw
        wr_s[...] = jnp.broadcast_to(wr_ref[...].astype(F32).reshape(1, D), (RB, D))
        z_s[0] = 0
        kp_s[:, 0:48, :] = jnp.zeros((NHG, 48, 128), I32)

    def static(c):
        return isinstance(c, int)

    def hide(c):
        return z_s[0] if static(c) else 0

    def terms(kind, c):
        if static(c) and c == (NC - 1 if kind == 3 else 1):
            return hb_w
        return oa_s if kind == 3 else ha_w

    def ln_stats(c, j):
        m, _, inv = _stats(x_s[_ds(z_s[0] + c * TM + j * RB, RB), :].astype(F32))
        inv = jnp.broadcast_to(inv, (RB, 128))
        st_s[0, _ds(j * RB, RB)] = jnp.broadcast_to(m, (RB, 128))
        st_s[1, _ds(j * RB, RB)] = inv
        return inv

    def ln_in(c, j):
        def h(b, i):
            r = b * 128 + j * 16
            x = x_s[_ds(z_s[0] + c * TM + r, 16), i * 128:(i + 1) * 128].astype(F32)
            return (x - st_s[0, _ds(r, 16)]) * st_s[1, _ds(r, 16)]

        for i in range(4):
            terms = _lhs_terms(h(0, i), h(0, i + 4), h(1, i), h(1, i + 4))
            for m, a in enumerate(terms):
                (hb_s if static(c) and c == 1 else ha_s)[m, i, _ds(j * 16, 16), :] = a.astype(BF)
        return jnp.concatenate(terms[:2], 0)

    def prep_o(c, i, e):
        words = [o_w[g, _ds((2 * c + b) * 64 + e * 32, 32), :] for b in range(2) for g in (i, i + 4)]
        for m, a in enumerate(_on_words(_lhs_terms, words)):
            terms(3, c)[m, i, e * 32:(e + 1) * 32] = a
        return pltpu.bitcast(a, F32)

    def prep_w(kind, u, i):
        src = wo_w if kind == 3 else w_w.at[kind]
        z = z_s[0] if kind == 3 else 0
        words = [src[z + 2 * u + n % 2, pl.ds((i + 4 * (n // 2)) * 64, 64), :] for n in range(4)]
        if kind in (0, 2):
            words = [pltpu.bitcast(pltpu.bitcast(w, BF).T, I32) for w in words]
        for m, a in enumerate(_on_words(_rhs_terms, words)):
            ws_s[kind * 4 + u, m, i] = a
        return pltpu.bitcast(a[32:], F32)

    def emit(kind, c, b, g, y):
        if kind == 0:
            qt_s[2 * c + b, g] = (y * QSCALE).astype(BF)
        elif kind == 1:
            kf_s[g, b] = y
        elif kind == 2:
            vt_s[2 * c + b, g] = y.astype(BF)
        else:
            rows = _ds((2 * c + b) * 128, 128)
            x1_s[g, rows, :] = (x_s[rows, g * 128:(g + 1) * 128].astype(F32) + y).astype(BF)

    def proj(kind, c, u, m):
        src = terms(kind, c)
        a = _bf16([src[hide(c) + m, i] for i in range(4)], 1)
        w = [ws_s[kind * 4 + u, m, i] for i in range(4)]
        y = _nt(_bf16(w, 1), a) if kind in (0, 2) else _nn(a, _bf16(w, 0))
        if m == 6:
            c_s[0] = y
        elif m == 4:
            c_s[0] -= y
            c_s[1] = y
        elif m == 2:
            emit(kind, c, 0, 2 * u + 1, c_s[1] + y)
            c_s[3] = y
        elif m == 0:
            c_s[0] += y
            c_s[3] += y
        elif m == 3:
            emit(kind, c, 0, 2 * u, c_s[0] + y)
            c_s[2] = y
        elif m == 1:
            emit(kind, c, 1, 2 * u, c_s[2] + y)
            c_s[3] -= y
        else:
            emit(kind, c, 1, 2 * u + 1, c_s[3] + y)
        return y

    def k_rep(g, c):
        blocks = [kp_s[g, _ds(hide(c) + (c * 8 + i) * 16, 16), :] for i in range(3)]
        for i in range(8):
            ld = lambda o: kf_s[(z_s[0] if KP else hide(c)) + g, i // 4, pl.ds((i % 4) * 32 + o, 8, stride=4), :]
            blocks.append(jnp.concatenate([_pack(ld(0), ld(2)), _pack(ld(1), ld(3))], 0))
        for i in range(8, 11):
            kp_s[g, _ds((c * 8 + i) * 16, 16), :] = blocks[i]
        for j in range(8):
            r = [blocks[j]] + [pltpu.roll(blocks[j + s], 32 * s, 1) for s in (1, 2, 3)]
            y = [jnp.where(mk["odd"], r[(m + 1) % 4], r[m]) for m in range(4)]
            for h in range(4):
                kr_s[g * 4 + h, _ds((c * 8 + j) * 16, 16), :] = jnp.where(
                    mk["high"], y[(2 - h) % 4], y[-h % 4])

    def qk(g, b, slot):
        lo = max(5 - 4 * b, 0) if isinstance(b, int) else 0
        order = ([8] if lo else [0, 8]) + list(range(max(lo, 1), 8))
        res = []
        for h in range(4):
            q = qt_w[b, g, h * 16:(h + 1) * 16, :]
            w = jnp.concatenate([jnp.where(mk["grp"][:16] == (p - h) % 4, q, 0) for p in range(4)], 0)
            k = jnp.concatenate(
                [kr_s[g * 4 + h, _ds(hide(b) + (4 * b - 5 + i) * 16, 16), :] for i in order], 0)
            s = _nn(pltpu.bitcast(k, BF), pltpu.bitcast(w, BF))
            s = {i: s[n * 32:(n + 1) * 32] for n, i in enumerate(order)}
            s[0] = jnp.where(mk["tri"], s.pop(8), NEG if lo else s[0])
            for i in range(lo, lo + 3 if lo else 0):
                s[i] = jnp.where(mk["grp"] >= lo + 3 - i, s[i], NEG)
            m = functools.reduce(jnp.maximum, s.values())
            for i, v in s.items():
                s_s[slot][h, i] = v
            s_s[slot][h, 8, 0:8] = jnp.broadcast_to(jnp.max(m, axis=0, keepdims=True), (8, 128))
            res.append(sorted(s))
        return res

    def softmax(slot, h, live):
        m = jnp.concatenate([s_s[slot][z_s[0] + h, 8, 0:8]] * 4, 0)
        p = {i: jnp.exp2(s_s[slot][z_s[0] + h, i] - m) for i in live}
        l = jnp.sum(functools.reduce(jnp.add, p.values()), axis=0, keepdims=True)
        zero = jnp.zeros((16, 128), I32)
        u = [_pack(p[i][:16], p[i][16:]) if i in p else zero for i in range(8)]
        u = [jnp.where(mk["odd"], u[(i - 1) % 8], u[i]) for i in range(8)]
        u = [jnp.where(mk["high"], u[(i - 2) % 8], u[i]) for i in range(8)]
        edge = jnp.concatenate(u[:4], 0)
        z = (slot * 4 + h) * 3
        p_s[z] = edge & tri_s[0]
        p_s[z + 1] = jnp.concatenate(u[4:], 0)
        p_s[z + 2] = edge & tri_s[1]
        return pl.reciprocal(l, full_range=False) if RC else 1.0 / l

    def pv(g, b, slot, sm):
        n = min(b + 1, 3) if isinstance(b, int) else 3
        outs = []
        for h, linv in enumerate(sm):
            v = jnp.concatenate([pltpu.bitcast(vt_w[b - i, g, h * 16:(h + 1) * 16, :], BF)
                                 for i in range(n - 1, -1, -1)], 1)
            outs.append(_nn(v, _bf16([p_s[(slot * 4 + h) * 3 + i] for i in range(3 - n, 3)], 0)) * linv)
        o_s[g, _ds(b * 128, 128), :] = jnp.concatenate(outs, 0).T.astype(BF)

    def post(c, j):
        rows = _ds(z_s[0] + c * (TM // 2) + j * (RB // 2), RB // 2)
        x1 = _bf16([x1_w[g, rows, :] for g in range(8)], 1).astype(F32)
        h = _rb2(_ln(x1))
        x_s[_ds(c * TM + j * RB, RB), :] = (x1 + h).astype(BF)
        r = _rb(jnp.sum(h * wr_s[...], axis=1, keepdims=True))
        r = jnp.broadcast_to(r, (RB, 128))
        top, at = top_s[...], at_s[...]
        for i in range(0, RB, 8):
            better = r[i:i + 8] > top
            top = jnp.where(better, r[i:i + 8], top)
            at = jnp.where(better, c * TM + j * RB + i + iota((8, 128), 0), at)
        top_s[...], at_s[...] = top, at
        return r

    P = functools.partial

    def pieces(kind, c, u):
        return [P(proj, kind, c, u, m) for m in (6, 4, 2, 0, 3, 1, 5)]

    def release(y, follow):
        follow = [f.func for f in follow]
        for g in range(8) if post in follow else []:
            x1_w[g, S // 2:] = pltpu.bitcast(y[:8], I32)
        if ln_in in follow or ln_stats in follow:
            x_s[S:, :] = jnp.concatenate([y[:16]] * 8, 1).astype(BF)
        if k_rep in follow:
            kf_s[NHG, 0, 0:8] = y[:8]
        if prep_w in follow:
            wo_s[8, 0:16] = y[:16].astype(BF)

    def stage(t, qkv=True, out=True, load=False):
        make_masks()
        slots = [[] for _ in range(65)]
        nd = 16 if qkv and out else 0
        if load:
            slots[15] += [P(wait, 7), P(start, 8)]
            _spread(slots, [P(prep_w, 3, u, i) for u in range(4) for i in range(4)], 16, 48)
        if qkv and out:
            _spread(slots, [P(ln_in, t + 1, j) for j in range(8)], L0, L1)
        if qkv:
            c = 2 if static(t) else jnp.minimum(t + 2, NC - 1)
            _spread(slots, [P(ln_stats, c, j) for j in range(8)], *((17, 33) if load else (T0, T1)))
            _spread(slots, [P(k_rep, g, t + 1) for g in range(NHG)], K0, K1)
        if out and qkv:
            _spread(slots, [P(post, t - 1, j) for j in range(8)], P0, P1)
        for i in range(4):
            for e in range(2):
                slots[min(16 * i + O0 + O1 * e, 64)].append(P(prep_o, t, i, e))
        fs = [f for u in range(4) for f in pieces(3, t - 1, u)] if out else []
        if qkv:
            _spread(slots, fs, 0, nd)
            fs = [f for kind, u in todo for f in pieces(kind, t + 1, u)]
        _spread(slots, fs[:-E1], nd, 64)
        slots[64] += fs[-E1:]
        quads = [(i + g, 2 * t + b) for i in range(4) for g in (0, 4) for b in range(2)]
        due = {}
        nxt = qk(*quads[0], 0)
        for n, quad in enumerate(quads):
            cur = nxt
            if n + 1 < len(quads):
                nxt = qk(*quads[n + 1], (n + 1) % 2)
            sm, y = [], None
            for h in range(4):
                sm.append(softmax(n % 2, h, cur[h]))
                i = 4 * n + h
                for f in slots[i]:
                    if f.func in (post, ln_in, ln_stats, prep_w, prep_o):
                        due.setdefault(i + LAG, []).append(f())
                    elif f.func is proj:
                        y = f()
                    else:
                        f()
                for e, v in enumerate(due.pop(i, []) if i < 63 else []):
                    s_s[(i + 1) // 4 % 2][4, 1 + e] = v
                if y is not None and i < 63:
                    s_s[(i + 1) // 4 % 2][4, 0, 0:8] = y[:8]
                    release(y, slots[i + 1])
            pv(*quad, n % 2, sm)
        for f in slots[64]:
            f()

    def first_chunk(load):
        def prep(n):
            if n % 2 == 0:
                wait(n // 2 + 1)
                if n != 8:
                    start(min(n // 2 + 3, 7))
            return [P(prep_w, *todo[n], i) for i in range(4)]

        if load:
            start(0)
            start(1)
            setup()
            wait(0)
            for j in range(8):
                ln_stats(0, j)
            start(2)
            for j in range(8):
                ln_in(0, j)
            for f in prep(0):
                f()
        make_masks()
        norm = [P(f, 1, j) for f in (ln_stats, ln_in) for j in range(8)]
        for n, (kind, u) in enumerate(todo):
            side = prep(n + 1) if load and n < 11 else []
            if n >= 4:
                side += [P(k_rep, n - 4, 0), ]
            if n >= 6:
                side += norm[(n - 6) * 3:(n - 5) * 3]
            for f in pieces(kind, 0, u):
                y = f()
                now, side = side[:1 + len(side) // 8], side[1 + len(side) // 8:]
                release(y, now)
                for g in now:
                    g()

    def overlap(main, side, pad, lag):
        due = {}
        for n, f in enumerate(main):
            for e, v in enumerate(due.pop(n, [])):
                pad[e % 2 * 32:e % 2 * 32 + 32] = pltpu.bitcast(v, I32)
            y = f()[:, 0:128]
            release(y, side.get(n, []))
            due[n + lag] = [g() for g in side.get(n, [])]

    def argmax():
        top = jnp.max(top_s[...], axis=0, keepdims=True)
        return top[:, 0:1], jnp.min(jnp.where(top_s[...] == top, at_s[...], S - 1)[:, 0:1])

    def block(row):
        return jnp.concatenate([x1_s[g, _ds(row, 16), :] for g in range(8)], 1).astype(F32)

    def glu(hs, t0, n):
        gate, up = (_rb(_nn(hs, _bf16([w[t0 + i] for i in range(n)], 1))) for w in (wg_w, wu_w))
        return gate, (_rb(gate * jax.nn.sigmoid(gate)) * up).astype(BF)

    def layer(li):
        first, last = li == 0, li == 1
        first_chunk(first)
        top_s[...] = jnp.full((8, 128), -jnp.inf, F32)
        at_s[...] = iota((8, 128), 0)
        stage(0, out=False, load=first)
        if first:
            wait(8)
            start(9)

        def body(t, _):
            stage(t)
            if last:
                for cp in out_copies(_ds((t - 1) * TM, TM)):
                    cp.start()

        lax.fori_loop(1, NC - 1, body, None)
        if first:
            wait(9)
        stage(NC - 1, qkv=False)
        post(NC - 2, 0)
        overlap([f for u in range(4) for f in pieces(3, NC - 1, u)],
                {j * 5 // 2 - 1: [P(post, NC - 2, j)] for j in range(1, 8)}, hb_w.at[7, 0], 7)

        guess = argmax()[1] // 16 * 16
        hs = _ln(block(guess)).astype(BF)
        acts = []
        post(NC - 1, 0)
        post(NC - 1, 1)

        def up(j):
            gate, a = glu(hs, z_s[0] + 4 * j, 4)
            acts.append(a)
            return gate

        def down(j):
            y = _nn(acts[j], _bf16([wd_w[z_s[0] + g, j * 256:(j + 1) * 256] for g in range(8)], 1))
            y_s[...] = y_s[...] + y if j else y
            return y

        overlap([P(up, j) for j in range(7)],
                {j: [P(post, NC - 1, j + 2)] for j in range(6)}, wg_w.at[F // 128], 2)
        rmax, idx = argmax()
        base = (idx // 16) * 16
        blk = _ds(base, 16)
        if last:
            for cp in out_copies(pl.ds(S - 2 * TM, 2 * TM)):
                cp.start()
        side = {}
        if first:
            for j in range(2):
                ln_stats(0, j)
            side = {n: [P(ln_stats, 0, 2 * n + 2 + e) for e in range(2)] for n in range(3)}
            side.update({n: [P(ln_in, 0, j) for j in range(3 * n - 9, min(3 * n - 6, 8))]
                         for n in range(3, 6)})
        overlap([P(down, j) for j in range(7)], side, wd_w.at[8], 4)
        x1 = block(base)
        hs = _ln(x1).astype(BF)

        def redo(j, _):
            a = glu(hs, 2 * j, 2)[1]
            y = _nn(a, _bf16([wd_w[g, _ds(j * 128, 128)] for g in range(8)], 1))
            y_s[...] = jnp.where(j == 0, y, y_s[...] + y)

        lax.fori_loop(0, jnp.where(base == guess, 0, F // 256), redo, None)
        y = _rb(_rb(y_s[...]) * _rb(jax.nn.sigmoid(rmax)))
        upd = jnp.where(iota((16, D), 0) == idx - base, y, 0.0)
        new = (x1 + _rb(hs.astype(F32) + upd)).astype(BF)
        if last:
            for rows in [_ds(c * TM, TM) for c in range(NC - 2)] + [pl.ds(S - 2 * TM, 2 * TM)]:
                for cp in out_copies(rows):
                    cp.wait()
        x_s[blk, :] = new
        if first:
            ln_stats(0, base % TM // RB)
            ln_in(0, base % 128 // 16)
        else:
            for cp in out_copies(blk):
                cp.start()
            for cp in out_copies(blk):
                cp.wait()

    layer(0)
    layer(1)


@jax.jit
def pallas_interleave_layers__sliding_block__moe_arch_mod__prompt_kernel(
    A_x: jax.Array,
    A_wqkv: jax.Array,
    A_wo: jax.Array,
    B_x: jax.Array,
    B_w_r: jax.Array,
    B_w_gate: jax.Array,
    B_w_up: jax.Array,
    B_w_down: jax.Array,
):
    del B_x
    hbm = pl.BlockSpec(memory_space=pl.ANY)
    out = pl.pallas_call(
        _kernel,
        out_shape=jax.ShapeDtypeStruct((S, D), BF),
        in_specs=[pl.BlockSpec(memory_space=pltpu.VMEM)] + [hbm] * 6,
        out_specs=hbm,
        scratch_shapes=[
            pltpu.VMEM((S + 16, D), BF),
            pltpu.VMEM((8, S + 16, 128), BF),
            pltpu.VMEM((7, 4, 128, 128), BF),
            pltpu.VMEM((8, 4, 128, 128), BF),
            pltpu.VMEM((7, 4, 64, 128), I32),
            pltpu.VMEM((NHG, S, 128), BF),
            pltpu.VMEM((3, NHG, D, 128), BF),
            pltpu.VMEM((9, D, 128), BF),
            pltpu.VMEM((F // 128 + 1, D, 128), BF),
            pltpu.VMEM((F // 128, D, 128), BF),
            pltpu.VMEM((9, F, 128), BF),
            pltpu.VMEM((16, 7, 4, 64, 128), I32),
            pltpu.VMEM((4, 128, 128), F32),
            pltpu.VMEM((NQB, NHG, 128, 128), BF),
            pltpu.VMEM((NQB, NHG, 128, 128), BF),
            pltpu.VMEM((NHG + 1, 2, 128, 128), F32),
            pltpu.VMEM((NHG, 67 * 16, 128), I32),
            pltpu.VMEM((32, 64 * 16, 128), I32),
            pltpu.VMEM((5, 9, 32, 128), F32),
            pltpu.VMEM((5, 9, 32, 128), F32),
            pltpu.VMEM((24, 64, 128), I32),
            pltpu.VMEM((2, 64, 128), I32),
            pltpu.VMEM((RB, D), F32),
            pltpu.VMEM((8, 128), F32),
            pltpu.VMEM((8, 128), I32),
            pltpu.VMEM((2, TM, 128), F32),
            pltpu.SMEM((1,), I32),
            pltpu.VMEM((16, D), F32),
            pltpu.SemaphoreType.DMA((11,)),
        ],
        compiler_params=pltpu.CompilerParams(vmem_limit_bytes=110 * 1024 * 1024),
    )(B_w_r, A_x.reshape(S, D), A_wqkv, A_wo, B_w_gate, B_w_up, B_w_down)
    return out.reshape(1, S, D)
```

```python
import functools

import jax
import jax.numpy as jnp
import numpy as np
from jax import lax
import jax.experimental.pallas as pl
import jax.experimental.pallas.tpu as pltpu

S, D, F = 2048, 1024, 3584
NHG = 8
NQB = S // 128
TM = 256
NC = S // TM
RB = TM // 8
Q, K, V, O = range(4)
BF, F32, I32 = jnp.bfloat16, jnp.float32, jnp.int32
NEG = -1e9
VAR = 1

_bf = lambda v: float(np.asarray(v, dtype=jnp.bfloat16).astype(np.float32))
QSCALE = _bf(32 ** -0.5) * float(np.log2(np.e))
EPS = _bf(1e-5)
P = functools.partial


def _rb(x):
    return x.astype(BF).astype(F32)


def _stats(x):
    m = jnp.mean(x, axis=1, keepdims=True)
    xc = x - m
    v = jnp.mean(xc * xc, axis=1, keepdims=True)
    return m, xc, 1.0 / _rb(jnp.sqrt(_rb(_rb(v) + EPS)))


def _ln(x):
    _, xc, inv = _stats(x)
    return xc * inv


def _nt(a, b):
    return lax.dot_general(a, b, (((1,), (1,)), ((), ())), preferred_element_type=F32)


def _nn(a, b):
    return jnp.dot(a, b, preferred_element_type=F32)


def _bf16(words, axis):
    return jnp.concatenate([pltpu.bitcast(w, BF) for w in words], axis)


def _lhs_terms(a11, a12, a21, a22):
    return [a11 + a22, a21 + a22, a11, a22, a11 + a12, a21 - a11, a12 - a22]


def _rhs_terms(b11, b12, b21, b22):
    return [b11 + b22, b11, b12 - b22, b21 - b11, b22, b11 + b12, b21 + b22]


def _static(i):
    return isinstance(i, int)


def _ds(start, size):
    return pl.ds(start if _static(start) else pl.multiple_of(start, size), size)


def _iota(shape, d):
    return lax.broadcasted_iota(I32, shape, d)


def _spread(slots, pieces, lo, hi):
    for i, f in enumerate(pieces):
        slots[lo + i * (hi - lo) // len(pieces)].append(f)


def _kernel(wr_ref, x_hbm, wqkv_hbm, wo_hbm, wg_hbm, wu_hbm, wd_hbm, out_hbm,
            x_s, x1_s, ha_s, hb_s, oa_s, o_s, w_s, wo_s, wg_s, wu_s, wd_s, ws_s, c_s,
            qt_s, vt_s, k_s, kr_s, s0_s, s1_s, e_s, p_s, tri_s, wr_s, st_s,
            z_s, y_s, top_s, at_s, sem):
    ha_w, hb_w, x1_w, o_w, w_w, wo_w, qt_w, vt_w, wg_w, wu_w, wd_w, oa_w, ws_w, k_w, e_w = (
        r.bitcast(I32) for r in (ha_s, hb_s, x1_s, o_s, w_s, wo_s, qt_s, vt_s, wg_s, wu_s, wd_s,
                                 oa_s, ws_s, k_s, e_s))
    s_s = (s0_s, s1_s)
    todo = [(kind, u) for kind in (K, Q, V) for u in range(4)]

    def x_in(lo, hi):
        rows = pl.ds(lo * TM, (hi - lo) * TM)
        return [(x_hbm.at[rows], x_s.at[rows])]

    def w_in(*ns):
        tiles = [(todo[n][0], 2 * todo[n][1] + e) for n in ns for e in range(2)]
        return [(wqkv_hbm.at[:, pl.ds(j * D + g * 128, 128)], w_s.at[j, g]) for j, g in tiles]

    def slabs(src, dst):
        return [(src.at[:, pl.ds(g * 128, 128)], dst.at[g]) for g in range(src.shape[1] // 128)]

    groups = [x_in(0, 1), w_in(0, 1), w_in(2, 3), w_in(4, 5), w_in(6, 7) + x_in(1, 2), w_in(8, 9),
              w_in(10, 11), x_in(2, 3) + slabs(wo_hbm, wo_s), x_in(3, NC),
              slabs(wg_hbm, wg_s) + slabs(wu_hbm, wu_s) + slabs(wd_hbm, wd_s)]

    def start(n):
        for src, dst in groups[n]:
            pltpu.make_async_copy(src, dst, sem.at[n]).start()

    def wait(n):
        for src, dst in groups[n]:
            pltpu.make_async_copy(src, dst, sem.at[n]).wait()

    def out_copy(rows):
        return pltpu.make_async_copy(x_s.at[rows], out_hbm.at[rows], sem.at[len(groups)])

    def zero():
        return z_s[0]

    def hide(c):
        return zero() if _static(c) else 0

    def setup():
        row, col = _iota((64, 128), 0), _iota((64, 128), 1)
        tri = jnp.where(2 * row <= col, 0xFFFF, 0) | jnp.where(2 * row + 1 <= col, -65536, 0)
        tri_s[0], tri_s[1] = ~tri, tri
        wr_s[...] = jnp.broadcast_to(wr_ref[...].astype(F32).reshape(1, D), (RB, D))
        z_s[0] = 0
        k_w[0:NHG, 0:48, :] = jnp.zeros((NHG, 48, 128), I32)

    mk = {}

    def make_masks():
        row, col = _iota((32, 128), 0) + zero(), _iota((32, 128), 1) + zero()
        mk["tri"] = row <= (col & 31)
        mk["grp"] = col >> 5
        mk["odd"], mk["high"] = (col[:16] & 32) != 0, col[:16] >= 64

    def lhs(kind, c):
        if _static(c) and c == (NC - 1 if kind == O else 1):
            return hb_s, hb_w
        return (oa_s, oa_w) if kind == O else (ha_s, ha_w)

    def ln_stats(c, j):
        m, _, inv = _stats(x_s[_ds(zero() + c * TM + j * RB, RB), :].astype(F32))
        inv = jnp.broadcast_to(inv, (RB, 128))
        st_s[0, _ds(j * RB, RB)] = jnp.broadcast_to(m, (RB, 128))
        st_s[1, _ds(j * RB, RB)] = inv
        return inv

    def ln_in(c, j):
        def h(b, i):
            r = b * 128 + j * 16
            x = x_s[_ds(zero() + c * TM + r, 16), i * 128:(i + 1) * 128].astype(F32)
            return (x - st_s[0, _ds(r, 16)]) * st_s[1, _ds(r, 16)]

        for i in range(4):
            terms = _lhs_terms(h(0, i), h(0, i + 4), h(1, i), h(1, i + 4))
            for m, a in enumerate(terms):
                lhs(Q, c)[0][m, i, _ds(j * 16, 16), :] = a.astype(BF)
        return jnp.concatenate(terms[:2], 0)

    def prep_o(c, i, e):
        words = [o_w[g, _ds((2 * c + b) * 64 + e * 32, 32), :] for b in range(2) for g in (i, i + 4)]
        for m, a in enumerate(_lhs_terms(*[pltpu.bitcast(w, BF).astype(F32) for w in words])):
            lhs(O, c)[0][m, i, e * 64:(e + 1) * 64] = a.astype(BF)
        return a[32:]

    def prep_w(kind, u, i):
        src, z = (wo_w, zero()) if kind == O else (w_w.at[kind], 0)
        words = [src[z + 2 * u + n % 2, pl.ds((i + 4 * (n // 2)) * 64, 64), :] for n in range(4)]
        tiles = [pltpu.bitcast(w, BF) for w in words]
        tiles = [(w.T if kind in (Q, V) else w).astype(F32) for w in tiles]
        for m, a in enumerate(_rhs_terms(*tiles)):
            ws_s[kind * 4 + u, m, i] = a.astype(BF)
        return a[96:]

    def emit(kind, c, b, g, y):
        if kind == Q:
            qt_s[2 * c + b, g] = (y * QSCALE).astype(BF)
        elif kind == K:
            k_s[g, pl.ds(_ds((2 * c + b) * 128, 128).start + 96, 128), :] = y.astype(BF)
        elif kind == V:
            vt_s[2 * c + b, g] = y.astype(BF)
        else:
            rows = _ds((2 * c + b) * 128, 128)
            x1_s[g, rows, :] = (x_s[rows, g * 128:(g + 1) * 128].astype(F32) + y).astype(BF)

    def proj(kind, c, u, m):
        a = _bf16([lhs(kind, c)[1][hide(c) + m, i] for i in range(4)], 1)
        w = [ws_w[kind * 4 + u, m, i] for i in range(4)]
        y = _nt(_bf16(w, 1), a) if kind in (Q, V) else _nn(a, _bf16(w, 0))
        if m == 6:
            c_s[0] = y
        elif m == 4:
            c_s[0] -= y
            c_s[1] = y
        elif m == 2:
            emit(kind, c, 0, 2 * u + 1, c_s[1] + y)
            c_s[3] = y
        elif m == 0:
            c_s[0] += y
            c_s[3] += y
        elif m == 3:
            emit(kind, c, 0, 2 * u, c_s[0] + y)
            c_s[2] = y
        elif m == 1:
            emit(kind, c, 1, 2 * u, c_s[2] + y)
            c_s[3] -= y
        else:
            emit(kind, c, 1, 2 * u + 1, c_s[3] + y)
        return y

    def products(kind, c, u):
        return [P(proj, kind, c, u, m) for m in (6, 4, 2, 0, 3, 1, 5)]

    def k_rep(g, c):
        blocks = [k_w[zero() + g, _ds((c * 8 + i) * 16, 16), :] for i in range(11)]
        for j in range(8):
            r = [blocks[j]] + [pltpu.roll(blocks[j + s], 32 * s, 1) for s in (1, 2, 3)]
            y = [jnp.where(mk["odd"], r[(m + 1) % 4], r[m]) for m in range(4)]
            for h in range(4):
                kr_s[g * 4 + h, _ds((c * 8 + j) * 16, 16), :] = jnp.where(
                    mk["high"], y[(2 - h) % 4], y[-h % 4])

    def qk(g, b, slot):
        lo = max(5 - 4 * b, 0) if _static(b) else 0
        order = ([8] if lo else [0, 8]) + list(range(max(lo, 1), 8))
        for h in range(4):
            q = qt_w[b, g, h * 16:(h + 1) * 16, :]
            w = [jnp.where(mk["grp"][:16] == (p - h) % 4, q, 0) for p in range(4)]
            k = [kr_s[g * 4 + h, _ds(hide(b) + (4 * b - 5 + i) * 16, 16), :] for i in order]
            s = _nn(pltpu.bitcast(jnp.concatenate(k, 0), BF), pltpu.bitcast(jnp.concatenate(w, 0), BF))
            s = {i: s[n * 32:(n + 1) * 32] for n, i in enumerate(order)}
            s[0] = jnp.where(mk["tri"], s.pop(8), NEG if lo else s[0])
            for i in range(lo, lo + 3 if lo else 0):
                s[i] = jnp.where(mk["grp"] >= lo + 3 - i, s[i], NEG)
            m = functools.reduce(jnp.maximum, s.values())
            for i, v in s.items():
                s_s[slot][h, i] = v
            s_s[slot][h, 8, 0:8] = jnp.broadcast_to(jnp.max(m, axis=0, keepdims=True), (8, 128))
        return sorted(s)

    def softmax(slot, h, live):
        m = jnp.concatenate([s_s[slot][zero() + h, 8, 0:8]] * 4, 0)
        p = {i: jnp.exp2(s_s[slot][zero() + h, i] - m) for i in live}
        l = jnp.sum(functools.reduce(jnp.add, p.values()), axis=0, keepdims=True)
        none = jnp.zeros((16, 128), I32)
        if VAR == 0:
            u = [pltpu.bitcast(p[i].astype(BF), I32) if i in p else none for i in range(8)]
        else:
            for i in p:
                e_s[h, i] = p[i].astype(BF)
            u = [e_w[(zero() if VAR == 2 else 0) + h, i] if i in p else none for i in range(8)]
        u = [jnp.where(mk["odd"], u[(i - 1) % 8], u[i]) for i in range(8)]
        u = [jnp.where(mk["high"], u[(i - 2) % 8], u[i]) for i in range(8)]
        edge = jnp.concatenate(u[:4], 0)
        n = (slot * 4 + h) * 3
        p_s[n] = edge & tri_s[0]
        p_s[n + 1] = jnp.concatenate(u[4:], 0)
        p_s[n + 2] = edge & tri_s[1]
        return 1.0 / l

    def pv(g, b, slot, sums):
        n = min(b + 1, 3) if _static(b) else 3
        outs = []
        for h, linv in enumerate(sums):
            v = _bf16([vt_w[b - i, g, h * 16:(h + 1) * 16, :] for i in range(n - 1, -1, -1)], 1)
            p = _bf16([p_s[(slot * 4 + h) * 3 + i] for i in range(3 - n, 3)], 0)
            outs.append(_nn(v, p) * linv)
        o_s[g, _ds(b * 128, 128), :] = jnp.concatenate(outs, 0).T.astype(BF)

    def route(c, j):
        rows = _ds(zero() + c * (TM // 2) + j * (RB // 2), RB // 2)
        x1 = _bf16([x1_w[g, rows, :] for g in range(8)], 1).astype(F32)
        h = _rb(_ln(x1))
        x_s[_ds(c * TM + j * RB, RB), :] = (x1 + h).astype(BF)
        r = jnp.broadcast_to(_rb(jnp.sum(h * wr_s[...], axis=1, keepdims=True)), (RB, 128))
        top, at = top_s[...], at_s[...]
        for i in range(0, RB, 8):
            better = r[i:i + 8] > top
            top = jnp.where(better, r[i:i + 8], top)
            at = jnp.where(better, c * TM + j * RB + i + _iota((8, 128), 0), at)
        top_s[...], at_s[...] = top, at
        return r

    def argmax():
        top = jnp.max(top_s[...], axis=0, keepdims=True)
        return top[:, 0:1], jnp.min(jnp.where(top_s[...] == top, at_s[...], S - 1)[:, 0:1])

    def block(row):
        return jnp.concatenate([x1_s[g, _ds(row, 16), :] for g in range(8)], 1).astype(F32)

    def glu(hs, t0, n):
        gate, up = (_rb(_nn(hs, _bf16([w[t0 + i] for i in range(n)], 1))) for w in (wg_w, wu_w))
        return gate, (_rb(gate * jax.nn.sigmoid(gate)) * up).astype(BF)

    def release(y, follow):
        follow = [f.func for f in follow]
        for g in range(8) if route in follow else []:
            x1_w[g, S // 2:] = pltpu.bitcast(y[:8], I32)
        if ln_in in follow or ln_stats in follow:
            x_s[S:, :] = jnp.concatenate([y[:16]] * 8, 1).astype(BF)
        if k_rep in follow:
            k_w[NHG, 0:8] = pltpu.bitcast(y[:8], I32)
        if prep_w in follow:
            wo_s[8, 0:16] = y[:16].astype(BF)

    def overlap(main, side, spare, lag):
        due = {}
        for n, f in enumerate(main):
            for e, v in enumerate(due.pop(n, [])):
                spare[e % 2 * 32:e % 2 * 32 + 32] = pltpu.bitcast(v, I32)
            release(f()[:, 0:128], side.get(n, []))
            due[n + lag] = [g() for g in side.get(n, [])]

    def stage(t, qkv=True, out=True, load=False):
        make_masks()
        slots = [[] for _ in range(65)]
        nd = 16 if qkv and out else 0
        if load:
            slots[15] += [P(wait, 7), P(start, 8)]
            _spread(slots, [P(prep_w, O, u, i) for u in range(4) for i in range(4)], 16, 48)
        if qkv and out:
            _spread(slots, [P(ln_in, t + 1, j) for j in range(8)], 0, 12)
        if qkv:
            c = t + 2 if _static(t) else jnp.minimum(t + 2, NC - 1)
            _spread(slots, [P(ln_stats, c, j) for j in range(8)], *((17, 33) if load else (13, 29)))
            _spread(slots, [P(k_rep, g, t + 1) for g in range(NHG)], 26, 58)
        if qkv and out:
            _spread(slots, [P(route, t - 1, j) for j in range(8)], 28, 60)
        for i in range(4):
            for e in range(2):
                slots[min(16 * i + 19 + 4 * e, 64)].append(P(prep_o, t, i, e))
        fs = [f for u in range(4) for f in products(O, t - 1, u)] if out else []
        if qkv:
            _spread(slots, fs, 0, nd)
            fs = [f for kind, u in todo for f in products(kind, t + 1, u)]
        _spread(slots, fs[:-3], nd, 64)
        slots[64] += fs[-3:]

        quads = [(i + g, 2 * t + b) for i in range(4) for g in (0, 4) for b in range(2)]
        due = {}
        nxt = qk(*quads[0], 0)
        for n, quad in enumerate(quads):
            live = nxt
            if n + 1 < len(quads):
                nxt = qk(*quads[n + 1], (n + 1) % 2)
            sums, y = [], None
            for i in range(4 * n, 4 * n + 4):
                sums.append(softmax(n % 2, i % 4, live))
                for f in slots[i]:
                    if f.func in (route, ln_in, ln_stats, prep_w, prep_o):
                        due.setdefault(i + 2, []).append(f())
                    elif f.func is proj:
                        y = f()
                    else:
                        f()
                scores = s_s[(i + 1) // 4 % 2]
                for e, v in enumerate(due.pop(i, []) if i < 63 else []):
                    scores[4, 1 + e] = v
                if y is not None and i < 63:
                    scores[4, 0, 0:8] = y[:8]
                    release(y, slots[i + 1])
            pv(*quad, n % 2, sums)
        for f in slots[64]:
            f()

    def first_chunk(load):
        def prep(n):
            if n % 2 == 0:
                wait(n // 2 + 1)
                if n != 8:
                    start(min(n // 2 + 3, 7))
            return [P(prep_w, *todo[n], i) for i in range(4)]

        if load:
            start(0)
            start(1)
            setup()
            wait(0)
            for j in range(8):
                ln_stats(0, j)
            start(2)
            for j in range(8):
                ln_in(0, j)
            for f in prep(0):
                f()
        make_masks()
        norm = [P(f, 1, j) for f in (ln_stats, ln_in) for j in range(8)]
        for n, (kind, u) in enumerate(todo):
            side = prep(n + 1) if load and n < 11 else []
            if n >= 4:
                side.append(P(k_rep, n - 4, 0))
            if n >= 6:
                side += norm[(n - 6) * 3:(n - 5) * 3]
            for f in products(kind, 0, u):
                y = f()
                now, side = side[:1 + len(side) // 8], side[1 + len(side) // 8:]
                release(y, now)
                for g in now:
                    g()
            assert not side

    def layer(first):
        first_chunk(first)
        top_s[...] = jnp.full((8, 128), -jnp.inf, F32)
        at_s[...] = _iota((8, 128), 0)
        stage(0, out=False, load=first)
        if first:
            wait(8)
            start(9)

        def body(t, _):
            stage(t)
            if not first:
                out_copy(_ds((t - 1) * TM, TM)).start()

        lax.fori_loop(1, NC - 1, body, None)
        if first:
            wait(9)
        stage(NC - 1, qkv=False)
        route(NC - 2, 0)
        overlap([f for u in range(4) for f in products(O, NC - 1, u)],
                {j * 5 // 2 - 1: [P(route, NC - 2, j)] for j in range(1, 8)}, hb_w.at[7, 0], 7)

        guess = argmax()[1] // 16 * 16
        hs = _ln(block(guess)).astype(BF)
        acts = []
        route(NC - 1, 0)
        route(NC - 1, 1)

        def up(j):
            gate, a = glu(hs, zero() + 4 * j, 4)
            acts.append(a)
            return gate

        def down(j):
            y = _nn(acts[j], _bf16([wd_w[zero() + g, j * 256:(j + 1) * 256] for g in range(8)], 1))
            y_s[...] = y_s[...] + y if j else y
            return y

        overlap([P(up, j) for j in range(7)],
                {j: [P(route, NC - 1, j + 2)] for j in range(6)}, wg_w.at[F // 128], 2)
        rmax, idx = argmax()
        base = idx // 16 * 16
        tail = pl.ds(S - 2 * TM, 2 * TM)
        side = {}
        if first:
            for j in range(2):
                ln_stats(0, j)
            side = {n: [P(ln_stats, 0, 2 * n + 2 + e) for e in range(2)] for n in range(3)}
            side.update({n: [P(ln_in, 0, j) for j in range(3 * n - 9, min(3 * n - 6, 8))]
                         for n in range(3, 6)})
        else:
            out_copy(tail).start()
        overlap([P(down, j) for j in range(7)], side, wd_w.at[8], 4)
        x1 = block(base)
        hs = _ln(x1).astype(BF)

        def redo(j, _):
            a = glu(hs, 2 * j, 2)[1]
            y = _nn(a, _bf16([wd_w[g, _ds(j * 128, 128)] for g in range(8)], 1))
            y_s[...] = jnp.where(j == 0, y, y_s[...] + y)

        lax.fori_loop(0, jnp.where(base == guess, 0, F // 256), redo, None)
        y = _rb(_rb(y_s[...]) * _rb(jax.nn.sigmoid(rmax)))
        upd = jnp.where(_iota((16, D), 0) == idx - base, y, 0.0)
        new = (x1 + _rb(hs.astype(F32) + upd)).astype(BF)
        if first:
            x_s[_ds(base, 16), :] = new
            ln_stats(0, base % TM // RB)
            ln_in(0, base % 128 // 16)
        else:
            for rows in [_ds(c * TM, TM) for c in range(NC - 2)] + [tail]:
                out_copy(rows).wait()
            x_s[_ds(base, 16), :] = new
            out_copy(_ds(base, 16)).start()
            out_copy(_ds(base, 16)).wait()

    layer(True)
    layer(False)


@jax.jit
def pallas_interleave_layers__sliding_block__moe_arch_mod__prompt_kernel(
    A_x: jax.Array,
    A_wqkv: jax.Array,
    A_wo: jax.Array,
    B_x: jax.Array,
    B_w_r: jax.Array,
    B_w_gate: jax.Array,
    B_w_up: jax.Array,
    B_w_down: jax.Array,
):
    del B_x
    hbm = pl.BlockSpec(memory_space=pl.ANY)
    out = pl.pallas_call(
        _kernel,
        out_shape=jax.ShapeDtypeStruct((S, D), BF),
        in_specs=[pl.BlockSpec(memory_space=pltpu.VMEM)] + [hbm] * 6,
        out_specs=hbm,
        scratch_shapes=[
            pltpu.VMEM((S + 16, D), BF),
            pltpu.VMEM((8, S + 16, 128), BF),
            pltpu.VMEM((7, 4, 128, 128), BF),
            pltpu.VMEM((8, 4, 128, 128), BF),
            pltpu.VMEM((7, 4, 128, 128), BF),
            pltpu.VMEM((NHG, S, 128), BF),
            pltpu.VMEM((3, NHG, D, 128), BF),
            pltpu.VMEM((9, D, 128), BF),
            pltpu.VMEM((F // 128 + 1, D, 128), BF),
            pltpu.VMEM((F // 128, D, 128), BF),
            pltpu.VMEM((9, F, 128), BF),
            pltpu.VMEM((16, 7, 4, 128, 128), BF),
            pltpu.VMEM((4, 128, 128), F32),
            pltpu.VMEM((NQB, NHG, 128, 128), BF),
            pltpu.VMEM((NQB, NHG, 128, 128), BF),
            pltpu.VMEM((NHG + 1, 128 + S, 128), BF),
            pltpu.VMEM((32, 64 * 16, 128), I32),
            pltpu.VMEM((5, 9, 32, 128), F32),
            pltpu.VMEM((5, 9, 32, 128), F32),
            pltpu.VMEM((4, 8, 32, 128), BF),
            pltpu.VMEM((24, 64, 128), I32),
            pltpu.VMEM((2, 64, 128), I32),
            pltpu.VMEM((RB, D), F32),
            pltpu.VMEM((2, TM, 128), F32),
            pltpu.SMEM((1,), I32),
            pltpu.VMEM((16, D), F32),
            pltpu.VMEM((8, 128), F32),
            pltpu.VMEM((8, 128), I32),
            pltpu.SemaphoreType.DMA((11,)),
        ],
        compiler_params=pltpu.CompilerParams(vmem_limit_bytes=110 * 1024 * 1024),
    )(B_w_r, A_x.reshape(S, D), A_wqkv, A_wo, B_w_gate, B_w_up, B_w_down)
    return out.reshape(1, S, D)
```

```python
import functools

import jax
import jax.numpy as jnp
import numpy as np
from jax import lax
import jax.experimental.pallas as pl
import jax.experimental.pallas.tpu as pltpu

S, D, F = 2048, 1024, 3584
NHG = 8
NQB = S // 128
TM = 256
NC = S // TM
RB = TM // 8
Q, K, V, O = range(4)
BF, F32, I32 = jnp.bfloat16, jnp.float32, jnp.int32
NEG = -1e9

_bf = lambda v: float(np.asarray(v, dtype=jnp.bfloat16).astype(np.float32))
QSCALE = _bf(32 ** -0.5) * float(np.log2(np.e))
EPS = _bf(1e-5)
P = functools.partial


def _rb(x):
    return x.astype(BF).astype(F32)


def _stats(x):
    m = jnp.mean(x, axis=1, keepdims=True)
    xc = x - m
    v = jnp.mean(xc * xc, axis=1, keepdims=True)
    return m, xc, 1.0 / _rb(jnp.sqrt(_rb(_rb(v) + EPS)))


def _ln(x):
    _, xc, inv = _stats(x)
    return xc * inv


def _nt(a, b):
    return lax.dot_general(a, b, (((1,), (1,)), ((), ())), preferred_element_type=F32)


def _nn(a, b):
    return jnp.dot(a, b, preferred_element_type=F32)


def _bf16(words, axis):
    return jnp.concatenate([pltpu.bitcast(w, BF) for w in words], axis)


def _lhs_terms(a11, a12, a21, a22):
    return [a11 + a22, a21 + a22, a11, a22, a11 + a12, a21 - a11, a12 - a22]


def _rhs_terms(b11, b12, b21, b22):
    return [b11 + b22, b11, b12 - b22, b21 - b11, b22, b11 + b12, b21 + b22]


def _static(i):
    return isinstance(i, int)


def _ds(start, size):
    return pl.ds(start if _static(start) else pl.multiple_of(start, size), size)


def _iota(shape, d):
    return lax.broadcasted_iota(I32, shape, d)


def _spread(slots, pieces, lo, hi):
    for i, f in enumerate(pieces):
        slots[lo + i * (hi - lo) // len(pieces)].append(f)


def _kernel(wr_ref, x_hbm, wqkv_hbm, wo_hbm, wg_hbm, wu_hbm, wd_hbm, out_hbm,
            x_s, x1_s, ha_s, hb_s, oa_s, o_s, w_s, wo_s, wg_s, wu_s, wd_s, ws_s, c_s,
            qt_s, vt_s, k_s, kr_s, s0_s, s1_s, e_s, p_s, tri_s, wr_s, st_s,
            z_s, y_s, top_s, at_s, sem):
    ha_w, hb_w, x1_w, o_w, w_w, wo_w, qt_w, vt_w, wg_w, wu_w, wd_w, oa_w, ws_w, k_w, e_w = (
        r.bitcast(I32) for r in (ha_s, hb_s, x1_s, o_s, w_s, wo_s, qt_s, vt_s, wg_s, wu_s, wd_s,
                                 oa_s, ws_s, k_s, e_s))
    s_s = (s0_s, s1_s)
    todo = [(kind, u) for kind in (K, Q, V) for u in range(4)]

    def x_in(lo, hi):
        rows = pl.ds(lo * TM, (hi - lo) * TM)
        return [(x_hbm.at[rows], x_s.at[rows])]

    def w_in(*ns):
        tiles = [(todo[n][0], 2 * todo[n][1] + e) for n in ns for e in range(2)]
        return [(wqkv_hbm.at[:, pl.ds(j * D + g * 128, 128)], w_s.at[j, g]) for j, g in tiles]

    def slabs(src, dst):
        return [(src.at[:, pl.ds(g * 128, 128)], dst.at[g]) for g in range(src.shape[1] // 128)]

    groups = [x_in(0, 1), w_in(0, 1), w_in(2, 3), w_in(4, 5), w_in(6, 7) + x_in(1, 2), w_in(8, 9),
              w_in(10, 11), x_in(2, 3) + slabs(wo_hbm, wo_s), x_in(3, NC),
              slabs(wg_hbm, wg_s) + slabs(wu_hbm, wu_s) + slabs(wd_hbm, wd_s)]

    def start(n):
        for src, dst in groups[n]:
            pltpu.make_async_copy(src, dst, sem.at[n]).start()

    def wait(n):
        for src, dst in groups[n]:
            pltpu.make_async_copy(src, dst, sem.at[n]).wait()

    def out_copy(rows):
        return pltpu.make_async_copy(x_s.at[rows], out_hbm.at[rows], sem.at[len(groups)])

    def zero():
        return z_s[0]

    def hide(c):
        return zero() if _static(c) else 0

    def setup():
        row, col = _iota((64, 128), 0), _iota((64, 128), 1)
        tri = jnp.where(2 * row <= col, 0xFFFF, 0) | jnp.where(2 * row + 1 <= col, -65536, 0)
        tri_s[0], tri_s[1] = ~tri, tri
        wr_s[...] = jnp.broadcast_to(wr_ref[...].astype(F32).reshape(1, D), (RB, D))
        z_s[0] = 0
        k_w[0:NHG, 0:48, :] = jnp.zeros((NHG, 48, 128), I32)

    mk = {}

    def make_masks():
        row, col = _iota((32, 128), 0) + zero(), _iota((32, 128), 1) + zero()
        mk["tri"] = row <= (col & 31)
        mk["grp"] = col >> 5
        mk["odd"], mk["high"] = (col[:16] & 32) != 0, col[:16] >= 64

    def lhs(kind, c):
        if _static(c) and c == (NC - 1 if kind == O else 1):
            return hb_s, hb_w
        return (oa_s, oa_w) if kind == O else (ha_s, ha_w)

    def ln_stats(c, j):
        m, _, inv = _stats(x_s[_ds(zero() + c * TM + j * RB, RB), :].astype(F32))
        inv = jnp.broadcast_to(inv, (RB, 128))
        st_s[0, _ds(j * RB, RB)] = jnp.broadcast_to(m, (RB, 128))
        st_s[1, _ds(j * RB, RB)] = inv
        return inv

    def ln_in(c, j):
        def h(b, i):
            r = b * 128 + j * 16
            x = x_s[_ds(zero() + c * TM + r, 16), i * 128:(i + 1) * 128].astype(F32)
            return (x - st_s[0, _ds(r, 16)]) * st_s[1, _ds(r, 16)]

        for i in range(4):
            terms = _lhs_terms(h(0, i), h(0, i + 4), h(1, i), h(1, i + 4))
            for m, a in enumerate(terms):
                lhs(Q, c)[0][m, i, _ds(j * 16, 16), :] = a.astype(BF)
        return jnp.concatenate(terms[:2], 0)

    def prep_o(c, i, e):
        words = [o_w[g, _ds((2 * c + b) * 64 + e * 32, 32), :] for b in range(2) for g in (i, i + 4)]
        for m, a in enumerate(_lhs_terms(*[pltpu.bitcast(w, BF).astype(F32) for w in words])):
            lhs(O, c)[0][m, i, e * 64:(e + 1) * 64] = a.astype(BF)
        return a[32:]

    def prep_w(kind, u, i):
        src, z = (wo_w, zero()) if kind == O else (w_w.at[kind], 0)
        words = [src[z + 2 * u + n % 2, pl.ds((i + 4 * (n // 2)) * 64, 64), :] for n in range(4)]
        tiles = [pltpu.bitcast(w, BF) for w in words]
        tiles = [(w.T if kind in (Q, V) else w).astype(F32) for w in tiles]
        for m, a in enumerate(_rhs_terms(*tiles)):
            ws_s[kind * 4 + u, m, i] = a.astype(BF)
        return a[96:]

    def emit(kind, c, b, g, y):
        if kind == Q:
            qt_s[2 * c + b, g] = (y * QSCALE).astype(BF)
        elif kind == K:
            k_s[g, pl.ds(_ds((2 * c + b) * 128, 128).start + 96, 128), :] = y.astype(BF)
        elif kind == V:
            vt_s[2 * c + b, g] = y.astype(BF)
        else:
            rows = _ds((2 * c + b) * 128, 128)
            x1_s[g, rows, :] = (x_s[rows, g * 128:(g + 1) * 128].astype(F32) + y).astype(BF)

    def proj(kind, c, u, m):
        a = _bf16([lhs(kind, c)[1][hide(c) + m, i] for i in range(4)], 1)
        w = [ws_w[kind * 4 + u, m, i] for i in range(4)]
        y = _nt(_bf16(w, 1), a) if kind in (Q, V) else _nn(a, _bf16(w, 0))
        if m == 6:
            c_s[0] = y
        elif m == 4:
            c_s[0] -= y
            c_s[1] = y
        elif m == 2:
            emit(kind, c, 0, 2 * u + 1, c_s[1] + y)
            c_s[3] = y
        elif m == 0:
            c_s[0] += y
            c_s[3] += y
        elif m == 3:
            emit(kind, c, 0, 2 * u, c_s[0] + y)
            c_s[2] = y
        elif m == 1:
            emit(kind, c, 1, 2 * u, c_s[2] + y)
            c_s[3] -= y
        else:
            emit(kind, c, 1, 2 * u + 1, c_s[3] + y)
        return y

    def products(kind, c, u):
        return [P(proj, kind, c, u, m) for m in (6, 4, 2, 0, 3, 1, 5)]

    def k_rep(g, c):
        blocks = [k_w[zero() + g, _ds((c * 8 + i) * 16, 16), :] for i in range(11)]
        for j in range(8):
            r = [blocks[j]] + [pltpu.roll(blocks[j + s], 32 * s, 1) for s in (1, 2, 3)]
            y = [jnp.where(mk["odd"], r[(m + 1) % 4], r[m]) for m in range(4)]
            for h in range(4):
                kr_s[g * 4 + h, _ds((c * 8 + j) * 16, 16), :] = jnp.where(
                    mk["high"], y[(2 - h) % 4], y[-h % 4])

    def qk(g, b, slot):
        lo = max(5 - 4 * b, 0) if _static(b) else 0
        order = ([8] if lo else [0, 8]) + list(range(max(lo, 1), 8))
        for h in range(4):
            q = qt_w[b, g, h * 16:(h + 1) * 16, :]
            w = [jnp.where(mk["grp"][:16] == (p - h) % 4, q, 0) for p in range(4)]
            k = [kr_s[g * 4 + h, _ds(hide(b) + (4 * b - 5 + i) * 16, 16), :] for i in order]
            s = _nn(pltpu.bitcast(jnp.concatenate(k, 0), BF), pltpu.bitcast(jnp.concatenate(w, 0), BF))
            s = {i: s[n * 32:(n + 1) * 32] for n, i in enumerate(order)}
            s[0] = jnp.where(mk["tri"], s.pop(8), NEG if lo else s[0])
            for i in range(lo, lo + 3 if lo else 0):
                s[i] = jnp.where(mk["grp"] >= lo + 3 - i, s[i], NEG)
            m = functools.reduce(jnp.maximum, s.values())
            for i, v in s.items():
                s_s[slot][h, i] = v
            s_s[slot][h, 8, 0:8] = jnp.broadcast_to(jnp.max(m, axis=0, keepdims=True), (8, 128))
        return sorted(s)

    def softmax(slot, h, live):
        m = jnp.concatenate([s_s[slot][zero() + h, 8, 0:8]] * 4, 0)
        p = {i: jnp.exp2(s_s[slot][zero() + h, i] - m) for i in live}
        l = jnp.sum(functools.reduce(jnp.add, p.values()), axis=0, keepdims=True)
        none = jnp.zeros((16, 128), I32)
        for i in p:
            e_s[slot * 4 + h, i] = p[i].astype(BF)
        u = [e_w[slot * 4 + h, i] if i in p else none for i in range(8)]
        u = [jnp.where(mk["odd"], u[(i - 1) % 8], u[i]) for i in range(8)]
        u = [jnp.where(mk["high"], u[(i - 2) % 8], u[i]) for i in range(8)]
        edge = jnp.concatenate(u[:4], 0)
        n = (slot * 4 + h) * 3
        p_s[n] = edge & tri_s[0]
        p_s[n + 1] = jnp.concatenate(u[4:], 0)
        p_s[n + 2] = edge & tri_s[1]
        return 1.0 / l

    def pv(g, b, slot, sums):
        n = min(b + 1, 3) if _static(b) else 3
        outs = []
        for h, linv in enumerate(sums):
            v = _bf16([vt_w[b - i, g, h * 16:(h + 1) * 16, :] for i in range(n - 1, -1, -1)], 1)
            p = _bf16([p_s[(slot * 4 + h) * 3 + i] for i in range(3 - n, 3)], 0)
            outs.append(_nn(v, p) * linv)
        o_s[g, _ds(b * 128, 128), :] = jnp.concatenate(outs, 0).T.astype(BF)

    def route(c, j):
        rows = _ds(zero() + c * (TM // 2) + j * (RB // 2), RB // 2)
        x1 = _bf16([x1_w[g, rows, :] for g in range(8)], 1).astype(F32)
        h = _rb(_ln(x1))
        x_s[_ds(c * TM + j * RB, RB), :] = (x1 + h).astype(BF)
        r = jnp.broadcast_to(_rb(jnp.sum(h * wr_s[...], axis=1, keepdims=True)), (RB, 128))
        top, at = top_s[...], at_s[...]
        for i in range(0, RB, 8):
            better = r[i:i + 8] > top
            top = jnp.where(better, r[i:i + 8], top)
            at = jnp.where(better, c * TM + j * RB + i + _iota((8, 128), 0), at)
        top_s[...], at_s[...] = top, at
        return r

    def argmax():
        top = jnp.max(top_s[...], axis=0, keepdims=True)
        return top[:, 0:1], jnp.min(jnp.where(top_s[...] == top, at_s[...], S - 1)[:, 0:1])

    def block(row):
        return jnp.concatenate([x1_s[g, _ds(row, 16), :] for g in range(8)], 1).astype(F32)

    def glu(hs, t0, n):
        gate, up = (_rb(_nn(hs, _bf16([w[t0 + i] for i in range(n)], 1))) for w in (wg_w, wu_w))
        return gate, (_rb(gate * jax.nn.sigmoid(gate)) * up).astype(BF)

    def release(y, follow):
        follow = [f.func for f in follow]
        for g in range(8) if route in follow else []:
            x1_w[g, S // 2:] = pltpu.bitcast(y[:8], I32)
        if ln_in in follow or ln_stats in follow:
            x_s[S:, :] = jnp.concatenate([y[:16]] * 8, 1).astype(BF)
        if k_rep in follow:
            k_w[NHG, 0:8] = pltpu.bitcast(y[:8], I32)
        if prep_w in follow:
            wo_s[8, 0:16] = y[:16].astype(BF)

    def overlap(main, side, spare, lag):
        due = {}
        for n, f in enumerate(main):
            for e, v in enumerate(due.pop(n, [])):
                spare[e % 2 * 32:e % 2 * 32 + 32] = pltpu.bitcast(v, I32)
            release(f()[:, 0:128], side.get(n, []))
            due[n + lag] = [g() for g in side.get(n, [])]

    def stage(t, qkv=True, out=True, load=False):
        make_masks()
        slots = [[] for _ in range(65)]
        nd = 16 if qkv and out else 0
        if load:
            slots[15] += [P(wait, 7), P(start, 8)]
            _spread(slots, [P(prep_w, O, u, i) for u in range(4) for i in range(4)], 16, 48)
        if qkv and out:
            _spread(slots, [P(ln_in, t + 1, j) for j in range(8)], 0, 12)
        if qkv:
            c = t + 2 if _static(t) else jnp.minimum(t + 2, NC - 1)
            _spread(slots, [P(ln_stats, c, j) for j in range(8)], *((17, 33) if load else (13, 29)))
            _spread(slots, [P(k_rep, g, t + 1) for g in range(NHG)], 29, 61)
        if qkv and out:
            _spread(slots, [P(route, t - 1, j) for j in range(8)], 32, 64)
        for i in range(4):
            for e in range(2):
                slots[min(16 * i + 19 + 4 * e, 64)].append(P(prep_o, t, i, e))
        fs = [f for u in range(4) for f in products(O, t - 1, u)] if out else []
        if qkv:
            _spread(slots, fs, 0, nd)
            fs = [f for kind, u in todo for f in products(kind, t + 1, u)]
        _spread(slots, fs[:-3], nd, 64)
        slots[64] += fs[-3:]

        quads = [(i + g, 2 * t + b) for i in range(4) for g in (0, 4) for b in range(2)]
        due = {}
        nxt = qk(*quads[0], 0)
        for n, quad in enumerate(quads):
            live = nxt
            if n + 1 < len(quads):
                nxt = qk(*quads[n + 1], (n + 1) % 2)
            sums, y = [], None
            for i in range(4 * n, 4 * n + 4):
                sums.append(softmax(n % 2, i % 4, live))
                for f in slots[i]:
                    if f.func in (route, ln_in, ln_stats, prep_w, prep_o):
                        due.setdefault(i + 2, []).append(f())
                    elif f.func is proj:
                        y = f()
                    else:
                        f()
                scores = s_s[(i + 1) // 4 % 2]
                for e, v in enumerate(due.pop(i, []) if i < 63 else []):
                    scores[4, 1 + e] = v
                if y is not None and i < 63:
                    scores[4, 0, 0:8] = y[:8]
                    release(y, slots[i + 1])
            pv(*quad, n % 2, sums)
        for f in slots[64]:
            f()

    def first_chunk(load):
        def prep(n):
            if n % 2 == 0:
                wait(n // 2 + 1)
                if n != 8:
                    start(min(n // 2 + 3, 7))
            return [P(prep_w, *todo[n], i) for i in range(4)]

        if load:
            start(0)
            start(1)
            setup()
            wait(0)
            for j in range(8):
                ln_stats(0, j)
            start(2)
            for j in range(8):
                ln_in(0, j)
            for f in prep(0):
                f()
        make_masks()
        norm = [P(f, 1, j) for f in (ln_stats, ln_in) for j in range(8)]
        for n, (kind, u) in enumerate(todo):
            side = prep(n + 1) if load and n < 11 else []
            if n >= 4:
                side.append(P(k_rep, n - 4, 0))
            if n >= 6:
                side += norm[(n - 6) * 3:(n - 5) * 3]
            for f in products(kind, 0, u):
                y = f()
                now, side = side[:1 + len(side) // 8], side[1 + len(side) // 8:]
                release(y, now)
                for g in now:
                    g()
            assert not side

    def layer(first):
        first_chunk(first)
        top_s[...] = jnp.full((8, 128), -jnp.inf, F32)
        at_s[...] = _iota((8, 128), 0)
        stage(0, out=False, load=first)
        if first:
            wait(8)
            start(9)

        def body(t, _):
            stage(t)
            if not first:
                out_copy(_ds((t - 1) * TM, TM)).start()

        lax.fori_loop(1, NC - 1, body, None)
        if first:
            wait(9)
        stage(NC - 1, qkv=False)
        route(NC - 2, 0)
        overlap([f for u in range(4) for f in products(O, NC - 1, u)],
                {j * 5 // 2 - 1: [P(route, NC - 2, j)] for j in range(1, 8)}, hb_w.at[7, 0], 7)

        guess = argmax()[1] // 16 * 16
        hs = _ln(block(guess)).astype(BF)
        acts = []
        route(NC - 1, 0)
        route(NC - 1, 1)

        def up(j):
            gate, a = glu(hs, zero() + 4 * j, 4)
            acts.append(a)
            return gate

        def down(j):
            y = _nn(acts[j], _bf16([wd_w[zero() + g, j * 256:(j + 1) * 256] for g in range(8)], 1))
            y_s[...] = y_s[...] + y if j else y
            return y

        overlap([P(up, j) for j in range(7)],
                {j: [P(route, NC - 1, j + 2)] for j in range(6)}, wg_w.at[F // 128], 2)
        rmax, idx = argmax()
        base = idx // 16 * 16
        tail = pl.ds(S - 2 * TM, 2 * TM)
        side = {}
        if first:
            for j in range(2):
                ln_stats(0, j)
            side = {n: [P(ln_stats, 0, 2 * n + 2 + e) for e in range(2)] for n in range(3)}
            side.update({n: [P(ln_in, 0, j) for j in range(3 * n - 9, min(3 * n - 6, 8))]
                         for n in range(3, 6)})
        else:
            out_copy(tail).start()
        overlap([P(down, j) for j in range(7)], side, wd_w.at[8], 4)
        x1 = block(base)
        hs = _ln(x1).astype(BF)

        def redo(j, _):
            a = glu(hs, 2 * j, 2)[1]
            y = _nn(a, _bf16([wd_w[g, _ds(j * 128, 128)] for g in range(8)], 1))
            y_s[...] = jnp.where(j == 0, y, y_s[...] + y)

        lax.fori_loop(0, jnp.where(base == guess, 0, F // 256), redo, None)
        y = _rb(_rb(y_s[...]) * _rb(jax.nn.sigmoid(rmax)))
        upd = jnp.where(_iota((16, D), 0) == idx - base, y, 0.0)
        new = (x1 + _rb(hs.astype(F32) + upd)).astype(BF)
        if first:
            x_s[_ds(base, 16), :] = new
            ln_stats(0, base % TM // RB)
            ln_in(0, base % 128 // 16)
        else:
            for rows in [_ds(c * TM, TM) for c in range(NC - 2)] + [tail]:
                out_copy(rows).wait()
            x_s[_ds(base, 16), :] = new
            out_copy(_ds(base, 16)).start()
            out_copy(_ds(base, 16)).wait()

    layer(True)
    layer(False)


@jax.jit
def pallas_interleave_layers__sliding_block__moe_arch_mod__prompt_kernel(
    A_x: jax.Array,
    A_wqkv: jax.Array,
    A_wo: jax.Array,
    B_x: jax.Array,
    B_w_r: jax.Array,
    B_w_gate: jax.Array,
    B_w_up: jax.Array,
    B_w_down: jax.Array,
):
    del B_x
    hbm = pl.BlockSpec(memory_space=pl.ANY)
    out = pl.pallas_call(
        _kernel,
        out_shape=jax.ShapeDtypeStruct((S, D), BF),
        in_specs=[pl.BlockSpec(memory_space=pltpu.VMEM)] + [hbm] * 6,
        out_specs=hbm,
        scratch_shapes=[
            pltpu.VMEM((S + 16, D), BF),
            pltpu.VMEM((8, S + 16, 128), BF),
            pltpu.VMEM((7, 4, 128, 128), BF),
            pltpu.VMEM((8, 4, 128, 128), BF),
            pltpu.VMEM((7, 4, 128, 128), BF),
            pltpu.VMEM((NHG, S, 128), BF),
            pltpu.VMEM((3, NHG, D, 128), BF),
            pltpu.VMEM((9, D, 128), BF),
            pltpu.VMEM((F // 128 + 1, D, 128), BF),
            pltpu.VMEM((F // 128, D, 128), BF),
            pltpu.VMEM((9, F, 128), BF),
            pltpu.VMEM((16, 7, 4, 128, 128), BF),
            pltpu.VMEM((4, 128, 128), F32),
            pltpu.VMEM((NQB, NHG, 128, 128), BF),
            pltpu.VMEM((NQB, NHG, 128, 128), BF),
            pltpu.VMEM((NHG + 1, 128 + S, 128), BF),
            pltpu.VMEM((32, 64 * 16, 128), I32),
            pltpu.VMEM((5, 9, 32, 128), F32),
            pltpu.VMEM((5, 9, 32, 128), F32),
            pltpu.VMEM((8, 8, 32, 128), BF),
            pltpu.VMEM((24, 64, 128), I32),
            pltpu.VMEM((2, 64, 128), I32),
            pltpu.VMEM((RB, D), F32),
            pltpu.VMEM((2, TM, 128), F32),
            pltpu.SMEM((1,), I32),
            pltpu.VMEM((16, D), F32),
            pltpu.VMEM((8, 128), F32),
            pltpu.VMEM((8, 128), I32),
            pltpu.SemaphoreType.DMA((11,)),
        ],
        compiler_params=pltpu.CompilerParams(vmem_limit_bytes=110 * 1024 * 1024),
    )(B_w_r, A_x.reshape(S, D), A_wqkv, A_wo, B_w_gate, B_w_up, B_w_down)
    return out.reshape(1, S, D)
```

```python
import functools

import jax
import jax.numpy as jnp
import numpy as np
from jax import lax
import jax.experimental.pallas as pl
import jax.experimental.pallas.tpu as pltpu

S, D, F = 2048, 1024, 3584
NHG = 8
NQB = S // 128
TM = 256
NC = S // TM
RB = TM // 8
Q, K, V, O = range(4)
BF, F32, I32 = jnp.bfloat16, jnp.float32, jnp.int32
NEG = -1e9

_bf = lambda v: float(np.asarray(v, dtype=jnp.bfloat16).astype(np.float32))
QSCALE = _bf(32 ** -0.5) * float(np.log2(np.e))
EPS = _bf(1e-5)
P = functools.partial


def _rb(x):
    return x.astype(BF).astype(F32)


def _moments(x):
    m = jnp.mean(x, axis=1, keepdims=True)
    xc = x - m
    return m, xc, jnp.mean(xc * xc, axis=1, keepdims=True)


def _inv_std(v):
    return 1.0 / _rb(jnp.sqrt(_rb(_rb(v) + EPS)))


def _ln(x):
    _, xc, v = _moments(x)
    return xc * _inv_std(v)


def _nt(a, b):
    return lax.dot_general(a, b, (((1,), (1,)), ((), ())), preferred_element_type=F32)


def _nn(a, b):
    return jnp.dot(a, b, preferred_element_type=F32)


def _bf16(words, axis):
    return jnp.concatenate([pltpu.bitcast(w, BF) for w in words], axis)


def _lhs_terms(a11, a12, a21, a22):
    return [a11 + a22, a21 + a22, a11, a22, a11 + a12, a21 - a11, a12 - a22]


def _rhs_terms(b11, b12, b21, b22):
    return [b11 + b22, b11, b12 - b22, b21 - b11, b22, b11 + b12, b21 + b22]


def _static(i):
    return isinstance(i, int)


def _ds(start, size):
    return pl.ds(start if _static(start) else pl.multiple_of(start, size), size)


def _iota(shape, d):
    return lax.broadcasted_iota(I32, shape, d)


def _spread(slots, pieces, lo, hi):
    for i, f in enumerate(pieces):
        slots[lo + i * (hi - lo) // len(pieces)].append(f)


def _kernel(wr_ref, x_hbm, wqkv_hbm, wo_hbm, wg_hbm, wu_hbm, wd_hbm, out_hbm,
            x_s, x1_s, ha_s, hb_s, oa_s, o_s, w_s, wo_s, wg_s, wu_s, wd_s, ws_s, c_s,
            qt_s, vt_s, k_s, kr_s, s0_s, s1_s, e_s, p_s, tri_s, wr_s, st_s,
            z_s, y_s, top_s, at_s, sem):
    ha_w, hb_w, x1_w, o_w, w_w, wo_w, qt_w, vt_w, wg_w, wu_w, wd_w, oa_w, ws_w, k_w, e_w = (
        r.bitcast(I32) for r in (ha_s, hb_s, x1_s, o_s, w_s, wo_s, qt_s, vt_s, wg_s, wu_s, wd_s,
                                 oa_s, ws_s, k_s, e_s))
    s_s = (s0_s, s1_s)
    todo = [(kind, u) for kind in (K, Q, V) for u in range(4)]

    def x_in(lo, hi):
        rows = pl.ds(lo * TM, (hi - lo) * TM)
        return [(x_hbm.at[rows], x_s.at[rows])]

    def w_in(*ns):
        tiles = [(todo[n][0], 2 * todo[n][1] + e) for n in ns for e in range(2)]
        return [(wqkv_hbm.at[:, pl.ds(j * D + g * 128, 128)], w_s.at[j, g]) for j, g in tiles]

    def slabs(src, dst):
        return [(src.at[:, pl.ds(g * 128, 128)], dst.at[g]) for g in range(src.shape[1] // 128)]

    groups = [x_in(0, 1), w_in(0, 1), w_in(2, 3), w_in(4, 5), w_in(6, 7) + x_in(1, 2), w_in(8, 9),
              w_in(10, 11), x_in(2, 3) + slabs(wo_hbm, wo_s), x_in(3, NC),
              slabs(wg_hbm, wg_s) + slabs(wu_hbm, wu_s) + slabs(wd_hbm, wd_s)]

    def start(n):
        for src, dst in groups[n]:
            pltpu.make_async_copy(src, dst, sem.at[n]).start()

    def wait(n):
        for src, dst in groups[n]:
            pltpu.make_async_copy(src, dst, sem.at[n]).wait()

    def out_copy(rows):
        return pltpu.make_async_copy(x_s.at[rows], out_hbm.at[rows], sem.at[len(groups)])

    def zero():
        return z_s[0]

    def hide(c):
        return zero() if _static(c) else 0

    def setup():
        row, col = _iota((64, 128), 0), _iota((64, 128), 1)
        tri = jnp.where(2 * row <= col, 0xFFFF, 0) | jnp.where(2 * row + 1 <= col, -65536, 0)
        tri_s[0], tri_s[1] = ~tri, tri
        wr_s[...] = jnp.broadcast_to(wr_ref[...].astype(F32).reshape(1, D), (RB, D))
        z_s[0] = 0
        k_w[0:NHG, 0:48, :] = jnp.zeros((NHG, 48, 128), I32)

    mk = {}

    def make_masks():
        row, col = _iota((32, 128), 0) + zero(), _iota((32, 128), 1) + zero()
        mk["tri"] = row <= (col & 31)
        mk["grp"] = col >> 5
        mk["odd"], mk["high"] = (col[:16] & 32) != 0, col[:16] >= 64

    def lhs(kind, c):
        if _static(c) and c == (NC - 1 if kind == O else 1):
            return hb_s, hb_w
        return (oa_s, oa_w) if kind == O else (ha_s, ha_w)

    def ln_stats(c, j):
        m, _, v = _moments(x_s[_ds(zero() + c * TM + j * RB, RB), :].astype(F32))
        st_s[0, _ds(j * RB, RB)] = jnp.broadcast_to(m, (RB, 128))
        v = jnp.broadcast_to(v, (RB, 128))
        if _static(j):
            st_s[2, 0:RB] = jnp.where(_iota((RB, 128), 1) == j, v, st_s[2, 0:RB]) if j else v
        else:
            st_s[1, _ds(j * RB, RB)] = _inv_std(v)
        return v

    def ln_scales():
        inv = _inv_std(st_s[2, 0:RB])
        for j in range(8):
            st_s[1, j * RB:(j + 1) * RB] = jnp.broadcast_to(inv[:, j:j + 1], (RB, 128))
        return inv

    def stats(c):
        return [P(ln_stats, c, j) for j in range(8)] + [P(ln_scales)]

    def ln_in(c, j):
        def h(b, i):
            r = b * 128 + j * 16
            x = x_s[_ds(zero() + c * TM + r, 16), i * 128:(i + 1) * 128].astype(F32)
            return (x - st_s[0, _ds(r, 16)]) * st_s[1, _ds(r, 16)]

        for i in range(4):
            terms = _lhs_terms(h(0, i), h(0, i + 4), h(1, i), h(1, i + 4))
            for m, a in enumerate(terms):
                lhs(Q, c)[0][m, i, _ds(j * 16, 16), :] = a.astype(BF)
        return jnp.concatenate(terms[:2], 0)

    def prep_o(c, i, e):
        words = [o_w[g, _ds((2 * c + b) * 64 + e * 32, 32), :] for b in range(2) for g in (i, i + 4)]
        for m, a in enumerate(_lhs_terms(*[pltpu.bitcast(w, BF).astype(F32) for w in words])):
            lhs(O, c)[0][m, i, e * 64:(e + 1) * 64] = a.astype(BF)
        return a[32:]

    def prep_w(kind, u, i):
        src, z = (wo_w, zero()) if kind == O else (w_w.at[kind], 0)
        words = [src[z + 2 * u + n % 2, pl.ds((i + 4 * (n // 2)) * 64, 64), :] for n in range(4)]
        tiles = [pltpu.bitcast(w, BF) for w in words]
        tiles = [(w.T if kind in (Q, V) else w).astype(F32) for w in tiles]
        for m, a in enumerate(_rhs_terms(*tiles)):
            ws_s[kind * 4 + u, m, i] = a.astype(BF)
        return a[96:]

    def emit(kind, c, b, g, y):
        if kind == Q:
            qt_s[2 * c + b, g] = (y * QSCALE).astype(BF)
        elif kind == K:
            k_s[g, pl.ds(_ds((2 * c + b) * 128, 128).start + 96, 128), :] = y.astype(BF)
        elif kind == V:
            vt_s[2 * c + b, g] = y.astype(BF)
        else:
            rows = _ds((2 * c + b) * 128, 128)
            x1_s[g, rows, :] = (x_s[rows, g * 128:(g + 1) * 128].astype(F32) + y).astype(BF)

    def proj(kind, c, u, m):
        a = _bf16([lhs(kind, c)[1][hide(c) + m, i] for i in range(4)], 1)
        w = [ws_w[kind * 4 + u, m, i] for i in range(4)]
        y = _nt(_bf16(w, 1), a) if kind in (Q, V) else _nn(a, _bf16(w, 0))
        if m == 6:
            c_s[0] = y
        elif m == 4:
            c_s[0] -= y
            c_s[1] = y
        elif m == 2:
            emit(kind, c, 0, 2 * u + 1, c_s[1] + y)
            c_s[3] = y
        elif m == 0:
            c_s[0] += y
            c_s[3] += y
        elif m == 3:
            emit(kind, c, 0, 2 * u, c_s[0] + y)
            c_s[2] = y
        elif m == 1:
            emit(kind, c, 1, 2 * u, c_s[2] + y)
            c_s[3] -= y
        else:
            emit(kind, c, 1, 2 * u + 1, c_s[3] + y)
        return y

    def products(kind, c, u):
        return [P(proj, kind, c, u, m) for m in (6, 4, 2, 0, 3, 1, 5)]

    def k_rep(g, c):
        blocks = [k_w[zero() + g, _ds((c * 8 + i) * 16, 16), :] for i in range(11)]
        for j in range(8):
            r = [blocks[j]] + [pltpu.roll(blocks[j + s], 32 * s, 1) for s in (1, 2, 3)]
            y = [jnp.where(mk["odd"], r[(m + 1) % 4], r[m]) for m in range(4)]
            for h in range(4):
                kr_s[g * 4 + h, _ds((c * 8 + j) * 16, 16), :] = jnp.where(
                    mk["high"], y[(2 - h) % 4], y[-h % 4])

    def qk(g, b, slot):
        lo = max(5 - 4 * b, 0) if _static(b) else 0
        order = ([8] if lo else [0, 8]) + list(range(max(lo, 1), 8))
        for h in range(4):
            q = qt_w[b, g, h * 16:(h + 1) * 16, :]
            w = [jnp.where(mk["grp"][:16] == (p - h) % 4, q, 0) for p in range(4)]
            k = [kr_s[g * 4 + h, _ds(hide(b) + (4 * b - 5 + i) * 16, 16), :] for i in order]
            s = _nn(pltpu.bitcast(jnp.concatenate(k, 0), BF), pltpu.bitcast(jnp.concatenate(w, 0), BF))
            s = {i: s[n * 32:(n + 1) * 32] for n, i in enumerate(order)}
            s[0] = jnp.where(mk["tri"], s.pop(8), NEG if lo else s[0])
            for i in range(lo, lo + 3 if lo else 0):
                s[i] = jnp.where(mk["grp"] >= lo + 3 - i, s[i], NEG)
            m = functools.reduce(jnp.maximum, s.values())
            for i, v in s.items():
                s_s[slot][h, i] = v
            s_s[slot][h, 8, 0:8] = jnp.broadcast_to(jnp.max(m, axis=0, keepdims=True), (8, 128))
        return sorted(s)

    def softmax(slot, h, live):
        m = jnp.concatenate([s_s[slot][zero() + h, 8, 0:8]] * 4, 0)
        p = {i: jnp.exp2(s_s[slot][zero() + h, i] - m) for i in live}
        l = jnp.sum(functools.reduce(jnp.add, p.values()), axis=0, keepdims=True)
        none = jnp.zeros((16, 128), I32)
        for i in p:
            e_s[slot * 4 + h, i] = p[i].astype(BF)
        u = [e_w[slot * 4 + h, i] if i in p else none for i in range(8)]
        u = [jnp.where(mk["odd"], u[(i - 1) % 8], u[i]) for i in range(8)]
        u = [jnp.where(mk["high"], u[(i - 2) % 8], u[i]) for i in range(8)]
        edge = jnp.concatenate(u[:4], 0)
        n = (slot * 4 + h) * 3
        p_s[n] = edge & tri_s[0]
        p_s[n + 1] = jnp.concatenate(u[4:], 0)
        p_s[n + 2] = edge & tri_s[1]
        return 1.0 / l

    def pv(g, b, slot, sums):
        n = min(b + 1, 3) if _static(b) else 3
        outs = []
        for h, linv in enumerate(sums):
            v = _bf16([vt_w[b - i, g, h * 16:(h + 1) * 16, :] for i in range(n - 1, -1, -1)], 1)
            p = _bf16([p_s[(slot * 4 + h) * 3 + i] for i in range(3 - n, 3)], 0)
            outs.append(_nn(v, p) * linv)
        o_s[g, _ds(b * 128, 128), :] = jnp.concatenate(outs, 0).T.astype(BF)

    def route(c, j):
        rows = _ds(zero() + c * (TM // 2) + j * (RB // 2), RB // 2)
        x1 = _bf16([x1_w[g, rows, :] for g in range(8)], 1).astype(F32)
        h = _rb(_ln(x1))
        x_s[_ds(c * TM + j * RB, RB), :] = (x1 + h).astype(BF)
        r = jnp.broadcast_to(_rb(jnp.sum(h * wr_s[...], axis=1, keepdims=True)), (RB, 128))
        top, at = top_s[...], at_s[...]
        for i in range(0, RB, 8):
            better = r[i:i + 8] > top
            top = jnp.where(better, r[i:i + 8], top)
            at = jnp.where(better, c * TM + j * RB + i + _iota((8, 128), 0), at)
        top_s[...], at_s[...] = top, at
        return r

    def argmax():
        top = jnp.max(top_s[...], axis=0, keepdims=True)
        return top[:, 0:1], jnp.min(jnp.where(top_s[...] == top, at_s[...], S - 1)[:, 0:1])

    def block(row):
        return jnp.concatenate([x1_s[g, _ds(row, 16), :] for g in range(8)], 1).astype(F32)

    def glu(hs, t0, n):
        gate, up = (_rb(_nn(hs, _bf16([w[t0 + i] for i in range(n)], 1))) for w in (wg_w, wu_w))
        return gate, (_rb(gate * jax.nn.sigmoid(gate)) * up).astype(BF)

    def release(y, follow):
        follow = [f.func for f in follow]
        for g in range(8) if route in follow else []:
            x1_w[g, S // 2:] = pltpu.bitcast(y[:8], I32)
        if ln_in in follow or ln_stats in follow:
            x_s[S:, :] = jnp.concatenate([y[:16]] * 8, 1).astype(BF)
        if k_rep in follow:
            k_w[NHG, 0:8] = pltpu.bitcast(y[:8], I32)
        if prep_w in follow:
            wo_s[8, 0:16] = y[:16].astype(BF)

    def overlap(main, side, spare, lag):
        due = {}
        for n, f in enumerate(main):
            for e, v in enumerate(due.pop(n, [])):
                spare[e % 2 * 32:e % 2 * 32 + 32] = pltpu.bitcast(v, I32)
            release(f()[:, 0:128], side.get(n, []))
            due[n + lag] = [g() for g in side.get(n, [])]

    def stage(t, qkv=True, out=True, load=False):
        make_masks()
        slots = [[] for _ in range(65)]
        nd = 16 if qkv and out else 0
        if load:
            slots[15] += [P(wait, 7), P(start, 8)]
            _spread(slots, [P(prep_w, O, u, i) for u in range(4) for i in range(4)], 16, 48)
        if qkv and out:
            _spread(slots, [P(ln_in, t + 1, j) for j in range(8)], 0, 12)
        if qkv:
            c = t + 2 if _static(t) else jnp.minimum(t + 2, NC - 1)
            _spread(slots, stats(c), *((17, 35) if load else (13, 31)))
            _spread(slots, [P(k_rep, g, t + 1) for g in range(NHG)], 29, 61)
        if qkv and out:
            _spread(slots, [P(route, t - 1, j) for j in range(8)], 32, 64)
        for i in range(4):
            for e in range(2):
                slots[min(16 * i + 19 + 4 * e, 64)].append(P(prep_o, t, i, e))
        fs = [f for u in range(4) for f in products(O, t - 1, u)] if out else []
        if qkv:
            _spread(slots, fs, 0, nd)
            fs = [f for kind, u in todo for f in products(kind, t + 1, u)]
        _spread(slots, fs[:-3], nd, 64)
        slots[64] += fs[-3:]

        quads = [(i + g, 2 * t + b) for i in range(4) for g in (0, 4) for b in range(2)]
        due = {}
        nxt = qk(*quads[0], 0)
        for n, quad in enumerate(quads):
            live = nxt
            if n + 1 < len(quads):
                nxt = qk(*quads[n + 1], (n + 1) % 2)
            sums, y = [], None
            for i in range(4 * n, 4 * n + 4):
                sums.append(softmax(n % 2, i % 4, live))
                for f in slots[i]:
                    if f.func in (route, ln_in, ln_stats, ln_scales, prep_w, prep_o):
                        due.setdefault(i + 2, []).append(f())
                    elif f.func is proj:
                        y = f()
                    else:
                        f()
                scores = s_s[(i + 1) // 4 % 2]
                for e, v in enumerate(due.pop(i, []) if i < 63 else []):
                    scores[4, 1 + e] = v
                if y is not None and i < 63:
                    scores[4, 0, 0:8] = y[:8]
                    release(y, slots[i + 1])
            pv(*quad, n % 2, sums)
        for f in slots[64]:
            f()

    def first_chunk(load):
        def prep(n):
            if n % 2 == 0:
                wait(n // 2 + 1)
                if n != 8:
                    start(min(n // 2 + 3, 7))
            return [P(prep_w, *todo[n], i) for i in range(4)]

        if load:
            start(0)
            start(1)
            setup()
            wait(0)
            for f in stats(0):
                f()
            start(2)
            for j in range(8):
                ln_in(0, j)
            for f in prep(0):
                f()
        make_masks()
        norm = stats(1) + [P(ln_in, 1, j) for j in range(8)]
        for n, (kind, u) in enumerate(todo):
            side = prep(n + 1) if load and n < 11 else []
            if n >= 4:
                side.append(P(k_rep, n - 4, 0))
            if n >= 6:
                side += norm[(n - 6) * 3:(n - 5) * 3]
            for f in products(kind, 0, u):
                y = f()
                now, side = side[:1 + len(side) // 8], side[1 + len(side) // 8:]
                release(y, now)
                for g in now:
                    g()
            assert not side

    def layer(first):
        first_chunk(first)
        top_s[...] = jnp.full((8, 128), -jnp.inf, F32)
        at_s[...] = _iota((8, 128), 0)
        stage(0, out=False, load=first)
        if first:
            wait(8)
            start(9)

        def body(t, _):
            stage(t)
            if not first:
                out_copy(_ds((t - 1) * TM, TM)).start()

        lax.fori_loop(1, NC - 1, body, None)
        if first:
            wait(9)
        stage(NC - 1, qkv=False)
        route(NC - 2, 0)
        overlap([f for u in range(4) for f in products(O, NC - 1, u)],
                {j * 5 // 2 - 1: [P(route, NC - 2, j)] for j in range(1, 8)}, hb_w.at[7, 0], 7)

        guess = argmax()[1] // 16 * 16
        hs = _ln(block(guess)).astype(BF)
        acts = []
        route(NC - 1, 0)
        route(NC - 1, 1)

        def up(j):
            gate, a = glu(hs, zero() + 4 * j, 4)
            acts.append(a)
            return gate

        def down(j):
            y = _nn(acts[j], _bf16([wd_w[zero() + g, j * 256:(j + 1) * 256] for g in range(8)], 1))
            y_s[...] = y_s[...] + y if j else y
            return y

        overlap([P(up, j) for j in range(7)],
                {j: [P(route, NC - 1, j + 2)] for j in range(6)}, wg_w.at[F // 128], 2)
        rmax, idx = argmax()
        base = idx // 16 * 16
        tail = pl.ds(S - 2 * TM, 2 * TM)
        side = {}
        if first:
            norm = stats(0) + [P(ln_in, 0, j) for j in range(8)]
            for f in norm[:3]:
                f()
            side = {n: norm[3 * n + 3:3 * n + 6] for n in range(5)}
        else:
            out_copy(tail).start()
        overlap([P(down, j) for j in range(7)], side, wd_w.at[8], 4)
        x1 = block(base)
        hs = _ln(x1).astype(BF)

        def redo(j, _):
            a = glu(hs, 2 * j, 2)[1]
            y = _nn(a, _bf16([wd_w[g, _ds(j * 128, 128)] for g in range(8)], 1))
            y_s[...] = jnp.where(j == 0, y, y_s[...] + y)

        lax.fori_loop(0, jnp.where(base == guess, 0, F // 256), redo, None)
        y = _rb(_rb(y_s[...]) * _rb(jax.nn.sigmoid(rmax)))
        upd = jnp.where(_iota((16, D), 0) == idx - base, y, 0.0)
        new = (x1 + _rb(hs.astype(F32) + upd)).astype(BF)
        if first:
            x_s[_ds(base, 16), :] = new
            ln_stats(0, base % TM // RB)
            ln_in(0, base % 128 // 16)
        else:
            for rows in [_ds(c * TM, TM) for c in range(NC - 2)] + [tail]:
                out_copy(rows).wait()
            x_s[_ds(base, 16), :] = new
            out_copy(_ds(base, 16)).start()
            out_copy(_ds(base, 16)).wait()

    layer(True)
    layer(False)


@jax.jit
def pallas_interleave_layers__sliding_block__moe_arch_mod__prompt_kernel(
    A_x: jax.Array,
    A_wqkv: jax.Array,
    A_wo: jax.Array,
    B_x: jax.Array,
    B_w_r: jax.Array,
    B_w_gate: jax.Array,
    B_w_up: jax.Array,
    B_w_down: jax.Array,
):
    del B_x
    hbm = pl.BlockSpec(memory_space=pl.ANY)
    out = pl.pallas_call(
        _kernel,
        out_shape=jax.ShapeDtypeStruct((S, D), BF),
        in_specs=[pl.BlockSpec(memory_space=pltpu.VMEM)] + [hbm] * 6,
        out_specs=hbm,
        scratch_shapes=[
            pltpu.VMEM((S + 16, D), BF),
            pltpu.VMEM((8, S + 16, 128), BF),
            pltpu.VMEM((7, 4, 128, 128), BF),
            pltpu.VMEM((8, 4, 128, 128), BF),
            pltpu.VMEM((7, 4, 128, 128), BF),
            pltpu.VMEM((NHG, S, 128), BF),
            pltpu.VMEM((3, NHG, D, 128), BF),
            pltpu.VMEM((9, D, 128), BF),
            pltpu.VMEM((F // 128 + 1, D, 128), BF),
            pltpu.VMEM((F // 128, D, 128), BF),
            pltpu.VMEM((9, F, 128), BF),
            pltpu.VMEM((16, 7, 4, 128, 128), BF),
            pltpu.VMEM((4, 128, 128), F32),
            pltpu.VMEM((NQB, NHG, 128, 128), BF),
            pltpu.VMEM((NQB, NHG, 128, 128), BF),
            pltpu.VMEM((NHG + 1, 128 + S, 128), BF),
            pltpu.VMEM((32, 64 * 16, 128), I32),
            pltpu.VMEM((5, 9, 32, 128), F32),
            pltpu.VMEM((5, 9, 32, 128), F32),
            pltpu.VMEM((8, 8, 32, 128), BF),
            pltpu.VMEM((24, 64, 128), I32),
            pltpu.VMEM((2, 64, 128), I32),
            pltpu.VMEM((RB, D), F32),
            pltpu.VMEM((3, TM, 128), F32),
            pltpu.SMEM((1,), I32),
            pltpu.VMEM((16, D), F32),
            pltpu.VMEM((8, 128), F32),
            pltpu.VMEM((8, 128), I32),
            pltpu.SemaphoreType.DMA((11,)),
        ],
        compiler_params=pltpu.CompilerParams(vmem_limit_bytes=110 * 1024 * 1024),
    )(B_w_r, A_x.reshape(S, D), A_wqkv, A_wo, B_w_gate, B_w_up, B_w_down)
    return out.reshape(1, S, D)
```

```python
import functools

import jax
import jax.numpy as jnp
import numpy as np
from jax import lax
import jax.experimental.pallas as pl
import jax.experimental.pallas.tpu as pltpu

S, D, F = 2048, 1024, 3584
NHG = 8
NQB = S // 128
TM = 256
NC = S // TM
RB = TM // 8
Q, K, V, O = range(4)
BF, F32, I32 = jnp.bfloat16, jnp.float32, jnp.int32
NEG = -1e9

_bf = lambda v: float(np.asarray(v, dtype=jnp.bfloat16).astype(np.float32))
QSCALE = _bf(32 ** -0.5) * float(np.log2(np.e))
EPS = _bf(1e-5)
P = functools.partial


def _rb(x):
    return x.astype(BF).astype(F32)


def _moments(x):
    m = jnp.mean(x, axis=1, keepdims=True)
    xc = x - m
    return m, xc, jnp.mean(xc * xc, axis=1, keepdims=True)


def _inv_std(v):
    return 1.0 / _rb(jnp.sqrt(_rb(_rb(v) + EPS)))


def _ln(x):
    _, xc, v = _moments(x)
    return xc * _inv_std(v)


def _nt(a, b):
    return lax.dot_general(a, b, (((1,), (1,)), ((), ())), preferred_element_type=F32)


def _nn(a, b):
    return jnp.dot(a, b, preferred_element_type=F32)


def _bf16(words, axis):
    return jnp.concatenate([pltpu.bitcast(w, BF) for w in words], axis)


def _lhs_terms(a11, a12, a21, a22):
    return [a11 + a22, a21 + a22, a11, a22, a11 + a12, a21 - a11, a12 - a22]


def _rhs_terms(b11, b12, b21, b22):
    return [b11 + b22, b11, b12 - b22, b21 - b11, b22, b11 + b12, b21 + b22]


def _static(i):
    return isinstance(i, int)


def _ds(start, size):
    return pl.ds(start if _static(start) else pl.multiple_of(start, size), size)


def _iota(shape, d):
    return lax.broadcasted_iota(I32, shape, d)


def _spread(slots, pieces, lo, hi):
    for i, f in enumerate(pieces):
        slots[lo + i * (hi - lo) // len(pieces)].append(f)


def _kernel(wr_ref, x_hbm, wqkv_hbm, wo_hbm, wg_hbm, wu_hbm, wd_hbm, out_hbm,
            x_s, x1_s, ha_s, hb_s, oa_s, o_s, w_s, wo_s, wg_s, wu_s, wd_s, ws_s, c_s,
            qt_s, vt_s, k_s, kr_s, s0_s, s1_s, e_s, p_s, tri_s, wr_s, st_s,
            z_s, y_s, top_s, at_s, sem):
    ha_w, hb_w, x1_w, o_w, w_w, wo_w, qt_w, vt_w, wg_w, wu_w, wd_w, oa_w, ws_w, k_w, e_w = (
        r.bitcast(I32) for r in (ha_s, hb_s, x1_s, o_s, w_s, wo_s, qt_s, vt_s, wg_s, wu_s, wd_s,
                                 oa_s, ws_s, k_s, e_s))
    s_s = (s0_s, s1_s)
    todo = [(kind, u) for kind in (K, Q, V) for u in range(4)]

    def x_in(lo, hi):
        rows = pl.ds(lo * TM, (hi - lo) * TM)
        return [(x_hbm.at[rows], x_s.at[rows])]

    def w_in(*ns):
        tiles = [(todo[n][0], 2 * todo[n][1] + e) for n in ns for e in range(2)]
        return [(wqkv_hbm.at[:, pl.ds(j * D + g * 128, 128)], w_s.at[j, g]) for j, g in tiles]

    def slabs(src, dst):
        return [(src.at[:, pl.ds(g * 128, 128)], dst.at[g]) for g in range(src.shape[1] // 128)]

    groups = [x_in(0, 1), w_in(0, 1), w_in(2, 3), w_in(4, 5), w_in(6, 7) + x_in(1, 2), w_in(8, 9),
              w_in(10, 11), x_in(2, 3) + slabs(wo_hbm, wo_s), x_in(3, NC),
              slabs(wg_hbm, wg_s) + slabs(wu_hbm, wu_s) + slabs(wd_hbm, wd_s)]

    def start(n):
        for src, dst in groups[n]:
            pltpu.make_async_copy(src, dst, sem.at[n]).start()

    def wait(n):
        for src, dst in groups[n]:
            pltpu.make_async_copy(src, dst, sem.at[n]).wait()

    def out_copy(rows):
        return pltpu.make_async_copy(x_s.at[rows], out_hbm.at[rows], sem.at[len(groups)])

    def zero():
        return z_s[0]

    def hide(c):
        return zero() if _static(c) else 0

    def setup():
        row, col = _iota((64, 128), 0), _iota((64, 128), 1)
        tri = jnp.where(2 * row <= col, 0xFFFF, 0) | jnp.where(2 * row + 1 <= col, -65536, 0)
        tri_s[0], tri_s[1] = ~tri, tri
        wr_s[...] = jnp.broadcast_to(wr_ref[...].astype(F32).reshape(1, D), (RB, D))
        z_s[0] = 0
        k_w[0:NHG, 0:48, :] = jnp.zeros((NHG, 48, 128), I32)

    mk = {}

    def make_masks():
        row, col = _iota((32, 128), 0) + zero(), _iota((32, 128), 1) + zero()
        mk["tri"] = row <= (col & 31)
        mk["grp"] = col >> 5
        mk["odd"], mk["high"] = (col[:16] & 32) != 0, col[:16] >= 64

    def lhs(kind, c):
        if _static(c) and c == (NC - 1 if kind == O else 1):
            return hb_s, hb_w
        return (oa_s, oa_w) if kind == O else (ha_s, ha_w)

    def ln_stats(c, j):
        m, _, v = _moments(x_s[_ds(zero() + c * TM + j * RB, RB), :].astype(F32))
        st_s[0, _ds(j * RB, RB)] = jnp.broadcast_to(m, (RB, 128))
        v = jnp.broadcast_to(v, (RB, 128))
        if _static(j):
            st_s[2, 0:RB] = jnp.where(_iota((RB, 128), 1) == j, v, st_s[2, 0:RB]) if j else v
        else:
            st_s[1, _ds(j * RB, RB)] = _inv_std(v)
        return v

    def ln_scales():
        inv = _inv_std(st_s[2, 0:RB])
        for j in range(8):
            st_s[1, j * RB:(j + 1) * RB] = jnp.broadcast_to(inv[:, j:j + 1], (RB, 128))
        return inv

    def stats(c):
        return [P(ln_stats, c, j) for j in range(8)] + [P(ln_scales)]

    def ln_in(c, j):
        def h(b, i):
            r = b * 128 + j * 16
            x = x_s[_ds(zero() + c * TM + r, 16), i * 128:(i + 1) * 128].astype(F32)
            return (x - st_s[0, _ds(r, 16)]) * st_s[1, _ds(r, 16)]

        for i in range(4):
            terms = _lhs_terms(h(0, i), h(0, i + 4), h(1, i), h(1, i + 4))
            for m, a in enumerate(terms):
                lhs(Q, c)[0][m, i, _ds(j * 16, 16), :] = a.astype(BF)
        return jnp.concatenate(terms[:2], 0)

    def prep_o(c, i, e):
        words = [o_w[g, _ds((2 * c + b) * 64 + e * 32, 32), :] for b in range(2) for g in (i, i + 4)]
        for m, a in enumerate(_lhs_terms(*[pltpu.bitcast(w, BF).astype(F32) for w in words])):
            if m in (2, 3):
                lhs(O, c)[1][m, i, e * 32:(e + 1) * 32] = words[3 * (m - 2)]
            else:
                lhs(O, c)[0][m, i, e * 64:(e + 1) * 64] = a.astype(BF)
        return a[32:]

    def prep_w(kind, u, i):
        src, z = (wo_w, zero()) if kind == O else (w_w.at[kind], 0)
        words = [src[z + 2 * u + n % 2, pl.ds((i + 4 * (n // 2)) * 64, 64), :] for n in range(4)]
        tiles = [pltpu.bitcast(w, BF) for w in words]
        if kind in (Q, V):
            tiles = [w.T for w in tiles]
        for m, a in enumerate(_rhs_terms(*[w.astype(F32) for w in tiles])):
            if m in (1, 4):
                ws_w[kind * 4 + u, m, i] = pltpu.bitcast(tiles[m - 1], I32)
            else:
                ws_s[kind * 4 + u, m, i] = a.astype(BF)
        return a[96:]

    def emit(kind, c, b, g, y):
        if kind == Q:
            qt_s[2 * c + b, g] = (y * QSCALE).astype(BF)
        elif kind == K:
            k_s[g, pl.ds(_ds((2 * c + b) * 128, 128).start + 96, 128), :] = y.astype(BF)
        elif kind == V:
            vt_s[2 * c + b, g] = y.astype(BF)
        else:
            rows = _ds((2 * c + b) * 128, 128)
            x1_s[g, rows, :] = (x_s[rows, g * 128:(g + 1) * 128].astype(F32) + y).astype(BF)

    def proj(kind, c, u, m):
        a = _bf16([lhs(kind, c)[1][hide(c) + m, i] for i in range(4)], 1)
        w = [ws_w[kind * 4 + u, m, i] for i in range(4)]
        y = _nt(_bf16(w, 1), a) if kind in (Q, V) else _nn(a, _bf16(w, 0))
        if m == 6:
            c_s[0] = y
        elif m == 4:
            c_s[0] -= y
            c_s[1] = y
        elif m == 2:
            emit(kind, c, 0, 2 * u + 1, c_s[1] + y)
            c_s[3] = y
        elif m == 0:
            c_s[0] += y
            c_s[3] += y
        elif m == 3:
            emit(kind, c, 0, 2 * u, c_s[0] + y)
            c_s[2] = y
        elif m == 1:
            emit(kind, c, 1, 2 * u, c_s[2] + y)
            c_s[3] -= y
        else:
            emit(kind, c, 1, 2 * u + 1, c_s[3] + y)
        return y

    def products(kind, c, u):
        return [P(proj, kind, c, u, m) for m in (6, 4, 2, 0, 3, 1, 5)]

    def k_rep(g, c):
        blocks = [k_w[zero() + g, _ds((c * 8 + i) * 16, 16), :] for i in range(11)]
        for j in range(8):
            r = [blocks[j]] + [pltpu.roll(blocks[j + s], 32 * s, 1) for s in (1, 2, 3)]
            y = [jnp.where(mk["odd"], r[(m + 1) % 4], r[m]) for m in range(4)]
            for h in range(4):
                kr_s[g * 4 + h, _ds((c * 8 + j) * 16, 16), :] = jnp.where(
                    mk["high"], y[(2 - h) % 4], y[-h % 4])

    def qk(g, b, slot):
        lo = max(5 - 4 * b, 0) if _static(b) else 0
        order = ([8] if lo else [0, 8]) + list(range(max(lo, 1), 8))
        for h in range(4):
            q = qt_w[b, g, h * 16:(h + 1) * 16, :]
            w = [jnp.where(mk["grp"][:16] == (p - h) % 4, q, 0) for p in range(4)]
            k = [kr_s[g * 4 + h, _ds(hide(b) + (4 * b - 5 + i) * 16, 16), :] for i in order]
            s = _nn(pltpu.bitcast(jnp.concatenate(k, 0), BF), pltpu.bitcast(jnp.concatenate(w, 0), BF))
            s = {i: s[n * 32:(n + 1) * 32] for n, i in enumerate(order)}
            s[0] = jnp.where(mk["tri"], s.pop(8), NEG if lo else s[0])
            for i in range(lo, lo + 3 if lo else 0):
                s[i] = jnp.where(mk["grp"] >= lo + 3 - i, s[i], NEG)
            m = functools.reduce(jnp.maximum, s.values())
            for i, v in s.items():
                s_s[slot][h, i] = v
            s_s[slot][h, 8, 0:8] = jnp.broadcast_to(jnp.max(m, axis=0, keepdims=True), (8, 128))
        return sorted(s)

    def softmax(slot, h, live, after):
        m = jnp.concatenate([s_s[slot][zero() + h, 8, 0:8]] * 4, 0)
        l = 0.0
        for n, i in enumerate(live):
            if n // 2 < len(after) and n % 2 == 0:
                s_s[slot][4, 0, 0:8] = after[n // 2]
            p = jnp.exp2(s_s[slot][zero() + h, i] - m)
            e_s[slot * 4 + h, i] = p.astype(BF)
            p = (p[0:8] + p[8:16]) + (p[16:24] + p[24:32])
            l = l + p if n else p
        l = jnp.sum(l, axis=0, keepdims=True)
        none = jnp.zeros((16, 128), I32)
        u = [e_w[slot * 4 + h, i] if i in live else none for i in range(8)]
        u = [jnp.where(mk["odd"], u[(i - 1) % 8], u[i]) for i in range(8)]
        u = [jnp.where(mk["high"], u[(i - 2) % 8], u[i]) for i in range(8)]
        edge = jnp.concatenate(u[:4], 0)
        n = (slot * 4 + h) * 3
        p_s[n] = edge & tri_s[0]
        p_s[n + 1] = jnp.concatenate(u[4:], 0)
        p_s[n + 2] = edge & tri_s[1]
        return 1.0 / l

    def pv(g, b, slot, sums):
        n = min(b + 1, 3) if _static(b) else 3
        outs = []
        for h, linv in enumerate(sums):
            v = _bf16([vt_w[b - i, g, h * 16:(h + 1) * 16, :] for i in range(n - 1, -1, -1)], 1)
            p = _bf16([p_s[(slot * 4 + h) * 3 + i] for i in range(3 - n, 3)], 0)
            outs.append(_nn(v, p) * linv)
        o_s[g, _ds(b * 128, 128), :] = jnp.concatenate(outs, 0).T.astype(BF)

    def route(c, j):
        rows = _ds(zero() + c * (TM // 2) + j * (RB // 2), RB // 2)
        x1 = _bf16([x1_w[g, rows, :] for g in range(8)], 1).astype(F32)
        h = _rb(_ln(x1))
        x_s[_ds(c * TM + j * RB, RB), :] = (x1 + h).astype(BF)
        r = jnp.broadcast_to(_rb(jnp.sum(h * wr_s[...], axis=1, keepdims=True)), (RB, 128))
        top, at = top_s[...], at_s[...]
        for i in range(0, RB, 8):
            better = r[i:i + 8] > top
            top = jnp.where(better, r[i:i + 8], top)
            at = jnp.where(better, c * TM + j * RB + i + _iota((8, 128), 0), at)
        top_s[...], at_s[...] = top, at
        return r

    def argmax():
        top = jnp.max(top_s[...], axis=0, keepdims=True)
        return top[:, 0:1], jnp.min(jnp.where(top_s[...] == top, at_s[...], S - 1)[:, 0:1])

    def block(row):
        return jnp.concatenate([x1_s[g, _ds(row, 16), :] for g in range(8)], 1).astype(F32)

    def glu(hs, t0, n):
        gate, up = (_rb(_nn(hs, _bf16([w[t0 + i] for i in range(n)], 1))) for w in (wg_w, wu_w))
        return gate, (_rb(gate * jax.nn.sigmoid(gate)) * up).astype(BF)

    def release(y, follow):
        follow = [f.func for f in follow]
        for g in range(8) if route in follow else []:
            x1_w[g, S // 2:] = pltpu.bitcast(y[:8], I32)
        if ln_in in follow or ln_stats in follow:
            x_s[S:, :] = jnp.concatenate([y[:16]] * 8, 1).astype(BF)
        if k_rep in follow:
            k_w[NHG, 0:8] = pltpu.bitcast(y[:8], I32)
        if prep_w in follow:
            wo_s[8, 0:16] = y[:16].astype(BF)

    def overlap(main, side, spare, lag):
        due = {}
        for n, f in enumerate(main):
            for e, v in enumerate(due.pop(n, [])):
                spare[e % 2 * 32:e % 2 * 32 + 32] = pltpu.bitcast(v, I32)
            release(f()[:, 0:128], side.get(n, []))
            due[n + lag] = [g() for g in side.get(n, [])]

    def stage(t, qkv=True, out=True, load=False):
        make_masks()
        slots = [[] for _ in range(65)]
        nd = 16 if qkv and out else 0
        if load:
            slots[15] += [P(wait, 7), P(start, 8)]
            _spread(slots, [P(prep_w, O, u, i) for u in range(4) for i in range(4)], 16, 64)
        if qkv and out:
            _spread(slots, [P(ln_in, t + 1, j) for j in range(8)], 0, 12)
        if qkv:
            c = (t + 2) & (NC - 1)
            _spread(slots, stats(c), *((17, 35) if load else (13, 31)))
            _spread(slots, [P(k_rep, g, t + 1) for g in range(NHG)], 29, 61)
        if qkv and out:
            _spread(slots, [P(route, t - 1, j) for j in range(8)], 32, 64)
        for i in range(4):
            for e in range(2):
                slots[min(16 * i + 19 + 4 * e, 64)].append(P(prep_o, t, i, e))
        fs = [f for u in range(4) for f in products(O, t - 1, u)] if out else []
        if qkv:
            _spread(slots, fs, 0, nd)
            fs = [f for kind, u in todo for f in products(kind, t + 1, u)]
        _spread(slots, fs[:-2], nd, 64)
        slots[64] += fs[-2:]

        quads = [(i + g, 2 * t + b) for i in range(4) for g in (0, 4) for b in range(2)]
        due, after = {}, []
        nxt = qk(*quads[0], 0)
        for n, quad in enumerate(quads):
            live = nxt
            if n + 1 < len(quads):
                nxt = qk(*quads[n + 1], (n + 1) % 2)
            sums, y = [], None
            for i in range(4 * n, 4 * n + 4):
                sums.append(softmax(n % 2, i % 4, live, after))
                ys, after = [], []
                for f in slots[i]:
                    if f.func in (route, ln_in, ln_stats, ln_scales, prep_w, prep_o):
                        due.setdefault(i + 2, []).append(f())
                    elif f.func is proj:
                        y = f()
                        ys.append(y)
                    else:
                        f()
                scores = s_s[(i + 1) // 4 % 2]
                for e, v in enumerate(due.pop(i, []) if i < 63 else []):
                    scores[4, 1 + e] = v
                if y is not None and i < 63:
                    if qkv:
                        after = [ys[0][r:r + 8] for r in range(0, 128, 32)]
                    release(y[64:], slots[i + 1])
            pv(*quad, n % 2, sums)
        for f in slots[64]:
            f()

    def first_chunk(load):
        def prep(n):
            if n % 2 == 0:
                wait(n // 2 + 1)
                if n != 8:
                    start(min(n // 2 + 3, 7))
            return [P(prep_w, *todo[n], i) for i in range(4)]

        if load:
            start(0)
            start(1)
            setup()
            wait(0)
            for f in stats(0):
                f()
            start(2)
            for j in range(8):
                ln_in(0, j)
            for f in prep(0):
                f()
        make_masks()
        norm = stats(1) + [P(ln_in, 1, j) for j in range(8)]
        for n, (kind, u) in enumerate(todo):
            side = prep(n + 1) if load and n < 11 else []
            if n >= 4:
                side.append(P(k_rep, n - 4, 0))
            if n >= 6:
                side += norm[(n - 6) * 3:(n - 5) * 3]
            for f in products(kind, 0, u):
                y = f()
                now, side = side[:1 + len(side) // 8], side[1 + len(side) // 8:]
                release(y, now)
                for g in now:
                    g()
            assert not side

    def finish(first):
        route(NC - 2, 0)
        overlap([f for u in range(4) for f in products(O, NC - 1, u)],
                {j * 11 // 4 - 1: [P(route, NC - 2, j)] for j in range(1, 8)}, hb_w.at[7, 0], 6)

        guess = argmax()[1] // 16 * 16
        hs = _ln(block(guess)).astype(BF)
        acts = []
        route(NC - 1, 0)
        route(NC - 1, 1)

        def up(j):
            gate, a = glu(hs, zero() + 4 * j, 4)
            acts.append(a)
            return gate

        def down(j):
            y = _nn(acts[j], _bf16([wd_w[zero() + g, j * 256:(j + 1) * 256] for g in range(8)], 1))
            y_s[...] = y_s[...] + y if j else y
            return y

        overlap([P(up, j) for j in range(7)],
                {j: [P(route, NC - 1, j + 2)] for j in range(6)}, wg_w.at[F // 128], 2)
        rmax, idx = argmax()
        base = idx // 16 * 16
        tail = pl.ds(S - 2 * TM, 2 * TM)
        side = {}
        if first:
            ln_in(0, 0)
            ln_in(0, 1)
            side = {n: [P(ln_in, 0, n + 2)] for n in range(6)}
        else:
            out_copy(tail).start()
        overlap([P(down, j) for j in range(7)], side, wd_w.at[8], 2)
        x1 = block(base)
        hs = _ln(x1).astype(BF)

        def redo(j, _):
            a = glu(hs, 7 * j, 7)[1]
            y = _nn(a, _bf16([wd_w[g, pl.ds(pl.multiple_of(j * 448, 64), 448)] for g in range(8)], 1))
            y_s[...] = jnp.where(j == 0, y, y_s[...] + y)

        lax.fori_loop(0, jnp.where(base == guess, 0, 4), redo, None)
        y = _rb(_rb(y_s[...]) * _rb(jax.nn.sigmoid(rmax)))
        upd = jnp.where(_iota((16, D), 0) == idx - base, y, 0.0)
        new = (x1 + _rb(hs.astype(F32) + upd)).astype(BF)
        if first:
            x_s[_ds(base, 16), :] = new
            ln_stats(0, base % TM // RB)
            ln_in(0, base % 128 // 16)
        else:
            for rows in [_ds(c * TM, TM) for c in range(NC - 2)] + [tail]:
                out_copy(rows).wait()
            x_s[_ds(base, 16), :] = new
            out_copy(_ds(base, 16)).start()
            out_copy(_ds(base, 16)).wait()

    def layer(first):
        first_chunk(first)
        top_s[...] = jnp.full((8, 128), -jnp.inf, F32)
        at_s[...] = _iota((8, 128), 0)
        stage(0, out=False, load=first)
        if first:
            wait(8)
            start(9)

        def body(t, _):
            stage(t)
            if not first:
                out_copy(_ds((t - 1) * TM, TM)).start()

        lax.fori_loop(1, NC - 1, body, None)
        if first:
            wait(9)
        stage(NC - 1, qkv=False)
        finish(first)

    layer(True)
    layer(False)


@jax.jit
def pallas_interleave_layers__sliding_block__moe_arch_mod__prompt_kernel(
    A_x: jax.Array,
    A_wqkv: jax.Array,
    A_wo: jax.Array,
    B_x: jax.Array,
    B_w_r: jax.Array,
    B_w_gate: jax.Array,
    B_w_up: jax.Array,
    B_w_down: jax.Array,
):
    del B_x
    hbm = pl.BlockSpec(memory_space=pl.ANY)
    out = pl.pallas_call(
        _kernel,
        out_shape=jax.ShapeDtypeStruct((S, D), BF),
        in_specs=[pl.BlockSpec(memory_space=pltpu.VMEM)] + [hbm] * 6,
        out_specs=hbm,
        scratch_shapes=[
            pltpu.VMEM((S + 16, D), BF),
            pltpu.VMEM((8, S + 16, 128), BF),
            pltpu.VMEM((7, 4, 128, 128), BF),
            pltpu.VMEM((8, 4, 128, 128), BF),
            pltpu.VMEM((7, 4, 128, 128), BF),
            pltpu.VMEM((NHG, S, 128), BF),
            pltpu.VMEM((3, NHG, D, 128), BF),
            pltpu.VMEM((9, D, 128), BF),
            pltpu.VMEM((F // 128 + 1, D, 128), BF),
            pltpu.VMEM((F // 128, D, 128), BF),
            pltpu.VMEM((9, F, 128), BF),
            pltpu.VMEM((16, 7, 4, 128, 128), BF),
            pltpu.VMEM((4, 128, 128), F32),
            pltpu.VMEM((NQB, NHG, 128, 128), BF),
            pltpu.VMEM((NQB, NHG, 128, 128), BF),
            pltpu.VMEM((NHG + 1, 128 + S, 128), BF),
            pltpu.VMEM((32, 64 * 16, 128), I32),
            pltpu.VMEM((5, 9, 32, 128), F32),
            pltpu.VMEM((5, 9, 32, 128), F32),
            pltpu.VMEM((8, 8, 32, 128), BF),
            pltpu.VMEM((24, 64, 128), I32),
            pltpu.VMEM((2, 64, 128), I32),
            pltpu.VMEM((RB, D), F32),
            pltpu.VMEM((3, TM, 128), F32),
            pltpu.SMEM((1,), I32),
            pltpu.VMEM((16, D), F32),
            pltpu.VMEM((8, 128), F32),
            pltpu.VMEM((8, 128), I32),
            pltpu.SemaphoreType.DMA((11,)),
        ],
        compiler_params=pltpu.CompilerParams(vmem_limit_bytes=110 * 1024 * 1024),
    )(B_w_r, A_x.reshape(S, D), A_wqkv, A_wo, B_w_gate, B_w_up, B_w_down)
    return out.reshape(1, S, D)
```

```python
import functools

import jax
import jax.numpy as jnp
import numpy as np
from jax import lax
import jax.experimental.pallas as pl
import jax.experimental.pallas.tpu as pltpu

S, D, F = 2048, 1024, 3584
NHG = 8
NQB = S // 128
TM = 256
NC = S // TM
RB = TM // 8
Q, K, V, O = range(4)
BF, F32, I32 = jnp.bfloat16, jnp.float32, jnp.int32
NEG = -1e9

_bf = lambda v: float(np.asarray(v, dtype=jnp.bfloat16).astype(np.float32))
QSCALE = _bf(32 ** -0.5) * float(np.log2(np.e))
EPS = _bf(1e-5)
P = functools.partial


def _rb(x):
    return x.astype(BF).astype(F32)


def _moments(x):
    m = jnp.mean(x, axis=1, keepdims=True)
    xc = x - m
    return m, xc, jnp.mean(xc * xc, axis=1, keepdims=True)


def _inv_std(v):
    return 1.0 / _rb(jnp.sqrt(_rb(_rb(v) + EPS)))


def _ln(x):
    _, xc, v = _moments(x)
    return xc * _inv_std(v)


def _nt(a, b):
    return lax.dot_general(a, b, (((1,), (1,)), ((), ())), preferred_element_type=F32)


def _nn(a, b):
    return jnp.dot(a, b, preferred_element_type=F32)


def _bf16(words, axis):
    return jnp.concatenate([pltpu.bitcast(w, BF) for w in words], axis)


def _lhs_terms(a11, a12, a21, a22):
    return [a11 + a22, a21 + a22, a11, a22, a11 + a12, a21 - a11, a12 - a22]


def _rhs_terms(b11, b12, b21, b22):
    return [b11 + b22, b11, b12 - b22, b21 - b11, b22, b11 + b12, b21 + b22]


def _static(i):
    return isinstance(i, int)


def _ds(start, size):
    return pl.ds(start if _static(start) else pl.multiple_of(start, size), size)


def _iota(shape, d):
    return lax.broadcasted_iota(I32, shape, d)


def _spread(slots, pieces, lo, hi):
    for i, f in enumerate(pieces):
        slots[lo + i * (hi - lo) // len(pieces)].append(f)


def _kernel(wr_ref, x_hbm, wqkv_hbm, wo_hbm, wg_hbm, wu_hbm, wd_hbm, out_hbm,
            x_s, x1_s, ha_s, hb_s, oa_s, o_s, w_s, wo_s, wg_s, wu_s, wd_s, ws_s, c_s,
            qt_s, vt_s, k_s, kr_s, s0_s, s1_s, e_s, p_s, tri_s, wr_s, st_s,
            z_s, a_s, y_s, top_s, at_s, sem):
    ha_w, hb_w, x1_w, o_w, w_w, wo_w, qt_w, vt_w, wg_w, wu_w, wd_w, oa_w, ws_w, k_w, e_w = (
        r.bitcast(I32) for r in (ha_s, hb_s, x1_s, o_s, w_s, wo_s, qt_s, vt_s, wg_s, wu_s, wd_s,
                                 oa_s, ws_s, k_s, e_s))
    s_s = (s0_s, s1_s)
    todo = [(kind, u) for kind in (K, Q, V) for u in range(4)]

    def x_in(lo, hi):
        rows = pl.ds(lo * TM, (hi - lo) * TM)
        return [(x_hbm.at[rows], x_s.at[rows])]

    def w_in(*ns):
        tiles = [(todo[n][0], 2 * todo[n][1] + e) for n in ns for e in range(2)]
        return [(wqkv_hbm.at[:, pl.ds(j * D + g * 128, 128)], w_s.at[j, g]) for j, g in tiles]

    def slabs(src, dst):
        return [(src.at[:, pl.ds(g * 128, 128)], dst.at[g]) for g in range(src.shape[1] // 128)]

    groups = [x_in(0, 1), w_in(0, 1), w_in(2, 3), w_in(4, 5), w_in(6, 7) + x_in(1, 2), w_in(8, 9),
              w_in(10, 11), x_in(2, 3) + slabs(wo_hbm, wo_s), x_in(3, NC),
              slabs(wg_hbm, wg_s) + slabs(wu_hbm, wu_s) + slabs(wd_hbm, wd_s)]

    def start(n):
        for src, dst in groups[n]:
            pltpu.make_async_copy(src, dst, sem.at[n]).start()

    def wait(n):
        for src, dst in groups[n]:
            pltpu.make_async_copy(src, dst, sem.at[n]).wait()

    def out_copy(rows):
        return pltpu.make_async_copy(x_s.at[rows], out_hbm.at[rows], sem.at[len(groups)])

    def zero():
        return z_s[0]

    def hide(c):
        return zero() if _static(c) else 0

    def setup():
        row, col = _iota((64, 128), 0), _iota((64, 128), 1)
        tri = jnp.where(2 * row <= col, 0xFFFF, 0) | jnp.where(2 * row + 1 <= col, -65536, 0)
        tri_s[0], tri_s[1] = ~tri, tri
        wr_s[...] = jnp.broadcast_to(wr_ref[...].astype(F32).reshape(1, D), (RB, D))
        z_s[0] = 0
        k_w[0:NHG, 0:48, :] = jnp.zeros((NHG, 48, 128), I32)

    mk = {}

    def make_masks():
        row, col = _iota((32, 128), 0) + zero(), _iota((32, 128), 1) + zero()
        mk["tri"] = row <= (col & 31)
        mk["grp"] = col >> 5
        mk["odd"], mk["high"] = (col[:16] & 32) != 0, col[:16] >= 64

    def lhs(kind, c):
        if _static(c) and c == (NC - 1 if kind == O else 1):
            return hb_s, hb_w
        return (oa_s, oa_w) if kind == O else (ha_s, ha_w)

    def ln_stats(c, j):
        m, _, v = _moments(x_s[_ds(zero() + c * TM + j * RB, RB), :].astype(F32))
        st_s[0, _ds(j * RB, RB)] = jnp.broadcast_to(m, (RB, 128))
        v = jnp.broadcast_to(v, (RB, 128))
        if _static(j):
            st_s[2, 0:RB] = jnp.where(_iota((RB, 128), 1) == j, v, st_s[2, 0:RB]) if j else v
        else:
            st_s[1, _ds(j * RB, RB)] = _inv_std(v)
        return v

    def ln_scales():
        inv = _inv_std(st_s[2, 0:RB])
        for j in range(8):
            st_s[1, j * RB:(j + 1) * RB] = jnp.broadcast_to(inv[:, j:j + 1], (RB, 128))
        return inv

    def stats(c):
        return [P(ln_stats, c, j) for j in range(8)] + [P(ln_scales)]

    def ln_in(c, j):
        def h(b, i):
            r = b * 128 + j * 16
            x = x_s[_ds(zero() + c * TM + r, 16), i * 128:(i + 1) * 128].astype(F32)
            return (x - st_s[0, _ds(r, 16)]) * st_s[1, _ds(r, 16)]

        for i in range(4):
            terms = _lhs_terms(h(0, i), h(0, i + 4), h(1, i), h(1, i + 4))
            for m, a in enumerate(terms):
                lhs(Q, c)[0][m, i, _ds(j * 16, 16), :] = a.astype(BF)
        return jnp.concatenate(terms[:2], 0)

    def prep_o(c, i, e):
        words = [o_w[g, _ds((2 * c + b) * 64 + e * 32, 32), :] for b in range(2) for g in (i, i + 4)]
        for m, a in enumerate(_lhs_terms(*[pltpu.bitcast(w, BF).astype(F32) for w in words])):
            if m in (2, 3):
                lhs(O, c)[1][m, i, e * 32:(e + 1) * 32] = words[3 * (m - 2)]
            else:
                lhs(O, c)[0][m, i, e * 64:(e + 1) * 64] = a.astype(BF)
        return a[32:]

    def prep_w(kind, u, i):
        src, z = (wo_w, zero()) if kind == O else (w_w.at[kind], 0)
        words = [src[z + 2 * u + n % 2, pl.ds((i + 4 * (n // 2)) * 64, 64), :] for n in range(4)]
        tiles = [pltpu.bitcast(w, BF) for w in words]
        if kind in (Q, V):
            tiles = [w.T for w in tiles]
        for m, a in enumerate(_rhs_terms(*[w.astype(F32) for w in tiles])):
            if m in (1, 4):
                ws_w[kind * 4 + u, m, i] = pltpu.bitcast(tiles[m - 1], I32)
            else:
                ws_s[kind * 4 + u, m, i] = a.astype(BF)
        return a[96:]

    def emit(kind, c, b, g, y):
        if kind == Q:
            qt_s[2 * c + b, g] = (y * QSCALE).astype(BF)
        elif kind == K:
            k_s[g, pl.ds(_ds((2 * c + b) * 128, 128).start + 96, 128), :] = y.astype(BF)
        elif kind == V:
            vt_s[2 * c + b, g] = y.astype(BF)
        else:
            rows = _ds((2 * c + b) * 128, 128)
            x1_s[g, rows, :] = (x_s[rows, g * 128:(g + 1) * 128].astype(F32) + y).astype(BF)

    def proj(kind, c, u, m):
        a = _bf16([lhs(kind, c)[1][hide(c) + m, i] for i in range(4)], 1)
        w = [ws_w[kind * 4 + u, m, i] for i in range(4)]
        y = _nt(_bf16(w, 1), a) if kind in (Q, V) else _nn(a, _bf16(w, 0))
        if m == 6:
            c_s[0] = y
        elif m == 4:
            c_s[0] -= y
            c_s[1] = y
        elif m == 2:
            emit(kind, c, 0, 2 * u + 1, c_s[1] + y)
            c_s[3] = y
        elif m == 0:
            c_s[0] += y
            c_s[3] += y
        elif m == 3:
            emit(kind, c, 0, 2 * u, c_s[0] + y)
            c_s[2] = y
        elif m == 1:
            emit(kind, c, 1, 2 * u, c_s[2] + y)
            c_s[3] -= y
        else:
            emit(kind, c, 1, 2 * u + 1, c_s[3] + y)
        return y

    def products(kind, c, u):
        return [P(proj, kind, c, u, m) for m in (6, 4, 2, 0, 3, 1, 5)]

    def k_rep(g, c):
        blocks = [k_w[zero() + g, _ds((c * 8 + i) * 16, 16), :] for i in range(11)]
        for j in range(8):
            r = [blocks[j]] + [pltpu.roll(blocks[j + s], 32 * s, 1) for s in (1, 2, 3)]
            y = [jnp.where(mk["odd"], r[(m + 1) % 4], r[m]) for m in range(4)]
            for h in range(4):
                kr_s[g * 4 + h, _ds((c * 8 + j) * 16, 16), :] = jnp.where(
                    mk["high"], y[(2 - h) % 4], y[-h % 4])

    def qk(g, b, slot):
        lo = max(5 - 4 * b, 0) if _static(b) else 0
        order = ([8] if lo else [0, 8]) + list(range(max(lo, 1), 8))
        for h in range(4):
            q = qt_w[b, g, h * 16:(h + 1) * 16, :]
            w = [jnp.where(mk["grp"][:16] == (p - h) % 4, q, 0) for p in range(4)]
            k = [kr_s[g * 4 + h, _ds(hide(b) + (4 * b - 5 + i) * 16, 16), :] for i in order]
            s = _nn(pltpu.bitcast(jnp.concatenate(k, 0), BF), pltpu.bitcast(jnp.concatenate(w, 0), BF))
            s = {i: s[n * 32:(n + 1) * 32] for n, i in enumerate(order)}
            s[0] = jnp.where(mk["tri"], s.pop(8), NEG if lo else s[0])
            for i in range(lo, lo + 3 if lo else 0):
                s[i] = jnp.where(mk["grp"] >= lo + 3 - i, s[i], NEG)
            m = functools.reduce(jnp.maximum, s.values())
            for i, v in s.items():
                s_s[slot][h, i] = v
            s_s[slot][h, 8, 0:8] = jnp.broadcast_to(jnp.max(m, axis=0, keepdims=True), (8, 128))
        return s

    def softmax(slot, h, live, after):
        m = jnp.concatenate([s_s[slot][zero() + h, 8, 0:8]] * 4, 0)
        l = 0.0
        for n, i in enumerate(live):
            if n // 2 < len(after) and n % 2 == 0:
                s_s[slot][4, 0, 0:8] = after[n // 2]
            p = jnp.exp2(s_s[slot][zero() + h, i] - m)
            e_s[slot * 4 + h, i] = p.astype(BF)
            p = (p[0:8] + p[8:16]) + (p[16:24] + p[24:32])
            l = l + p if n else p
        l = jnp.sum(l, axis=0, keepdims=True)
        none = jnp.zeros((16, 128), I32)
        u = [e_w[slot * 4 + h, i] if i in live else none for i in range(8)]
        u = [jnp.where(mk["odd"], u[(i - 1) % 8], u[i]) for i in range(8)]
        u = [jnp.where(mk["high"], u[(i - 2) % 8], u[i]) for i in range(8)]
        edge = jnp.concatenate(u[:4], 0)
        n = (slot * 4 + h) * 3
        p_s[n] = edge & tri_s[0]
        p_s[n + 1] = jnp.concatenate(u[4:], 0)
        p_s[n + 2] = edge & tri_s[1]
        return 1.0 / l

    def pv(g, b, slot, sums):
        n = min(b + 1, 3) if _static(b) else 3
        outs = []
        for h, linv in enumerate(sums):
            v = _bf16([vt_w[b - i, g, h * 16:(h + 1) * 16, :] for i in range(n - 1, -1, -1)], 1)
            p = _bf16([p_s[(slot * 4 + h) * 3 + i] for i in range(3 - n, 3)], 0)
            outs.append(_nn(v, p) * linv)
        o_s[g, _ds(b * 128, 128), :] = jnp.concatenate(outs, 0).T.astype(BF)

    def route(c, j):
        rows = _ds(zero() + c * (TM // 2) + j * (RB // 2), RB // 2)
        x1 = _bf16([x1_w[g, rows, :] for g in range(8)], 1).astype(F32)
        h = _rb(_ln(x1))
        x_s[_ds(c * TM + j * RB, RB), :] = (x1 + h).astype(BF)
        r = jnp.broadcast_to(_rb(jnp.sum(h * wr_s[...], axis=1, keepdims=True)), (RB, 128))
        top, at = top_s[...], at_s[...]
        for i in range(0, RB, 8):
            better = r[i:i + 8] > top
            top = jnp.where(better, r[i:i + 8], top)
            at = jnp.where(better, c * TM + j * RB + i + _iota((8, 128), 0), at)
        top_s[...], at_s[...] = top, at
        return r

    def argmax():
        top = jnp.max(top_s[...], axis=0, keepdims=True)
        return top[:, 0:1], jnp.min(jnp.where(top_s[...] == top, at_s[...], S - 1)[:, 0:1])

    def block(row):
        return jnp.concatenate([x1_s[g, _ds(row, 16), :] for g in range(8)], 1).astype(F32)

    def glu(hs, t0, n):
        gate, up = (_rb(_nn(hs, _bf16([w[t0 + i] for i in range(n)], 1))) for w in (wg_w, wu_w))
        return gate, (_rb(gate * jax.nn.sigmoid(gate)) * up).astype(BF)

    def release(y, follow):
        follow = [f.func for f in follow]
        for g in range(8) if route in follow else []:
            x1_w[g, S // 2:] = pltpu.bitcast(y[:8], I32)
        if ln_in in follow or ln_stats in follow:
            x_s[S:, :] = jnp.concatenate([y[:16]] * 8, 1).astype(BF)
        if k_rep in follow:
            k_w[NHG, 0:8] = pltpu.bitcast(y[:8], I32)
        if prep_w in follow:
            wo_s[8, 0:16] = y[:16].astype(BF)

    def overlap(main, side, spare, lag):
        due = {}
        for n, f in enumerate(main):
            for e, v in enumerate(due.pop(n, [])):
                spare[e % 2 * 32:e % 2 * 32 + 32] = pltpu.bitcast(v, I32)
            release(f()[:, 0:128], side.get(n, []))
            due[n + lag] = [g() for g in side.get(n, [])]

    def stage(t, qkv=True, out=True, load=False):
        make_masks()
        slots = [[] for _ in range(65)]
        nd = 16 if qkv and out else 0
        if load:
            slots[15] += [P(wait, 7), P(start, 8)]
            _spread(slots, [P(prep_w, O, u, i) for u in range(4) for i in range(4)], 16, 64)
        if qkv and out:
            _spread(slots, [P(ln_in, t + 1, j) for j in range(8)], 0, 12)
        if qkv:
            c = (t + 2) & (NC - 1)
            _spread(slots, stats(c), *((17, 35) if load else (13, 31)))
            _spread(slots, [P(k_rep, g, t + 1) for g in range(NHG)], 29, 61)
        if qkv and out:
            _spread(slots, [P(route, t - 1, j) for j in range(8)], 32, 64)
        for i in range(4):
            for e in range(2):
                slots[min(16 * i + 19 + 4 * e, 64)].append(P(prep_o, t, i, e))
        fs = [f for u in range(4) for f in products(O, t - 1, u)] if out else []
        if qkv:
            _spread(slots, fs, 0, nd)
            fs = [f for kind, u in todo for f in products(kind, t + 1, u)]
        _spread(slots, fs[:-2], nd, 64)
        slots[64] += fs[-2:]

        quads = [(i + g, 2 * t + b) for i in range(4) for g in (0, 4) for b in range(2)]
        due, after = {}, []
        nxt = qk(*quads[0], 0)
        for n, quad in enumerate(quads):
            live = sorted(nxt)
            if n + 1 < len(quads):
                nxt = qk(*quads[n + 1], (n + 1) % 2)
            sums, y = [], None
            for i in range(4 * n, 4 * n + 4):
                if not qkv and n + 1 < len(quads) and i % 4:
                    after = [nxt[i % 4 * 2 - 2][:8]]
                sums.append(softmax(n % 2, i % 4, live, after))
                ys, after = [], []
                for f in slots[i]:
                    if f.func in (route, ln_in, ln_stats, ln_scales, prep_w, prep_o):
                        due.setdefault(i + 2, []).append(f())
                    elif f.func is proj:
                        y = f()
                        ys.append(y)
                    else:
                        f()
                scores = s_s[(i + 1) // 4 % 2]
                for e, v in enumerate(due.pop(i, []) if i < 63 else []):
                    scores[4, 1 + e] = v
                if y is not None and i < 63:
                    if qkv:
                        after = [ys[0][r:r + 8] for r in range(0, 128, 32)]
                    release(y[64:], slots[i + 1])
            pv(*quad, n % 2, sums)
        for f in slots[64]:
            f()

    def first_chunk(load):
        def prep(n):
            if n % 2 == 0:
                wait(n // 2 + 1)
                if n != 8:
                    start(min(n // 2 + 3, 7))
            return [P(prep_w, *todo[n], i) for i in range(4)]

        if load:
            start(0)
            start(1)
            setup()
            wait(0)
            for f in stats(0):
                f()
            start(2)
            for j in range(8):
                ln_in(0, j)
            for f in prep(0):
                f()
        make_masks()
        norm = stats(1) + [P(ln_in, 1, j) for j in range(8)]
        for n, (kind, u) in enumerate(todo):
            side = prep(n + 1) if load and n < 11 else []
            if n >= 4:
                side.append(P(k_rep, n - 4, 0))
            if n >= 6:
                side += norm[(n - 6) * 3:(n - 5) * 3]
            for f in products(kind, 0, u):
                y = f()
                now, side = side[:1 + len(side) // 8], side[1 + len(side) // 8:]
                release(y, now)
                for g in now:
                    g()
            assert not side

    def finish(first):
        route(NC - 2, 0)
        overlap([f for u in range(4) for f in products(O, NC - 1, u)],
                {j * 11 // 4 - 1: [P(route, NC - 2, j)] for j in range(1, 8)}, hb_w.at[7, 0], 6)

        guess = argmax()[1] // 16 * 16
        hs = _ln(block(guess)).astype(BF)
        acts = []
        route(NC - 1, 0)
        route(NC - 1, 1)

        def up(j):
            gate, a = glu(hs, zero() + 4 * j, 4)
            acts.append(a)
            return gate

        def down(j):
            y = _nn(acts[j], _bf16([wd_w[zero() + g, j * 256:(j + 1) * 256] for g in range(8)], 1))
            y_s[...] = y_s[...] + y if j else y
            return y

        overlap([P(up, j) for j in range(7)],
                {j: [P(route, NC - 1, j + 2)] for j in range(6)}, wg_w.at[F // 128], 2)
        rmax, idx = argmax()
        base = idx // 16 * 16
        tail = pl.ds(S - 2 * TM, 2 * TM)
        side = {}
        if first:
            ln_in(0, 0)
            ln_in(0, 1)
            side = {n: [P(ln_in, 0, n + 2)] for n in range(6)}
        else:
            out_copy(tail).start()
        overlap([P(down, j) for j in range(7)], side, wd_w.at[8], 2)
        x1 = block(base)
        hs = _ln(x1).astype(BF)

        def up_again(j, _):
            a_s[j] = glu(hs, 7 * j, 7)[1]

        def down_again(j, _):
            a = jnp.concatenate([a_s[i, :, :] for i in range(4)], 1)
            y_s[:, _ds(j * 512, 512)] = _nn(a, _bf16([wd_w[4 * j + g] for g in range(4)], 1))

        lax.fori_loop(0, jnp.where(base == guess, 0, 4), up_again, None)
        lax.fori_loop(0, jnp.where(base == guess, 0, 2), down_again, None)
        y = _rb(_rb(y_s[...]) * _rb(jax.nn.sigmoid(rmax)))
        upd = jnp.where(_iota((16, D), 0) == idx - base, y, 0.0)
        new = (x1 + _rb(hs.astype(F32) + upd)).astype(BF)
        if first:
            x_s[_ds(base, 16), :] = new
            ln_stats(0, base % TM // RB)
            ln_in(0, base % 128 // 16)
        else:
            for rows in [_ds(c * TM, TM) for c in range(NC - 2)] + [tail]:
                out_copy(rows).wait()
            x_s[_ds(base, 16), :] = new
            out_copy(_ds(base, 16)).start()
            out_copy(_ds(base, 16)).wait()

    def layer(first):
        first_chunk(first)
        top_s[...] = jnp.full((8, 128), -jnp.inf, F32)
        at_s[...] = _iota((8, 128), 0)
        stage(0, out=False, load=first)
        if first:
            wait(8)
            start(9)

        def body(t, _):
            stage(t)
            if not first:
                out_copy(_ds((t - 1) * TM, TM)).start()

        lax.fori_loop(1, NC - 1, body, None)
        if first:
            wait(9)
        stage(NC - 1, qkv=False)
        finish(first)

    layer(True)
    layer(False)


@jax.jit
def pallas_interleave_layers__sliding_block__moe_arch_mod__prompt_kernel(
    A_x: jax.Array,
    A_wqkv: jax.Array,
    A_wo: jax.Array,
    B_x: jax.Array,
    B_w_r: jax.Array,
    B_w_gate: jax.Array,
    B_w_up: jax.Array,
    B_w_down: jax.Array,
):
    del B_x
    hbm = pl.BlockSpec(memory_space=pl.ANY)
    out = pl.pallas_call(
        _kernel,
        out_shape=jax.ShapeDtypeStruct((S, D), BF),
        in_specs=[pl.BlockSpec(memory_space=pltpu.VMEM)] + [hbm] * 6,
        out_specs=hbm,
        scratch_shapes=[
            pltpu.VMEM((S + 16, D), BF),
            pltpu.VMEM((8, S + 16, 128), BF),
            pltpu.VMEM((7, 4, 128, 128), BF),
            pltpu.VMEM((8, 4, 128, 128), BF),
            pltpu.VMEM((7, 4, 128, 128), BF),
            pltpu.VMEM((NHG, S, 128), BF),
            pltpu.VMEM((3, NHG, D, 128), BF),
            pltpu.VMEM((9, D, 128), BF),
            pltpu.VMEM((F // 128 + 1, D, 128), BF),
            pltpu.VMEM((F // 128, D, 128), BF),
            pltpu.VMEM((9, F, 128), BF),
            pltpu.VMEM((16, 7, 4, 128, 128), BF),
            pltpu.VMEM((4, 128, 128), F32),
            pltpu.VMEM((NQB, NHG, 128, 128), BF),
            pltpu.VMEM((NQB, NHG, 128, 128), BF),
            pltpu.VMEM((NHG + 1, 128 + S, 128), BF),
            pltpu.VMEM((32, 64 * 16, 128), I32),
            pltpu.VMEM((5, 9, 32, 128), F32),
            pltpu.VMEM((5, 9, 32, 128), F32),
            pltpu.VMEM((8, 8, 32, 128), BF),
            pltpu.VMEM((24, 64, 128), I32),
            pltpu.VMEM((2, 64, 128), I32),
            pltpu.VMEM((RB, D), F32),
            pltpu.VMEM((3, TM, 128), F32),
            pltpu.SMEM((1,), I32),
            pltpu.VMEM((4, 16, F // 4), BF),
            pltpu.VMEM((16, D), F32),
            pltpu.VMEM((8, 128), F32),
            pltpu.VMEM((8, 128), I32),
            pltpu.SemaphoreType.DMA((11,)),
        ],
        compiler_params=pltpu.CompilerParams(vmem_limit_bytes=110 * 1024 * 1024),
    )(B_w_r, A_x.reshape(S, D), A_wqkv, A_wo, B_w_gate, B_w_up, B_w_down)
    return out.reshape(1, S, D)
```

```python
import functools

import jax
import jax.numpy as jnp
import numpy as np
from jax import lax
import jax.experimental.pallas as pl
import jax.experimental.pallas.tpu as pltpu

S, D, F = 2048, 1024, 3584
NHG = 8
NQB = S // 128
TM = 256
NC = S // TM
RB = TM // 8
Q, K, V, O = range(4)
BF, F32, I32 = jnp.bfloat16, jnp.float32, jnp.int32
NEG = -1e9

_bf = lambda v: float(np.asarray(v, dtype=jnp.bfloat16).astype(np.float32))
QSCALE = _bf(32 ** -0.5) * float(np.log2(np.e))
EPS = _bf(1e-5)
P = functools.partial


def _rb(x):
    return x.astype(BF).astype(F32)


def _moments(x):
    m = jnp.mean(x, axis=1, keepdims=True)
    xc = x - m
    return m, xc, jnp.mean(xc * xc, axis=1, keepdims=True)


def _inv_std(v):
    return 1.0 / _rb(jnp.sqrt(_rb(_rb(v) + EPS)))


def _ln(x):
    _, xc, v = _moments(x)
    return xc * _inv_std(v)


def _nt(a, b):
    return lax.dot_general(a, b, (((1,), (1,)), ((), ())), preferred_element_type=F32)


def _nn(a, b):
    return jnp.dot(a, b, preferred_element_type=F32)


def _bf16(words, axis):
    return jnp.concatenate([pltpu.bitcast(w, BF) for w in words], axis)


def _lhs_terms(a11, a12, a21, a22):
    return [a11 + a22, a21 + a22, a11, a22, a11 + a12, a21 - a11, a12 - a22]


def _rhs_terms(b11, b12, b21, b22):
    return [b11 + b22, b11, b12 - b22, b21 - b11, b22, b11 + b12, b21 + b22]


def _static(i):
    return isinstance(i, int)


def _ds(start, size):
    return pl.ds(start if _static(start) else pl.multiple_of(start, size), size)


def _iota(shape, d):
    return lax.broadcasted_iota(I32, shape, d)


def _spread(slots, pieces, lo, hi):
    for i, f in enumerate(pieces):
        slots[lo + i * (hi - lo) // len(pieces)].append(f)


def _kernel(wr_ref, x_hbm, wqkv_hbm, wo_hbm, wg_hbm, wu_hbm, wd_hbm, out_hbm,
            x_s, x1_s, ha_s, hb_s, oa_s, o_s, w_s, wo_s, wg_s, wu_s, wd_s, ws_s, c_s,
            qt_s, vt_s, k_s, kr_s, s0_s, s1_s, e_s, p_s, tri_s, wr_s, st_s,
            z_s, a_s, y_s, top_s, at_s, sem):
    ha_w, hb_w, x1_w, o_w, w_w, wo_w, qt_w, vt_w, wg_w, wu_w, wd_w, oa_w, ws_w, k_w, e_w = (
        r.bitcast(I32) for r in (ha_s, hb_s, x1_s, o_s, w_s, wo_s, qt_s, vt_s, wg_s, wu_s, wd_s,
                                 oa_s, ws_s, k_s, e_s))
    s_s = (s0_s, s1_s)
    todo = [(kind, u) for kind in (K, Q, V) for u in range(4)]

    def x_in(lo, hi):
        rows = pl.ds(lo * TM, (hi - lo) * TM)
        return [(x_hbm.at[rows], x_s.at[rows])]

    def w_in(*ns):
        tiles = [(todo[n][0], 2 * todo[n][1] + e) for n in ns for e in range(2)]
        return [(wqkv_hbm.at[:, pl.ds(j * D + g * 128, 128)], w_s.at[j, g]) for j, g in tiles]

    def slabs(src, dst):
        return [(src.at[:, pl.ds(g * 128, 128)], dst.at[g]) for g in range(src.shape[1] // 128)]

    groups = [x_in(0, 1), x_in(1, 2), w_in(0), w_in(1), w_in(2, 3), w_in(4, 5, 6), w_in(7, 8, 9),
              w_in(10, 11) + x_in(2, 3), slabs(wo_hbm, wo_s), x_in(3, NC),
              slabs(wg_hbm, wg_s) + slabs(wu_hbm, wu_s) + slabs(wd_hbm, wd_s)]

    def start(n):
        for src, dst in groups[n]:
            pltpu.make_async_copy(src, dst, sem.at[n]).start()

    def wait(n):
        for src, dst in groups[n]:
            pltpu.make_async_copy(src, dst, sem.at[n]).wait()

    def out_copy(rows):
        return pltpu.make_async_copy(x_s.at[rows], out_hbm.at[rows], sem.at[len(groups)])

    def zero():
        return z_s[0]

    def hide(c):
        return zero() if _static(c) else 0

    def setup():
        row, col = _iota((64, 128), 0), _iota((64, 128), 1)
        tri = jnp.where(2 * row <= col, 0xFFFF, 0) | jnp.where(2 * row + 1 <= col, -65536, 0)
        tri_s[0], tri_s[1] = ~tri, tri
        wr_s[...] = jnp.broadcast_to(wr_ref[...].astype(F32).reshape(1, D), (RB, D))
        z_s[0] = 0
        k_w[0:NHG, 0:48, :] = jnp.zeros((NHG, 48, 128), I32)

    mk = {}

    def make_masks():
        row, col = _iota((32, 128), 0) + zero(), _iota((32, 128), 1) + zero()
        mk["tri"] = row <= (col & 31)
        mk["grp"] = col >> 5
        mk["odd"], mk["high"] = (col[:16] & 32) != 0, col[:16] >= 64

    def lhs(kind, c):
        if _static(c) and c == (NC - 1 if kind == O else 1):
            return hb_s, hb_w
        return (oa_s, oa_w) if kind == O else (ha_s, ha_w)

    def ln_stats(c, j):
        m, _, v = _moments(x_s[_ds(zero() + c * TM + j * RB, RB), :].astype(F32))
        st_s[0, _ds(j * RB, RB)] = jnp.broadcast_to(m, (RB, 128))
        v = jnp.broadcast_to(v, (RB, 128))
        if _static(j):
            st_s[2, 0:RB] = jnp.where(_iota((RB, 128), 1) == j, v, st_s[2, 0:RB]) if j else v
        else:
            st_s[1, _ds(j * RB, RB)] = _inv_std(v)
        return v

    def ln_scales():
        inv = _inv_std(st_s[2, 0:RB])
        for j in range(8):
            st_s[1, j * RB:(j + 1) * RB] = jnp.broadcast_to(inv[:, j:j + 1], (RB, 128))
        return inv

    def stats(c):
        return [P(ln_stats, c, j) for j in range(8)] + [P(ln_scales)]

    def ln_in(c, j):
        def h(b, i):
            r = b * 128 + j * 16
            x = x_s[_ds(zero() + c * TM + r, 16), i * 128:(i + 1) * 128].astype(F32)
            return (x - st_s[0, _ds(r, 16)]) * st_s[1, _ds(r, 16)]

        for i in range(4):
            terms = _lhs_terms(h(0, i), h(0, i + 4), h(1, i), h(1, i + 4))
            for m, a in enumerate(terms):
                lhs(Q, c)[0][m, i, _ds(j * 16, 16), :] = a.astype(BF)
        return jnp.concatenate(terms[:2], 0)

    def prep_o(c, i, e):
        words = [o_w[g, _ds((2 * c + b) * 64 + e * 32, 32), :] for b in range(2) for g in (i, i + 4)]
        for m, a in enumerate(_lhs_terms(*[pltpu.bitcast(w, BF).astype(F32) for w in words])):
            if m in (2, 3):
                lhs(O, c)[1][m, i, e * 32:(e + 1) * 32] = words[3 * (m - 2)]
            else:
                lhs(O, c)[0][m, i, e * 64:(e + 1) * 64] = a.astype(BF)
        return a[32:]

    def prep_w(kind, u, i):
        src, z = (wo_w, zero()) if kind == O else (w_w.at[kind], 0)
        words = [src[z + 2 * u + n % 2, pl.ds((i + 4 * (n // 2)) * 64, 64), :] for n in range(4)]
        tiles = [pltpu.bitcast(w, BF) for w in words]
        if kind in (Q, V):
            tiles = [w.T for w in tiles]
        for m, a in enumerate(_rhs_terms(*[w.astype(F32) for w in tiles])):
            if m in (1, 4):
                ws_w[kind * 4 + u, m, i] = pltpu.bitcast(tiles[m - 1], I32)
            else:
                ws_s[kind * 4 + u, m, i] = a.astype(BF)
        return a[96:]

    def emit(kind, c, b, g, y):
        if kind == Q:
            qt_s[2 * c + b, g] = (y * QSCALE).astype(BF)
        elif kind == K:
            k_s[g, pl.ds(_ds((2 * c + b) * 128, 128).start + 96, 128), :] = y.astype(BF)
        elif kind == V:
            vt_s[2 * c + b, g] = y.astype(BF)
        else:
            rows = _ds((2 * c + b) * 128, 128)
            x1_s[g, rows, :] = (x_s[rows, g * 128:(g + 1) * 128].astype(F32) + y).astype(BF)

    def proj(kind, c, u, m):
        a = _bf16([lhs(kind, c)[1][hide(c) + m, i] for i in range(4)], 1)
        w = [ws_w[kind * 4 + u, m, i] for i in range(4)]
        y = _nt(_bf16(w, 1), a) if kind in (Q, V) else _nn(a, _bf16(w, 0))
        if m == 6:
            c_s[0] = y
        elif m == 4:
            c_s[0] -= y
            c_s[1] = y
        elif m == 2:
            emit(kind, c, 0, 2 * u + 1, c_s[1] + y)
            c_s[3] = y
        elif m == 0:
            c_s[0] += y
            c_s[3] += y
        elif m == 3:
            emit(kind, c, 0, 2 * u, c_s[0] + y)
            c_s[2] = y
        elif m == 1:
            emit(kind, c, 1, 2 * u, c_s[2] + y)
            c_s[3] -= y
        else:
            emit(kind, c, 1, 2 * u + 1, c_s[3] + y)
        return y

    def products(kind, c, u):
        return [P(proj, kind, c, u, m) for m in (6, 4, 2, 0, 3, 1, 5)]

    def k_rep(g, c):
        blocks = [k_w[zero() + g, _ds((c * 8 + i) * 16, 16), :] for i in range(11)]
        for j in range(8):
            r = [blocks[j]] + [pltpu.roll(blocks[j + s], 32 * s, 1) for s in (1, 2, 3)]
            y = [jnp.where(mk["odd"], r[(m + 1) % 4], r[m]) for m in range(4)]
            for h in range(4):
                kr_s[g * 4 + h, _ds((c * 8 + j) * 16, 16), :] = jnp.where(
                    mk["high"], y[(2 - h) % 4], y[-h % 4])

    def qk(g, b, slot):
        lo = max(5 - 4 * b, 0) if _static(b) else 0
        order = ([8] if lo else [0, 8]) + list(range(max(lo, 1), 8))
        for h in range(4):
            q = qt_w[b, g, h * 16:(h + 1) * 16, :]
            w = [jnp.where(mk["grp"][:16] == (p - h) % 4, q, 0) for p in range(4)]
            k = [kr_s[g * 4 + h, _ds(hide(b) + (4 * b - 5 + i) * 16, 16), :] for i in order]
            s = _nn(pltpu.bitcast(jnp.concatenate(k, 0), BF), pltpu.bitcast(jnp.concatenate(w, 0), BF))
            s = {i: s[n * 32:(n + 1) * 32] for n, i in enumerate(order)}
            s[0] = jnp.where(mk["tri"], s.pop(8), NEG if lo else s[0])
            for i in range(lo, lo + 3 if lo else 0):
                s[i] = jnp.where(mk["grp"] >= lo + 3 - i, s[i], NEG)
            m = functools.reduce(jnp.maximum, s.values())
            for i, v in s.items():
                s_s[slot][h, i] = v
            s_s[slot][h, 8, 0:8] = jnp.broadcast_to(jnp.max(m, axis=0, keepdims=True), (8, 128))
        return s

    def softmax(slot, h, live, after):
        m = jnp.concatenate([s_s[slot][zero() + h, 8, 0:8]] * 4, 0)
        l = 0.0
        for n, i in enumerate(live):
            if n // 2 < len(after) and n % 2 == 0:
                s_s[slot][4, 0, 0:8] = after[n // 2]
            p = jnp.exp2(s_s[slot][zero() + h, i] - m)
            e_s[slot * 4 + h, i] = p.astype(BF)
            p = (p[0:8] + p[8:16]) + (p[16:24] + p[24:32])
            l = l + p if n else p
        l = jnp.sum(l, axis=0, keepdims=True)
        none = jnp.zeros((16, 128), I32)
        u = [e_w[slot * 4 + h, i] if i in live else none for i in range(8)]
        u = [jnp.where(mk["odd"], u[(i - 1) % 8], u[i]) for i in range(8)]
        u = [jnp.where(mk["high"], u[(i - 2) % 8], u[i]) for i in range(8)]
        edge = jnp.concatenate(u[:4], 0)
        n = (slot * 4 + h) * 3
        p_s[n] = edge & tri_s[0]
        p_s[n + 1] = jnp.concatenate(u[4:], 0)
        p_s[n + 2] = edge & tri_s[1]
        return 1.0 / l

    def pv(g, b, slot, sums):
        n = min(b + 1, 3) if _static(b) else 3
        outs = []
        for h, linv in enumerate(sums):
            v = _bf16([vt_w[b - i, g, h * 16:(h + 1) * 16, :] for i in range(n - 1, -1, -1)], 1)
            p = _bf16([p_s[(slot * 4 + h) * 3 + i] for i in range(3 - n, 3)], 0)
            outs.append(_nn(v, p) * linv)
        o_s[g, _ds(b * 128, 128), :] = jnp.concatenate(outs, 0).T.astype(BF)

    def route(c, j):
        rows = _ds(zero() + c * (TM // 2) + j * (RB // 2), RB // 2)
        x1 = _bf16([x1_w[g, rows, :] for g in range(8)], 1).astype(F32)
        h = _rb(_ln(x1))
        x_s[_ds(c * TM + j * RB, RB), :] = (x1 + h).astype(BF)
        r = jnp.broadcast_to(_rb(jnp.sum(h * wr_s[...], axis=1, keepdims=True)), (RB, 128))
        top, at = top_s[...], at_s[...]
        for i in range(0, RB, 8):
            better = r[i:i + 8] > top
            top = jnp.where(better, r[i:i + 8], top)
            at = jnp.where(better, c * TM + j * RB + i + _iota((8, 128), 0), at)
        top_s[...], at_s[...] = top, at
        return r

    def argmax():
        top = jnp.max(top_s[...], axis=0, keepdims=True)
        return top[:, 0:1], jnp.min(jnp.where(top_s[...] == top, at_s[...], S - 1)[:, 0:1])

    def block(row):
        return jnp.concatenate([x1_s[g, _ds(row, 16), :] for g in range(8)], 1).astype(F32)

    def glu(hs, t0, n):
        gate, up = (_rb(_nn(hs, _bf16([w[t0 + i] for i in range(n)], 1))) for w in (wg_w, wu_w))
        return gate, (_rb(gate * jax.nn.sigmoid(gate)) * up).astype(BF)

    def release(y, follow):
        follow = [f.func for f in follow]
        for g in range(8) if route in follow else []:
            x1_w[g, S // 2:] = pltpu.bitcast(y[:8], I32)
        if ln_in in follow or ln_stats in follow:
            x_s[S:, :] = jnp.concatenate([y[:16]] * 8, 1).astype(BF)
        if k_rep in follow:
            k_w[NHG, 0:8] = pltpu.bitcast(y[:8], I32)
        if prep_w in follow:
            wo_s[8, 0:16] = y[:16].astype(BF)

    def overlap(main, side, spare, lag):
        due = {}
        for n, f in enumerate(main):
            for e, v in enumerate(due.pop(n, [])):
                spare[e % 2 * 32:e % 2 * 32 + 32] = pltpu.bitcast(v, I32)
            release(f()[:, 0:128], side.get(n, []))
            due[n + lag] = [g() for g in side.get(n, [])]

    def stage(t, qkv=True, out=True, load=False):
        make_masks()
        slots = [[] for _ in range(65)]
        nd = 16 if qkv and out else 0
        if load:
            _spread(slots, [P(prep_w, O, u, i) for u in range(4) for i in range(4)], 2, 66)
        if qkv and out:
            _spread(slots, [P(ln_in, t + 1, j) for j in range(8)], 0, 12)
        if qkv and not load:
            c = (t + 2) & (NC - 1)
            _spread(slots, stats(c), 13, 31)
            _spread(slots, [P(k_rep, g, t + 1) for g in range(NHG)], 29, 61)
        if qkv and out:
            _spread(slots, [P(route, t - 1, j) for j in range(8)], 32, 64)
        for i in range(4):
            for e in range(2):
                slots[min(16 * i + 19 + 4 * e, 64)].append(P(prep_o, t, i, e))
        fs = [f for u in range(4) for f in products(O, t - 1, u)] if out else []
        if qkv:
            _spread(slots, fs, 0, nd)
            fs = [f for kind, u in todo[8 * load:] for f in products(kind, t + 1, u)]
        _spread(slots, fs[:-2], nd, 64)
        slots[64] += fs[-2:]

        quads = [(i + g, 2 * t + b) for i in range(4) for g in (0, 4) for b in range(2)]
        due, after = {}, []
        nxt = qk(*quads[0], 0)
        for n, quad in enumerate(quads):
            live = sorted(nxt)
            if n + 1 < len(quads):
                nxt = qk(*quads[n + 1], (n + 1) % 2)
            sums, y = [], None
            for i in range(4 * n, 4 * n + 4):
                if (load or not qkv) and n + 1 < len(quads) and i % 4:
                    after = [nxt[sorted(nxt)[(i % 4 - 1) * len(nxt) // 4]][:8]]
                sums.append(softmax(n % 2, i % 4, live, after))
                ys, after = [], []
                for f in slots[i]:
                    if f.func in (route, ln_in, ln_stats, ln_scales, prep_w, prep_o):
                        due.setdefault(i + 2, []).append(f())
                    elif f.func is proj:
                        y = f()
                        ys.append(y)
                    else:
                        f()
                scores = s_s[(i + 1) // 4 % 2]
                for e, v in enumerate(due.pop(i, []) if i < 63 else []):
                    scores[4, 1 + e] = v
                if y is not None and i < 63:
                    if qkv and not load:
                        after = [ys[0][r:r + 8] for r in range(0, 128, 32)]
                    release(y[64:], slots[i + 1])
            pv(*quad, n % 2, sums)
        for f in slots[64]:
            f()

    def interleave(main, side):
        step = -(-len(side) // len(main))
        for n, f in enumerate(main):
            now = side[n * step:(n + 1) * step]
            release(f(), now)
            for g in now:
                g()

    def first_chunk(load):
        norm = stats(1) + [P(ln_in, 1, j) for j in range(8)]
        if load:
            start(0)
            setup()
            start(1)
            for n, fs in enumerate((stats(0) + [P(ln_in, 0, j) for j in range(8)], norm,
                                    [P(prep_w, *todo[0], i) for i in range(4)])):
                wait(n)
                start(n + 2)
                for f in fs:
                    f()
        make_masks()
        for n, (kind, u) in enumerate(todo):
            main, side = products(kind, 0, u), [P(k_rep, n - 4, 0)] if n >= 4 else []
            if not load:
                side += norm[max(n - 6, 0) * 3:max(n - 5, 0) * 3]
            else:
                if n == 0:
                    interleave(main, [])
                    main = []
                if n in (0, 1, 3, 6, 9):
                    group = (0, 1, 3, 6, 9).index(n) + 3
                    wait(group)
                    start(group + 2)
                side = [P(prep_w, *todo[n + 1], i) for i in range(4)] if n < 11 else stats(2)
                if n < 8:
                    main += products(kind, 1, u)
                if 1 <= n <= 8:
                    side += [P(k_rep, n - 1, c) for c in range(2)]
            interleave(main, side)
        if load:
            wait(8)

    def finish(first):
        route(NC - 2, 0)
        overlap([f for u in range(4) for f in products(O, NC - 1, u)],
                {j * 11 // 4 - 1: [P(route, NC - 2, j)] for j in range(1, 8)}, hb_w.at[7, 0], 6)

        guess = argmax()[1] // 16 * 16
        hs = _ln(block(guess)).astype(BF)
        acts = []
        route(NC - 1, 0)
        route(NC - 1, 1)

        def up(j):
            gate, a = glu(hs, zero() + 4 * j, 4)
            acts.append(a)
            return gate

        def down(j):
            y = _nn(acts[j], _bf16([wd_w[zero() + g, j * 256:(j + 1) * 256] for g in range(8)], 1))
            y_s[...] = y_s[...] + y if j else y
            return y

        overlap([P(up, j) for j in range(7)],
                {j: [P(route, NC - 1, j + 2)] for j in range(6)}, wg_w.at[F // 128], 2)
        rmax, idx = argmax()
        base = idx // 16 * 16
        tail = pl.ds(S - 2 * TM, 2 * TM)
        side = {}
        if first:
            ln_in(0, 0)
            ln_in(0, 1)
            side = {n: [P(ln_in, 0, n + 2)] for n in range(6)}
        else:
            out_copy(tail).start()
        overlap([P(down, j) for j in range(7)], side, wd_w.at[8], 2)
        x1 = block(base)
        hs = _ln(x1).astype(BF)

        def up_again(j, _):
            a_s[j] = glu(hs, 7 * j, 7)[1]

        def down_again(j, _):
            a = jnp.concatenate([a_s[i, :, :] for i in range(4)], 1)
            y_s[:, _ds(j * 512, 512)] = _nn(a, _bf16([wd_w[4 * j + g] for g in range(4)], 1))

        lax.fori_loop(0, jnp.where(base == guess, 0, 4), up_again, None)
        lax.fori_loop(0, jnp.where(base == guess, 0, 2), down_again, None)
        y = _rb(_rb(y_s[...]) * _rb(jax.nn.sigmoid(rmax)))
        upd = jnp.where(_iota((16, D), 0) == idx - base, y, 0.0)
        new = (x1 + _rb(hs.astype(F32) + upd)).astype(BF)
        if first:
            x_s[_ds(base, 16), :] = new
            ln_stats(0, base % TM // RB)
            ln_in(0, base % 128 // 16)
        else:
            for rows in [_ds(c * TM, TM) for c in range(NC - 2)] + [tail]:
                out_copy(rows).wait()
            x_s[_ds(base, 16), :] = new
            out_copy(_ds(base, 16)).start()
            out_copy(_ds(base, 16)).wait()

    def layer(first):
        first_chunk(first)
        top_s[...] = jnp.full((8, 128), -jnp.inf, F32)
        at_s[...] = _iota((8, 128), 0)
        stage(0, out=False, load=first)
        if first:
            wait(9)
            start(10)

        def body(t, _):
            stage(t)
            if not first:
                out_copy(_ds((t - 1) * TM, TM)).start()

        lax.fori_loop(1, NC - 1, body, None)
        if first:
            wait(10)
        stage(NC - 1, qkv=False)
        finish(first)

    layer(True)
    layer(False)


@jax.jit
def pallas_interleave_layers__sliding_block__moe_arch_mod__prompt_kernel(
    A_x: jax.Array,
    A_wqkv: jax.Array,
    A_wo: jax.Array,
    B_x: jax.Array,
    B_w_r: jax.Array,
    B_w_gate: jax.Array,
    B_w_up: jax.Array,
    B_w_down: jax.Array,
):
    del B_x
    hbm = pl.BlockSpec(memory_space=pl.ANY)
    out = pl.pallas_call(
        _kernel,
        out_shape=jax.ShapeDtypeStruct((S, D), BF),
        in_specs=[pl.BlockSpec(memory_space=pltpu.VMEM)] + [hbm] * 6,
        out_specs=hbm,
        scratch_shapes=[
            pltpu.VMEM((S + 16, D), BF),
            pltpu.VMEM((8, S + 16, 128), BF),
            pltpu.VMEM((7, 4, 128, 128), BF),
            pltpu.VMEM((8, 4, 128, 128), BF),
            pltpu.VMEM((7, 4, 128, 128), BF),
            pltpu.VMEM((NHG, S, 128), BF),
            pltpu.VMEM((3, NHG, D, 128), BF),
            pltpu.VMEM((9, D, 128), BF),
            pltpu.VMEM((F // 128 + 1, D, 128), BF),
            pltpu.VMEM((F // 128, D, 128), BF),
            pltpu.VMEM((9, F, 128), BF),
            pltpu.VMEM((16, 7, 4, 128, 128), BF),
            pltpu.VMEM((4, 128, 128), F32),
            pltpu.VMEM((NQB, NHG, 128, 128), BF),
            pltpu.VMEM((NQB, NHG, 128, 128), BF),
            pltpu.VMEM((NHG + 1, 128 + S, 128), BF),
            pltpu.VMEM((32, 64 * 16, 128), I32),
            pltpu.VMEM((5, 9, 32, 128), F32),
            pltpu.VMEM((5, 9, 32, 128), F32),
            pltpu.VMEM((8, 8, 32, 128), BF),
            pltpu.VMEM((24, 64, 128), I32),
            pltpu.VMEM((2, 64, 128), I32),
            pltpu.VMEM((RB, D), F32),
            pltpu.VMEM((3, TM, 128), F32),
            pltpu.SMEM((1,), I32),
            pltpu.VMEM((4, 16, F // 4), BF),
            pltpu.VMEM((16, D), F32),
            pltpu.VMEM((8, 128), F32),
            pltpu.VMEM((8, 128), I32),
            pltpu.SemaphoreType.DMA((12,)),
        ],
        compiler_params=pltpu.CompilerParams(vmem_limit_bytes=110 * 1024 * 1024),
    )(B_w_r, A_x.reshape(S, D), A_wqkv, A_wo, B_w_gate, B_w_up, B_w_down)
    return out.reshape(1, S, D)
```

```python
import functools

import jax
import jax.numpy as jnp
import numpy as np
from jax import lax
import jax.experimental.pallas as pl
import jax.experimental.pallas.tpu as pltpu

S, D, F = 2048, 1024, 3584
NHG = 8
NQB = S // 128
TM = 256
NC = S // TM
RB = TM // 8
Q, K, V, O = range(4)
BF, F32, I32 = jnp.bfloat16, jnp.float32, jnp.int32
NEG = -1e9

_bf = lambda v: float(np.asarray(v, dtype=jnp.bfloat16).astype(np.float32))
QSCALE = _bf(32 ** -0.5) * float(np.log2(np.e))
EPS = _bf(1e-5)
P = functools.partial


def _rb(x):
    return x.astype(BF).astype(F32)


def _moments(x):
    m = jnp.mean(x, axis=1, keepdims=True)
    xc = x - m
    return m, xc, jnp.mean(xc * xc, axis=1, keepdims=True)


def _inv_std(v):
    return 1.0 / _rb(jnp.sqrt(_rb(_rb(v) + EPS)))


def _ln(x):
    _, xc, v = _moments(x)
    return xc * _inv_std(v)


def _nt(a, b):
    return lax.dot_general(a, b, (((1,), (1,)), ((), ())), preferred_element_type=F32)


def _nn(a, b):
    return jnp.dot(a, b, preferred_element_type=F32)


def _bf16(words, axis):
    return jnp.concatenate([pltpu.bitcast(w, BF) for w in words], axis)


def _lhs_terms(a11, a12, a21, a22):
    return [a11 + a22, a21 + a22, a11, a22, a11 + a12, a21 - a11, a12 - a22]


def _rhs_terms(b11, b12, b21, b22):
    return [b11 + b22, b11, b12 - b22, b21 - b11, b22, b11 + b12, b21 + b22]


def _static(i):
    return isinstance(i, int)


def _ds(start, size):
    return pl.ds(start if _static(start) else pl.multiple_of(start, size), size)


def _iota(shape, d):
    return lax.broadcasted_iota(I32, shape, d)


def _spread(slots, pieces, lo, hi):
    for i, f in enumerate(pieces):
        slots[lo + i * (hi - lo) // len(pieces)].append(f)


def _kernel(wr_ref, x_hbm, wqkv_hbm, wo_hbm, wg_hbm, wu_hbm, wd_hbm, out_hbm,
            x_s, x1_s, ha_s, hb_s, oa_s, o_s, w_s, wo_s, wg_s, wu_s, wd_s, ws_s, c_s,
            qt_s, vt_s, k_s, kr_s, s0_s, s1_s, e_s, p_s, tri_s, wr_s, st_s,
            z_s, a_s, y_s, top_s, at_s, sem):
    ha_w, hb_w, x1_w, o_w, w_w, wo_w, qt_w, vt_w, wg_w, wu_w, wd_w, oa_w, ws_w, k_w, e_w = (
        r.bitcast(I32) for r in (ha_s, hb_s, x1_s, o_s, w_s, wo_s, qt_s, vt_s, wg_s, wu_s, wd_s,
                                 oa_s, ws_s, k_s, e_s))
    s_s = (s0_s, s1_s)
    todo = [(kind, u) for kind in (K, Q, V) for u in range(4)]

    def x_in(lo, hi):
        rows = pl.ds(lo * TM, (hi - lo) * TM)
        return [(x_hbm.at[rows], x_s.at[rows])]

    def w_in(*ns):
        tiles = [(todo[n][0], 2 * todo[n][1] + e) for n in ns for e in range(2)]
        return [(wqkv_hbm.at[:, pl.ds(j * D + g * 128, 128)], w_s.at[j, g]) for j, g in tiles]

    def slabs(src, dst):
        return [(src.at[:, pl.ds(g * 128, 128)], dst.at[g]) for g in range(src.shape[1] // 128)]

    groups = [x_in(0, 1), x_in(1, 2), w_in(0), w_in(1), w_in(2, 3), w_in(4, 5, 6), w_in(7, 8, 9),
              w_in(10, 11) + x_in(2, 3), slabs(wo_hbm, wo_s), x_in(3, NC),
              slabs(wg_hbm, wg_s) + slabs(wu_hbm, wu_s) + slabs(wd_hbm, wd_s)]

    def start(n):
        for src, dst in groups[n]:
            pltpu.make_async_copy(src, dst, sem.at[n]).start()

    def wait(n):
        for src, dst in groups[n]:
            pltpu.make_async_copy(src, dst, sem.at[n]).wait()

    def out_copy(rows):
        return pltpu.make_async_copy(x_s.at[rows], out_hbm.at[rows], sem.at[len(groups)])

    def zero():
        return z_s[0]

    def hide(c):
        return zero() if _static(c) else 0

    def setup():
        row, col = _iota((64, 128), 0), _iota((64, 128), 1)
        tri = jnp.where(2 * row <= col, 0xFFFF, 0) | jnp.where(2 * row + 1 <= col, -65536, 0)
        tri_s[0], tri_s[1] = ~tri, tri
        wr_s[...] = jnp.broadcast_to(wr_ref[...].astype(F32).reshape(1, D), (RB, D))
        z_s[0] = 0
        k_w[0:NHG, 0:48, :] = jnp.zeros((NHG, 48, 128), I32)

    mk = {}

    def make_masks():
        row, col = _iota((32, 128), 0) + zero(), _iota((32, 128), 1) + zero()
        mk["tri"] = row <= (col & 31)
        mk["grp"] = col >> 5
        mk["odd"], mk["high"] = (col[:16] & 32) != 0, col[:16] >= 64

    def lhs(kind, c):
        if _static(c) and c == (NC - 1 if kind == O else 1):
            return hb_s, hb_w
        return (oa_s, oa_w) if kind == O else (ha_s, ha_w)

    def ln_stats(c, j):
        m, _, v = _moments(x_s[_ds(zero() + c * TM + j * RB, RB), :].astype(F32))
        st_s[0, _ds(j * RB, RB)] = jnp.broadcast_to(m, (RB, 128))
        v = jnp.broadcast_to(v, (RB, 128))
        if _static(j):
            st_s[2, 0:RB] = jnp.where(_iota((RB, 128), 1) == j, v, st_s[2, 0:RB]) if j else v
        else:
            st_s[1, _ds(j * RB, RB)] = _inv_std(v)
        return v

    def ln_scales():
        inv = _inv_std(st_s[2, 0:RB])
        for j in range(8):
            st_s[1, j * RB:(j + 1) * RB] = jnp.broadcast_to(inv[:, j:j + 1], (RB, 128))
        return inv

    def stats(c):
        return [P(ln_stats, c, j) for j in range(8)] + [P(ln_scales)]

    def ln_in(c, j):
        def h(b, i):
            r = b * 128 + j * 16
            x = x_s[_ds(zero() + c * TM + r, 16), i * 128:(i + 1) * 128].astype(F32)
            return (x - st_s[0, _ds(r, 16)]) * st_s[1, _ds(r, 16)]

        for i in range(4):
            terms = _lhs_terms(h(0, i), h(0, i + 4), h(1, i), h(1, i + 4))
            for m, a in enumerate(terms):
                lhs(Q, c)[0][m, i, _ds(j * 16, 16), :] = a.astype(BF)
        return jnp.concatenate(terms[:2], 0)

    def prep_o(c, i, e):
        words = [o_w[g, _ds((2 * c + b) * 64 + e * 32, 32), :] for b in range(2) for g in (i, i + 4)]
        for m, a in enumerate(_lhs_terms(*[pltpu.bitcast(w, BF).astype(F32) for w in words])):
            if m in (2, 3):
                lhs(O, c)[1][m, i, e * 32:(e + 1) * 32] = words[3 * (m - 2)]
            else:
                lhs(O, c)[0][m, i, e * 64:(e + 1) * 64] = a.astype(BF)
        return a[32:]

    def prep_w(kind, u, i):
        src, z = (wo_w, zero()) if kind == O else (w_w.at[kind], 0)
        words = [src[z + 2 * u + n % 2, pl.ds((i + 4 * (n // 2)) * 64, 64), :] for n in range(4)]
        tiles = [pltpu.bitcast(w, BF) for w in words]
        if kind in (Q, V):
            tiles = [w.T for w in tiles]
        for m, a in enumerate(_rhs_terms(*[w.astype(F32) for w in tiles])):
            if m in (1, 4):
                ws_w[kind * 4 + u, m, i] = pltpu.bitcast(tiles[m - 1], I32)
            else:
                ws_s[kind * 4 + u, m, i] = a.astype(BF)
        return a[96:]

    def emit(kind, c, b, g, y):
        if kind == Q:
            qt_s[2 * c + b, g] = (y * QSCALE).astype(BF)
        elif kind == K:
            k_s[g, pl.ds(_ds((2 * c + b) * 128, 128).start + 96, 128), :] = y.astype(BF)
        elif kind == V:
            vt_s[2 * c + b, g] = y.astype(BF)
        else:
            rows = _ds((2 * c + b) * 128, 128)
            x1_s[g, rows, :] = (x_s[rows, g * 128:(g + 1) * 128].astype(F32) + y).astype(BF)

    def proj(kind, c, u, m):
        a = _bf16([lhs(kind, c)[1][hide(c) + m, i] for i in range(4)], 1)
        w = [ws_w[kind * 4 + u, m, i] for i in range(4)]
        y = _nt(_bf16(w, 1), a) if kind in (Q, V) else _nn(a, _bf16(w, 0))
        if m == 6:
            c_s[0] = y
        elif m == 4:
            c_s[0] -= y
            c_s[1] = y
        elif m == 2:
            emit(kind, c, 0, 2 * u + 1, c_s[1] + y)
            c_s[3] = y
        elif m == 0:
            c_s[0] += y
            c_s[3] += y
        elif m == 3:
            emit(kind, c, 0, 2 * u, c_s[0] + y)
            c_s[2] = y
        elif m == 1:
            emit(kind, c, 1, 2 * u, c_s[2] + y)
            c_s[3] -= y
        else:
            emit(kind, c, 1, 2 * u + 1, c_s[3] + y)
        return y

    def products(kind, c, u):
        return [P(proj, kind, c, u, m) for m in (6, 4, 2, 0, 3, 1, 5)]

    def k_rep(g, c):
        blocks = [k_w[zero() + g, _ds((c * 8 + i) * 16, 16), :] for i in range(11)]
        for j in range(8):
            r = [blocks[j]] + [pltpu.roll(blocks[j + s], 32 * s, 1) for s in (1, 2, 3)]
            y = [jnp.where(mk["odd"], r[(m + 1) % 4], r[m]) for m in range(4)]
            for h in range(4):
                kr_s[g * 4 + h, _ds((c * 8 + j) * 16, 16), :] = jnp.where(
                    mk["high"], y[(2 - h) % 4], y[-h % 4])

    def qk(g, b, slot):
        lo = max(5 - 4 * b, 0) if _static(b) else 0
        order = ([8] if lo else [0, 8]) + list(range(max(lo, 1), 8))
        for h in range(4):
            q = qt_w[b, g, h * 16:(h + 1) * 16, :]
            w = [jnp.where(mk["grp"][:16] == (p - h) % 4, q, 0) for p in range(4)]
            k = [kr_s[g * 4 + h, _ds(hide(b) + (4 * b - 5 + i) * 16, 16), :] for i in order]
            s = _nn(pltpu.bitcast(jnp.concatenate(k, 0), BF), pltpu.bitcast(jnp.concatenate(w, 0), BF))
            s = {i: s[n * 32:(n + 1) * 32] for n, i in enumerate(order)}
            s[0] = jnp.where(mk["tri"], s.pop(8), NEG if lo else s[0])
            for i in range(lo, lo + 3 if lo else 0):
                s[i] = jnp.where(mk["grp"] >= lo + 3 - i, s[i], NEG)
            m = functools.reduce(jnp.maximum, s.values())
            for i, v in s.items():
                s_s[slot][h, i] = v
            s_s[slot][h, 8, 0:8] = jnp.broadcast_to(jnp.max(m, axis=0, keepdims=True), (8, 128))
        return s

    def softmax(slot, h, live, after):
        m = jnp.concatenate([s_s[slot][zero() + h, 8, 0:8]] * 4, 0)
        l = 0.0
        for n, i in enumerate(live):
            if n // 2 < len(after) and n % 2 == 0:
                s_s[slot][4, 0, 0:8] = after[n // 2]
            p = jnp.exp2(s_s[slot][zero() + h, i] - m)
            e_s[slot * 4 + h, i] = p.astype(BF)
            p = (p[0:8] + p[8:16]) + (p[16:24] + p[24:32])
            l = l + p if n else p
        l = jnp.sum(l, axis=0, keepdims=True)
        none = jnp.zeros((16, 128), I32)
        u = [e_w[slot * 4 + h, i] if i in live else none for i in range(8)]
        u = [jnp.where(mk["odd"], u[(i - 1) % 8], u[i]) for i in range(8)]
        u = [jnp.where(mk["high"], u[(i - 2) % 8], u[i]) for i in range(8)]
        edge = jnp.concatenate(u[:4], 0)
        n = (slot * 4 + h) * 3
        p_s[n] = edge & tri_s[0]
        p_s[n + 1] = jnp.concatenate(u[4:], 0)
        p_s[n + 2] = edge & tri_s[1]
        return 1.0 / l

    def pv(g, b, slot, sums):
        n = min(b + 1, 3) if _static(b) else 3
        outs = []
        for h, linv in enumerate(sums):
            v = _bf16([vt_w[b - i, g, h * 16:(h + 1) * 16, :] for i in range(n - 1, -1, -1)], 1)
            p = _bf16([p_s[(slot * 4 + h) * 3 + i] for i in range(3 - n, 3)], 0)
            outs.append(_nn(v, p) * linv)
        o_s[g, _ds(b * 128, 128), :] = jnp.concatenate(outs, 0).T.astype(BF)

    def route(c, j):
        rows = _ds(zero() + c * (TM // 2) + j * (RB // 2), RB // 2)
        x1 = _bf16([x1_w[g, rows, :] for g in range(8)], 1).astype(F32)
        h = _rb(_ln(x1))
        x_s[_ds(c * TM + j * RB, RB), :] = (x1 + h).astype(BF)
        r = jnp.broadcast_to(_rb(jnp.sum(h * wr_s[...], axis=1, keepdims=True)), (RB, 128))
        top, at = top_s[...], at_s[...]
        for i in range(0, RB, 8):
            better = r[i:i + 8] > top
            top = jnp.where(better, r[i:i + 8], top)
            at = jnp.where(better, c * TM + j * RB + i + _iota((8, 128), 0), at)
        top_s[...], at_s[...] = top, at
        return r

    def argmax():
        top = jnp.max(top_s[...], axis=0, keepdims=True)
        return top[:, 0:1], jnp.min(jnp.where(top_s[...] == top, at_s[...], S - 1)[:, 0:1])

    def block(row):
        return jnp.concatenate([x1_s[g, _ds(row, 16), :] for g in range(8)], 1).astype(F32)

    def glu(hs, t0, n):
        gate, up = (_rb(_nn(hs, _bf16([w[t0 + i] for i in range(n)], 1))) for w in (wg_w, wu_w))
        return gate, (_rb(gate * jax.nn.sigmoid(gate)) * up).astype(BF)

    def release(y, follow):
        follow = [f.func for f in follow]
        for g in range(8) if route in follow else []:
            x1_w[g, S // 2:] = pltpu.bitcast(y[:8], I32)
        if ln_in in follow or ln_stats in follow:
            x_s[S:, :] = jnp.concatenate([y[:16]] * 8, 1).astype(BF)
        if k_rep in follow:
            k_w[NHG, 0:8] = pltpu.bitcast(y[:8], I32)
        if prep_w in follow:
            wo_s[8, 0:16] = y[:16].astype(BF)

    def overlap(main, side, spare, lag):
        due = {}
        for n, f in enumerate(main):
            for e, v in enumerate(due.pop(n, [])):
                spare[e % 2 * 32:e % 2 * 32 + 32] = pltpu.bitcast(v, I32)
            release(f()[:, 0:128], side.get(n, []))
            due[n + lag] = [g() for g in side.get(n, [])]

    def stage(t, qkv=True, out=True, load=False):
        make_masks()
        slots = [[] for _ in range(65)]
        nd = 16 if qkv and out else 0
        if load:
            _spread(slots, [P(prep_w, O, u, i) for u in range(4) for i in range(4)], 2, 66)
        if qkv and out:
            _spread(slots, [P(ln_in, t + 1, j) for j in range(8)], 0, 12)
        if qkv and not load:
            c = (t + 2) & (NC - 1)
            _spread(slots, stats(c), 13, 31)
            _spread(slots, [P(k_rep, g, t + 1) for g in range(NHG)], 29, 61)
        if qkv and out:
            _spread(slots, [P(route, t - 1, j) for j in range(8)], 32, 64)
        for i in range(4):
            for e in range(2):
                slots[min(16 * i + 19 + 4 * e, 64)].append(P(prep_o, t, i, e))
        fs = [f for u in range(4) for f in products(O, t - 1, u)] if out else []
        if qkv:
            _spread(slots, fs, 0, nd)
            fs = [f for kind, u in todo[8 * load:] for f in products(kind, t + 1, u)]
        _spread(slots, fs[:-2], nd, 64)
        slots[64] += fs[-2:]

        quads = [(i + g, 2 * t + b) for i in range(4) for g in (0, 4) for b in range(2)]
        due, after = {}, []
        nxt = qk(*quads[0], 0)
        for n, quad in enumerate(quads):
            live = sorted(nxt)
            if n + 1 < len(quads):
                nxt = qk(*quads[n + 1], (n + 1) % 2)
            sums, y = [], None
            for i in range(4 * n, 4 * n + 4):
                if (load or not qkv) and n + 1 < len(quads) and i % 4:
                    after = [nxt[sorted(nxt)[(i % 4 - 1) * len(nxt) // 4]][:8]]
                sums.append(softmax(n % 2, i % 4, live, after))
                ys, after = [], []
                for f in slots[i]:
                    if f.func in (route, ln_in, ln_stats, ln_scales, prep_w, prep_o):
                        due.setdefault(i + 2, []).append(f())
                    elif f.func is proj:
                        y = f()
                        ys.append(y)
                    else:
                        f()
                scores = s_s[(i + 1) // 4 % 2]
                for e, v in enumerate(due.pop(i, []) if i < 63 else []):
                    scores[4, 1 + e] = v
                if y is not None and i < 63:
                    if qkv and not load:
                        after = [ys[0][r:r + 8] for r in range(0, 128, 32)]
                    release(y[64:], slots[i + 1])
            pv(*quad, n % 2, sums)
        for f in slots[64]:
            f()

    def interleave(main, side):
        step = -(-len(side) // len(main))
        for n, f in enumerate(main):
            now = side[n * step:(n + 1) * step]
            release(f(), now)
            for g in now:
                g()

    def first_chunk(load):
        norm = stats(1) + [P(ln_in, 1, j) for j in range(8)]
        if load:
            start(0)
            setup()
            start(1)
            for n, fs in enumerate((stats(0) + [P(ln_in, 0, j) for j in range(8)], norm,
                                    [P(prep_w, *todo[0], i) for i in range(4)])):
                wait(n)
                start(n + 2)
                for f in fs:
                    f()
        make_masks()
        for n, (kind, u) in enumerate(todo):
            main, side = products(kind, 0, u), [P(k_rep, n - 4, 0)] if n >= 4 else []
            if not load:
                side += norm[max(n - 6, 0) * 3:max(n - 5, 0) * 3]
            else:
                if n == 0:
                    interleave(main, [])
                    main = []
                if n in (0, 1, 3, 6, 9):
                    group = (0, 1, 3, 6, 9).index(n) + 3
                    wait(group)
                    start(group + 2)
                side = [P(prep_w, *todo[n + 1], i) for i in range(4)] if n < 11 else stats(2)
                if n < 8:
                    main += products(kind, 1, u)
                if 1 <= n <= 8:
                    side += [P(k_rep, n - 1, c) for c in range(2)]
            interleave(main, side)
        if load:
            wait(8)

    def finish(first):
        route(NC - 2, 0)
        overlap([f for u in range(4) for f in products(O, NC - 1, u)],
                {j * 11 // 4 - 1: [P(route, NC - 2, j)] for j in range(1, 8)}, hb_w.at[7, 0], 6)

        guess = argmax()[1] // 16 * 16
        hs = _ln(block(guess)).astype(BF)
        if not first:
            out_copy(_ds(S - 2 * TM, TM)).start()
        acts = []
        route(NC - 1, 0)
        route(NC - 1, 1)

        def up(j):
            gate, a = glu(hs, zero() + 4 * j, 4)
            acts.append(a)
            return gate

        def down(j):
            y = _nn(acts[j], _bf16([wd_w[zero() + g, j * 256:(j + 1) * 256] for g in range(8)], 1))
            y_s[...] = y_s[...] + y if j else y
            return y

        overlap([P(up, j) for j in range(7)],
                {j: [P(route, NC - 1, j + 2)] for j in range(6)}, wg_w.at[F // 128], 2)
        rmax, idx = argmax()
        base = idx // 16 * 16
        side = {}
        if first:
            ln_in(0, 0)
            ln_in(0, 1)
            side = {n: [P(ln_in, 0, n + 2)] for n in range(6)}
        else:
            out_copy(_ds(S - TM, TM)).start()
        overlap([P(down, j) for j in range(7)], side, wd_w.at[8], 2)
        x1 = block(base)
        hs = _ln(x1).astype(BF)

        def up_again(j, _):
            a_s[j] = glu(hs, 7 * j, 7)[1]

        def down_again(j, _):
            a = jnp.concatenate([a_s[i, :, :] for i in range(4)], 1)
            y_s[:, _ds(j * 512, 512)] = _nn(a, _bf16([wd_w[4 * j + g] for g in range(4)], 1))

        lax.fori_loop(0, jnp.where(base == guess, 0, 4), up_again, None)
        lax.fori_loop(0, jnp.where(base == guess, 0, 2), down_again, None)
        y = _rb(_rb(y_s[...]) * _rb(jax.nn.sigmoid(rmax)))
        upd = jnp.where(_iota((16, D), 0) == idx - base, y, 0.0)
        new = (x1 + _rb(hs.astype(F32) + upd)).astype(BF)
        if first:
            x_s[_ds(base, 16), :] = new

            @pl.when(base < TM)
            def _():
                ln_stats(0, base // RB)
                ln_in(0, base % 128 // 16)
        else:
            for c in range(NC):
                out_copy(_ds(c * TM, TM)).wait()
            x_s[_ds(base, 16), :] = new
            out_copy(_ds(base, 16)).start()
            out_copy(_ds(base, 16)).wait()

    def layer(first):
        first_chunk(first)
        top_s[...] = jnp.full((8, 128), -jnp.inf, F32)
        at_s[...] = _iota((8, 128), 0)
        stage(0, out=False, load=first)
        if first:
            wait(9)
            start(10)

        def body(t, _):
            stage(t)
            if not first:
                out_copy(_ds((t - 1) * TM, TM)).start()

        lax.fori_loop(1, NC - 1, body, None)
        if first:
            wait(10)
        stage(NC - 1, qkv=False)
        finish(first)

    layer(True)
    layer(False)


@jax.jit
def pallas_interleave_layers__sliding_block__moe_arch_mod__prompt_kernel(
    A_x: jax.Array,
    A_wqkv: jax.Array,
    A_wo: jax.Array,
    B_x: jax.Array,
    B_w_r: jax.Array,
    B_w_gate: jax.Array,
    B_w_up: jax.Array,
    B_w_down: jax.Array,
):
    del B_x
    hbm = pl.BlockSpec(memory_space=pl.ANY)
    out = pl.pallas_call(
        _kernel,
        out_shape=jax.ShapeDtypeStruct((S, D), BF),
        in_specs=[pl.BlockSpec(memory_space=pltpu.VMEM)] + [hbm] * 6,
        out_specs=hbm,
        scratch_shapes=[
            pltpu.VMEM((S + 16, D), BF),
            pltpu.VMEM((8, S + 16, 128), BF),
            pltpu.VMEM((7, 4, 128, 128), BF),
            pltpu.VMEM((8, 4, 128, 128), BF),
            pltpu.VMEM((7, 4, 128, 128), BF),
            pltpu.VMEM((NHG, S, 128), BF),
            pltpu.VMEM((3, NHG, D, 128), BF),
            pltpu.VMEM((9, D, 128), BF),
            pltpu.VMEM((F // 128 + 1, D, 128), BF),
            pltpu.VMEM((F // 128, D, 128), BF),
            pltpu.VMEM((9, F, 128), BF),
            pltpu.VMEM((16, 7, 4, 128, 128), BF),
            pltpu.VMEM((4, 128, 128), F32),
            pltpu.VMEM((NQB, NHG, 128, 128), BF),
            pltpu.VMEM((NQB, NHG, 128, 128), BF),
            pltpu.VMEM((NHG + 1, 128 + S, 128), BF),
            pltpu.VMEM((32, 64 * 16, 128), I32),
            pltpu.VMEM((5, 9, 32, 128), F32),
            pltpu.VMEM((5, 9, 32, 128), F32),
            pltpu.VMEM((8, 8, 32, 128), BF),
            pltpu.VMEM((24, 64, 128), I32),
            pltpu.VMEM((2, 64, 128), I32),
            pltpu.VMEM((RB, D), F32),
            pltpu.VMEM((3, TM, 128), F32),
            pltpu.SMEM((1,), I32),
            pltpu.VMEM((4, 16, F // 4), BF),
            pltpu.VMEM((16, D), F32),
            pltpu.VMEM((8, 128), F32),
            pltpu.VMEM((8, 128), I32),
            pltpu.SemaphoreType.DMA((12,)),
        ],
        compiler_params=pltpu.CompilerParams(vmem_limit_bytes=110 * 1024 * 1024),
    )(B_w_r, A_x.reshape(S, D), A_wqkv, A_wo, B_w_gate, B_w_up, B_w_down)
    return out.reshape(1, S, D)
```

```python
import functools

import jax
import jax.numpy as jnp
import numpy as np
from jax import lax
import jax.experimental.pallas as pl
import jax.experimental.pallas.tpu as pltpu

S, D, F = 2048, 1024, 3584
NHG = 8
NQB = S // 128
TM = 256
NC = S // TM
RB = TM // 8
Q, K, V, O = range(4)
BF, F32, I32 = jnp.bfloat16, jnp.float32, jnp.int32
NEG = -1e9

_bf = lambda v: float(np.asarray(v, dtype=jnp.bfloat16).astype(np.float32))
QSCALE = _bf(32 ** -0.5) * float(np.log2(np.e))
EPS = _bf(1e-5)
P = functools.partial


def _rb(x):
    return x.astype(BF).astype(F32)


def _moments(x):
    m = jnp.mean(x, axis=1, keepdims=True)
    xc = x - m
    return m, xc, jnp.mean(xc * xc, axis=1, keepdims=True)


def _inv_std(v):
    return 1.0 / _rb(jnp.sqrt(_rb(_rb(v) + EPS)))


def _ln(x):
    _, xc, v = _moments(x)
    return xc * _inv_std(v)


def _nt(a, b):
    return lax.dot_general(a, b, (((1,), (1,)), ((), ())), preferred_element_type=F32)


def _nn(a, b):
    return jnp.dot(a, b, preferred_element_type=F32)


def _bf16(words, axis):
    return jnp.concatenate([pltpu.bitcast(w, BF) for w in words], axis)


def _lhs_terms(a11, a12, a21, a22):
    return [a11 + a22, a21 + a22, a11, a22, a11 + a12, a21 - a11, a12 - a22]


def _rhs_terms(b11, b12, b21, b22):
    return [b11 + b22, b11, b12 - b22, b21 - b11, b22, b11 + b12, b21 + b22]


def _static(i):
    return isinstance(i, int)


def _ds(start, size):
    return pl.ds(start if _static(start) else pl.multiple_of(start, size), size)


def _iota(shape, d):
    return lax.broadcasted_iota(I32, shape, d)


def _spread(slots, pieces, lo, hi):
    for i, f in enumerate(pieces):
        slots[lo + i * (hi - lo) // len(pieces)].append(f)


def _kernel(wr_ref, x_hbm, wqkv_hbm, wo_hbm, wg_hbm, wu_hbm, wd_hbm, out_hbm,
            x_s, x1_s, ha_s, hb_s, oa_s, o_s, w_s, wo_s, wg_s, wu_s, wd_s, ws_s, c_s,
            qt_s, vt_s, k_s, kr_s, s0_s, s1_s, e_s, p_s, tri_s, wr_s, st_s,
            z_s, a_s, y_s, top_s, at_s, sem):
    ha_w, hb_w, x1_w, o_w, w_w, wo_w, qt_w, vt_w, wg_w, wu_w, wd_w, oa_w, ws_w, k_w, e_w = (
        r.bitcast(I32) for r in (ha_s, hb_s, x1_s, o_s, w_s, wo_s, qt_s, vt_s, wg_s, wu_s, wd_s,
                                 oa_s, ws_s, k_s, e_s))
    s_s = (s0_s, s1_s)
    todo = [(kind, u) for kind in (K, Q, V) for u in range(4)]

    def x_in(lo, hi):
        rows = pl.ds(lo * TM, (hi - lo) * TM)
        return [(x_hbm.at[rows], x_s.at[rows])]

    def w_in(*ns):
        tiles = [(todo[n][0], 2 * todo[n][1] + e) for n in ns for e in range(2)]
        return [(wqkv_hbm.at[:, pl.ds(j * D + g * 128, 128)], w_s.at[j, g]) for j, g in tiles]

    def slabs(src, dst):
        return [(src.at[:, pl.ds(g * 128, 128)], dst.at[g]) for g in range(src.shape[1] // 128)]

    groups = [x_in(0, 1), x_in(1, 2), w_in(0), w_in(1), w_in(2, 3), w_in(4, 5, 6), w_in(7, 8, 9),
              w_in(10, 11) + x_in(2, 3), slabs(wo_hbm, wo_s), x_in(3, NC),
              slabs(wg_hbm, wg_s) + slabs(wu_hbm, wu_s) + slabs(wd_hbm, wd_s)]

    def start(n):
        for src, dst in groups[n]:
            pltpu.make_async_copy(src, dst, sem.at[n]).start()

    def wait(n):
        for src, dst in groups[n]:
            pltpu.make_async_copy(src, dst, sem.at[n]).wait()

    def out_copy(rows):
        return pltpu.make_async_copy(x_s.at[rows], out_hbm.at[rows], sem.at[len(groups)])

    def zero():
        return z_s[0]

    def hide(c):
        return zero() if _static(c) else 0

    def setup():
        row, col = _iota((64, 128), 0), _iota((64, 128), 1)
        tri = jnp.where(2 * row <= col, 0xFFFF, 0) | jnp.where(2 * row + 1 <= col, -65536, 0)
        tri_s[0], tri_s[1] = ~tri, tri
        wr_s[...] = jnp.broadcast_to(wr_ref[...].astype(F32).reshape(1, D), (RB, D))
        z_s[0] = 0
        k_w[0:NHG, 0:48, :] = jnp.zeros((NHG, 48, 128), I32)

    mk = {}

    def make_masks():
        row, col = _iota((32, 128), 0) + zero(), _iota((32, 128), 1) + zero()
        mk["tri"] = row <= (col & 31)
        mk["grp"] = col >> 5
        mk["odd"], mk["high"] = (col[:16] & 32) != 0, col[:16] >= 64

    def lhs(kind, c):
        if _static(c) and c == (NC - 1 if kind == O else 1):
            return hb_s, hb_w
        return (oa_s, oa_w) if kind == O else (ha_s, ha_w)

    def ln_stats(c, j):
        m, _, v = _moments(x_s[_ds(zero() + c * TM + j * RB, RB), :].astype(F32))
        st_s[0, _ds(j * RB, RB)] = jnp.broadcast_to(m, (RB, 128))
        v = jnp.broadcast_to(v, (RB, 128))
        if _static(j):
            st_s[2, 0:RB] = jnp.where(_iota((RB, 128), 1) == j, v, st_s[2, 0:RB]) if j else v
        else:
            st_s[1, _ds(j * RB, RB)] = _inv_std(v)
        return v

    def ln_scales():
        inv = _inv_std(st_s[2, 0:RB])
        for j in range(8):
            st_s[1, j * RB:(j + 1) * RB] = jnp.broadcast_to(inv[:, j:j + 1], (RB, 128))
        return inv

    def stats(c):
        return [P(ln_stats, c, j) for j in range(8)] + [P(ln_scales)]

    def ln_in(c, j):
        def h(b, i):
            r = b * 128 + j * 16
            x = x_s[_ds(zero() + c * TM + r, 16), i * 128:(i + 1) * 128].astype(F32)
            return (x - st_s[0, _ds(r, 16)]) * st_s[1, _ds(r, 16)]

        for i in range(4):
            terms = _lhs_terms(h(0, i), h(0, i + 4), h(1, i), h(1, i + 4))
            for m, a in enumerate(terms):
                lhs(Q, c)[0][m, i, _ds(j * 16, 16), :] = a.astype(BF)
        return jnp.concatenate(terms[:2], 0)

    def prep_o(c, i, e):
        words = [o_w[g, _ds((2 * c + b) * 64 + e * 32, 32), :] for b in range(2) for g in (i, i + 4)]
        for m, a in enumerate(_lhs_terms(*[pltpu.bitcast(w, BF).astype(F32) for w in words])):
            if m in (2, 3):
                lhs(O, c)[1][m, i, e * 32:(e + 1) * 32] = words[3 * (m - 2)]
            else:
                lhs(O, c)[0][m, i, e * 64:(e + 1) * 64] = a.astype(BF)
        return a[32:]

    def prep_w(kind, u, i):
        src, z = (wo_w, zero()) if kind == O else (w_w.at[kind], 0)
        words = [src[z + 2 * u + n % 2, pl.ds((i + 4 * (n // 2)) * 64, 64), :] for n in range(4)]
        tiles = [pltpu.bitcast(w, BF) for w in words]
        if kind in (Q, V):
            tiles = [w.T for w in tiles]
        for m, a in enumerate(_rhs_terms(*[w.astype(F32) for w in tiles])):
            if m in (1, 4):
                ws_w[kind * 4 + u, m, i] = pltpu.bitcast(tiles[m - 1], I32)
            else:
                ws_s[kind * 4 + u, m, i] = a.astype(BF)
        return a[96:]

    def emit(kind, c, b, g, y):
        if kind == Q:
            qt_s[2 * c + b, g] = (y * QSCALE).astype(BF)
        elif kind == K:
            k_s[g, pl.ds(_ds((2 * c + b) * 128, 128).start + 96, 128), :] = y.astype(BF)
        elif kind == V:
            vt_s[2 * c + b, g] = y.astype(BF)
        else:
            rows = _ds((2 * c + b) * 128, 128)
            x1_s[g, rows, :] = (x_s[rows, g * 128:(g + 1) * 128].astype(F32) + y).astype(BF)

    def proj(kind, c, u, m):
        a = _bf16([lhs(kind, c)[1][hide(c) + m, i] for i in range(4)], 1)
        w = [ws_w[kind * 4 + u, m, i] for i in range(4)]
        y = _nt(_bf16(w, 1), a) if kind in (Q, V) else _nn(a, _bf16(w, 0))
        if m == 6:
            c_s[0] = y
        elif m == 4:
            c_s[0] -= y
            c_s[1] = y
        elif m == 2:
            emit(kind, c, 0, 2 * u + 1, c_s[1] + y)
            c_s[3] = y
        elif m == 0:
            c_s[0] += y
            c_s[3] += y
        elif m == 3:
            emit(kind, c, 0, 2 * u, c_s[0] + y)
            c_s[2] = y
        elif m == 1:
            emit(kind, c, 1, 2 * u, c_s[2] + y)
            c_s[3] -= y
        else:
            emit(kind, c, 1, 2 * u + 1, c_s[3] + y)
        return y

    def products(kind, c, u):
        return [P(proj, kind, c, u, m) for m in (6, 4, 2, 0, 3, 1, 5)]

    def k_rep(g, c):
        blocks = [k_w[zero() + g, _ds((c * 8 + i) * 16, 16), :] for i in range(11)]
        for j in range(8):
            r = [blocks[j]] + [pltpu.roll(blocks[j + s], 32 * s, 1) for s in (1, 2, 3)]
            y = [jnp.where(mk["odd"], r[(m + 1) % 4], r[m]) for m in range(4)]
            for h in range(4):
                kr_s[g * 4 + h, _ds((c * 8 + j) * 16, 16), :] = jnp.where(
                    mk["high"], y[(2 - h) % 4], y[-h % 4])

    def qk(g, b, slot):
        lo = max(5 - 4 * b, 0) if _static(b) else 0
        order = ([8] if lo else [0, 8]) + list(range(max(lo, 1), 8))
        for h in range(4):
            q = qt_w[b, g, h * 16:(h + 1) * 16, :]
            w = [jnp.where(mk["grp"][:16] == (p - h) % 4, q, 0) for p in range(4)]
            k = [kr_s[g * 4 + h, _ds(hide(b) + (4 * b - 5 + i) * 16, 16), :] for i in order]
            s = _nn(pltpu.bitcast(jnp.concatenate(k, 0), BF), pltpu.bitcast(jnp.concatenate(w, 0), BF))
            s = {i: s[n * 32:(n + 1) * 32] for n, i in enumerate(order)}
            s[0] = jnp.where(mk["tri"], s.pop(8), NEG if lo else s[0])
            for i in range(lo, lo + 3 if lo else 0):
                s[i] = jnp.where(mk["grp"] >= lo + 3 - i, s[i], NEG)
            m = functools.reduce(jnp.maximum, s.values())
            for i, v in s.items():
                s_s[slot][h, i] = v
            s_s[slot][h, 8, 0:8] = jnp.broadcast_to(jnp.max(m, axis=0, keepdims=True), (8, 128))
        return s

    def softmax(slot, h, live, after):
        m = jnp.concatenate([s_s[slot][zero() + h, 8, 0:8]] * 4, 0)
        l = 0.0
        for n, i in enumerate(live):
            if n // 2 < len(after) and n % 2 == 0:
                s_s[slot][4, 0, 0:8] = after[n // 2]
            p = jnp.exp2(s_s[slot][zero() + h, i] - m)
            e_s[slot * 4 + h, i] = p.astype(BF)
            p = (p[0:8] + p[8:16]) + (p[16:24] + p[24:32])
            l = l + p if n else p
        l = jnp.sum(l, axis=0, keepdims=True)
        none = jnp.zeros((16, 128), I32)
        u = [e_w[slot * 4 + h, i] if i in live else none for i in range(8)]
        u = [jnp.where(mk["odd"], u[(i - 1) % 8], u[i]) for i in range(8)]
        u = [jnp.where(mk["high"], u[(i - 2) % 8], u[i]) for i in range(8)]
        edge = jnp.concatenate(u[:4], 0)
        n = (slot * 4 + h) * 3
        p_s[n] = edge & tri_s[0]
        p_s[n + 1] = jnp.concatenate(u[4:], 0)
        p_s[n + 2] = edge & tri_s[1]
        return 1.0 / l

    def pv(g, b, slot, sums):
        n = min(b + 1, 3) if _static(b) else 3
        outs = []
        for h, linv in enumerate(sums):
            v = _bf16([vt_w[b - i, g, h * 16:(h + 1) * 16, :] for i in range(n - 1, -1, -1)], 1)
            p = _bf16([p_s[(slot * 4 + h) * 3 + i] for i in range(3 - n, 3)], 0)
            outs.append(_nn(v, p) * linv)
        o_s[g, _ds(b * 128, 128), :] = jnp.concatenate(outs, 0).T.astype(BF)

    def route(c, j):
        rows = _ds(zero() + c * (TM // 2) + j * (RB // 2), RB // 2)
        x1 = _bf16([x1_w[g, rows, :] for g in range(8)], 1).astype(F32)
        h = _rb(_ln(x1))
        x_s[_ds(c * TM + j * RB, RB), :] = (x1 + h).astype(BF)
        r = jnp.broadcast_to(_rb(jnp.sum(h * wr_s[...], axis=1, keepdims=True)), (RB, 128))
        top, at = top_s[...], at_s[...]
        for i in range(0, RB, 8):
            better = r[i:i + 8] > top
            top = jnp.where(better, r[i:i + 8], top)
            at = jnp.where(better, c * TM + j * RB + i + _iota((8, 128), 0), at)
        top_s[...], at_s[...] = top, at
        return r

    def argmax():
        top = jnp.max(top_s[...], axis=0, keepdims=True)
        return top[:, 0:1], jnp.min(jnp.where(top_s[...] == top, at_s[...], S - 1)[:, 0:1])

    def block(row):
        return jnp.concatenate([x1_s[g, _ds(row, 16), :] for g in range(8)], 1).astype(F32)

    def glu(hs, t0, n):
        gate, up = (_rb(_nn(hs, _bf16([w[t0 + i] for i in range(n)], 1))) for w in (wg_w, wu_w))
        return gate, (_rb(gate * jax.nn.sigmoid(gate)) * up).astype(BF)

    def release(y, follow):
        follow = [f.func for f in follow]
        for g in range(8) if route in follow else []:
            x1_w[g, S // 2:] = pltpu.bitcast(y[:8], I32)
        if ln_in in follow or ln_stats in follow:
            x_s[S:, :] = jnp.concatenate([y[:16]] * 8, 1).astype(BF)
        if k_rep in follow:
            k_w[NHG, 0:8] = pltpu.bitcast(y[:8], I32)
        if prep_w in follow:
            wo_s[8, 0:16] = y[:16].astype(BF)

    def overlap(main, side, spare, lag):
        due = {}
        for n, f in enumerate(main):
            for e, v in enumerate(due.pop(n, [])):
                spare[e % 2 * 32:e % 2 * 32 + 32] = pltpu.bitcast(v, I32)
            release(f()[:, 0:128], side.get(n, []))
            due[n + lag] = [v for v in [g() for g in side.get(n, [])] if v is not None]

    def stage(t, qkv=True, out=True, load=False):
        make_masks()
        slots = [[] for _ in range(65)]
        nd = 16 if qkv and out else 0
        if load:
            _spread(slots, [P(prep_w, O, u, i) for u in range(4) for i in range(4)], 2, 66)
        if qkv and out:
            _spread(slots, [P(ln_in, t + 1, j) for j in range(8)], 0, 12)
        if qkv and not load:
            c = (t + 2) & (NC - 1)
            _spread(slots, stats(c), 13, 31)
            _spread(slots, [P(k_rep, g, t + 1) for g in range(NHG)], 29, 61)
        if qkv and out:
            _spread(slots, [P(route, t - 1, j) for j in range(8)], 32, 64)
        for i in range(4):
            for e in range(2):
                slots[min(16 * i + 19 + 4 * e, 64)].append(P(prep_o, t, i, e))
        fs = [f for u in range(4) for f in products(O, t - 1, u)] if out else []
        if qkv:
            _spread(slots, fs, 0, nd)
            fs = [f for kind, u in todo[8 * load:] for f in products(kind, t + 1, u)]
        _spread(slots, fs[:-2], nd, 64)
        slots[64] += fs[-2:]

        quads = [(i + g, 2 * t + b) for i in range(4) for g in (0, 4) for b in range(2)]
        due, after = {}, []
        nxt = qk(*quads[0], 0)
        for n, quad in enumerate(quads):
            live = sorted(nxt)
            if n + 1 < len(quads):
                nxt = qk(*quads[n + 1], (n + 1) % 2)
            sums, y = [], None
            for i in range(4 * n, 4 * n + 4):
                if (load or not qkv) and n + 1 < len(quads) and i % 4:
                    after = [nxt[sorted(nxt)[(i % 4 - 1) * len(nxt) // 4]][:8]]
                sums.append(softmax(n % 2, i % 4, live, after))
                ys, after = [], []
                for f in slots[i]:
                    if f.func in (route, ln_in, ln_stats, ln_scales, prep_w, prep_o):
                        due.setdefault(i + 2, []).append(f())
                    elif f.func is proj:
                        y = f()
                        ys.append(y)
                    else:
                        f()
                scores = s_s[(i + 1) // 4 % 2]
                for e, v in enumerate(due.pop(i, []) if i < 63 else []):
                    scores[4, 1 + e] = v
                if y is not None and i < 63:
                    if qkv and not load:
                        after = [ys[0][r:r + 8] for r in range(0, 128, 32)]
                    release(y[64:], slots[i + 1])
            pv(*quad, n % 2, sums)
        for f in slots[64]:
            f()

    def interleave(main, side):
        step = -(-len(side) // len(main))
        for n, f in enumerate(main):
            now = side[n * step:(n + 1) * step]
            release(f(), now)
            for g in now:
                g()

    def normalise(c):
        return stats(c) + [P(ln_in, c, j) for j in range(8)]

    def load_and_project():
        start(0)
        setup()
        start(1)
        for n, fs in enumerate((normalise(0), normalise(1),
                                [P(prep_w, *todo[0], i) for i in range(4)])):
            wait(n)
            start(n + 2)
            for f in fs:
                f()
        make_masks()
        for n, (kind, u) in enumerate(todo):
            main = products(kind, 0, u)
            if n == 0:
                interleave(main, [])
                main = []
            if n in (0, 1, 3, 6, 9):
                group = (0, 1, 3, 6, 9).index(n) + 3
                wait(group)
                start(group + 2)
            side = [P(prep_w, *todo[n + 1], i) for i in range(4)] if n < 11 else stats(2)
            if n < 8:
                main += products(kind, 1, u)
            if 1 <= n <= 8:
                side += [P(k_rep, n - 1, c) for c in range(2)]
            interleave(main, side)
        wait(8)

    def project():
        make_masks()
        side = {1 + 4 * n: [f] for n, f in enumerate(normalise(1))}
        for g in range(NHG):
            side.setdefault(11 + 8 * g, []).append(P(k_rep, g, 0))
        overlap([f for kind, u in todo for f in products(kind, 0, u)], side, ha_w.at[7, 0], 5)

    def finish(first):
        route(NC - 2, 0)
        overlap([f for u in range(4) for f in products(O, NC - 1, u)],
                {j * 11 // 4 - 1: [P(route, NC - 2, j)] for j in range(1, 8)}, hb_w.at[7, 0], 6)

        guess = argmax()[1] // 16 * 16
        hs = _ln(block(guess)).astype(BF)
        if not first:
            out_copy(_ds(S - 2 * TM, TM)).start()
        acts = []
        route(NC - 1, 0)
        route(NC - 1, 1)

        def up(j):
            gate, a = glu(hs, zero() + 4 * j, 4)
            acts.append(a)
            return gate

        def down(j):
            y = _nn(acts[j], _bf16([wd_w[zero() + g, j * 256:(j + 1) * 256] for g in range(8)], 1))
            y_s[...] = y_s[...] + y if j else y
            return y

        overlap([P(up, j) for j in range(7)],
                {j: [P(route, NC - 1, j + 2)] for j in range(6)}, wg_w.at[F // 128], 2)
        rmax, idx = argmax()
        base = idx // 16 * 16
        side = {}
        if first:
            ln_in(0, 0)
            ln_in(0, 1)
            side = {n: [P(ln_in, 0, n + 2)] for n in range(6)}
        else:
            out_copy(_ds(S - TM, TM)).start()
        overlap([P(down, j) for j in range(7)], side, wd_w.at[8], 2)
        x1 = block(base)
        hs = _ln(x1).astype(BF)

        def up_again(j, _):
            a_s[j] = glu(hs, 7 * j, 7)[1]

        def down_again(j, _):
            a = jnp.concatenate([a_s[i, :, :] for i in range(4)], 1)
            y_s[:, _ds(j * 512, 512)] = _nn(a, _bf16([wd_w[4 * j + g] for g in range(4)], 1))

        lax.fori_loop(0, jnp.where(base == guess, 0, 4), up_again, None)
        lax.fori_loop(0, jnp.where(base == guess, 0, 2), down_again, None)
        y = _rb(_rb(y_s[...]) * _rb(jax.nn.sigmoid(rmax)))
        upd = jnp.where(_iota((16, D), 0) == idx - base, y, 0.0)
        new = (x1 + _rb(hs.astype(F32) + upd)).astype(BF)
        if first:
            x_s[_ds(base, 16), :] = new

            @pl.when(base < TM)
            def _():
                ln_stats(0, base // RB)
                ln_in(0, base % 128 // 16)
        else:
            for c in range(NC):
                out_copy(_ds(c * TM, TM)).wait()
            x_s[_ds(base, 16), :] = new
            out_copy(_ds(base, 16)).start()
            out_copy(_ds(base, 16)).wait()

    def layer(first):
        (load_and_project if first else project)()
        top_s[...] = jnp.full((8, 128), -jnp.inf, F32)
        at_s[...] = _iota((8, 128), 0)
        stage(0, out=False, load=first)
        if first:
            wait(9)
            start(10)

        def body(t, _):
            stage(t)
            if not first:
                out_copy(_ds((t - 1) * TM, TM)).start()

        lax.fori_loop(1, NC - 1, body, None)
        if first:
            wait(10)
        stage(NC - 1, qkv=False)
        finish(first)

    layer(True)
    layer(False)


@jax.jit
def pallas_interleave_layers__sliding_block__moe_arch_mod__prompt_kernel(
    A_x: jax.Array,
    A_wqkv: jax.Array,
    A_wo: jax.Array,
    B_x: jax.Array,
    B_w_r: jax.Array,
    B_w_gate: jax.Array,
    B_w_up: jax.Array,
    B_w_down: jax.Array,
):
    del B_x
    hbm = pl.BlockSpec(memory_space=pl.ANY)
    out = pl.pallas_call(
        _kernel,
        out_shape=jax.ShapeDtypeStruct((S, D), BF),
        in_specs=[pl.BlockSpec(memory_space=pltpu.VMEM)] + [hbm] * 6,
        out_specs=hbm,
        scratch_shapes=[
            pltpu.VMEM((S + 16, D), BF),
            pltpu.VMEM((8, S + 16, 128), BF),
            pltpu.VMEM((8, 4, 128, 128), BF),
            pltpu.VMEM((8, 4, 128, 128), BF),
            pltpu.VMEM((7, 4, 128, 128), BF),
            pltpu.VMEM((NHG, S, 128), BF),
            pltpu.VMEM((3, NHG, D, 128), BF),
            pltpu.VMEM((9, D, 128), BF),
            pltpu.VMEM((F // 128 + 1, D, 128), BF),
            pltpu.VMEM((F // 128, D, 128), BF),
            pltpu.VMEM((9, F, 128), BF),
            pltpu.VMEM((16, 7, 4, 128, 128), BF),
            pltpu.VMEM((4, 128, 128), F32),
            pltpu.VMEM((NQB, NHG, 128, 128), BF),
            pltpu.VMEM((NQB, NHG, 128, 128), BF),
            pltpu.VMEM((NHG + 1, 128 + S, 128), BF),
            pltpu.VMEM((32, 64 * 16, 128), I32),
            pltpu.VMEM((5, 9, 32, 128), F32),
            pltpu.VMEM((5, 9, 32, 128), F32),
            pltpu.VMEM((8, 8, 32, 128), BF),
            pltpu.VMEM((24, 64, 128), I32),
            pltpu.VMEM((2, 64, 128), I32),
            pltpu.VMEM((RB, D), F32),
            pltpu.VMEM((3, TM, 128), F32),
            pltpu.SMEM((1,), I32),
            pltpu.VMEM((4, 16, F // 4), BF),
            pltpu.VMEM((16, D), F32),
            pltpu.VMEM((8, 128), F32),
            pltpu.VMEM((8, 128), I32),
            pltpu.SemaphoreType.DMA((12,)),
        ],
        compiler_params=pltpu.CompilerParams(vmem_limit_bytes=110 * 1024 * 1024),
    )(B_w_r, A_x.reshape(S, D), A_wqkv, A_wo, B_w_gate, B_w_up, B_w_down)
    return out.reshape(1, S, D)
```
